```python
import jax
import jax.numpy as jnp

def _softmax(x, axis=-1):
    return jax.nn.softmax(x, axis=axis)

def _gelu(x):
    return jax.nn.gelu(x, approximate=True)

def _silu(x):
    return jax.nn.silu(x)

def _sigmoid(x):
    return jax.nn.sigmoid(x)

def _layernorm(x, axis=-1, eps=1e-05):
    m = jnp.mean(x, axis=axis, keepdims=True)
    v = jnp.var(x, axis=axis, keepdims=True)
    return (x - m) / jnp.sqrt(v + eps)

def _scatter_add(tgt, idx, src, axis=0):
    return tgt.at[idx].add(src)

def _segment_sum(src, seg, n):
    return jax.ops.segment_sum(src, seg, n)

class _Rng:

    def __init__(self, key):
        self._k = key

    def _next(self):
        self._k, sub = jax.random.split(self._k)
        return sub

    def normal(self, shape):
        return jax.random.normal(self._next(), shape, dtype=jnp.bfloat16)

    def randint(self, lo, hi, shape):
        return jax.random.randint(self._next(), shape, lo, hi, dtype=jnp.int32)

    def uniform(self, shape, lo=0.0, hi=1.0):
        return jax.random.uniform(self._next(), shape, jnp.bfloat16, lo, hi)

    def permutation(self, n):
        return jax.random.permutation(self._next(), n)
kernel_name = 'standalone__conformer_family_branchformer__speech'

def setup_inputs():
    _rng = _Rng(jax.random.key(int.from_bytes(__import__("os").urandom(4), "little")))
    _w = lambda a: (lambda t: t.astype(jnp.bfloat16) if jnp.issubdtype(t.dtype, jnp.floating) else t)(jnp.asarray(a))
    B, T, D, K = (2, 4000, 512, 31)
    s = float(D) ** (-0.5)
    return {'x': _w((lambda *s: _rng.normal(s) * 0.05)(B, T, D)), 'w_q': _w((lambda *s: _rng.normal(s) * 0.05)(D, D) * s), 'w_k': _w((lambda *s: _rng.normal(s) * 0.05)(D, D) * s), 'w_v': _w((lambda *s: _rng.normal(s) * 0.05)(D, D) * s), 'w_ao': _w((lambda *s: _rng.normal(s) * 0.05)(D, D) * s), 'w_up': _w((lambda *s: _rng.normal(s) * 0.05)(D, 2 * D) * s), 'dw': _w((lambda *s: _rng.normal(s) * 0.05)(K, D) * (1.0 / K)), 'w_dn': _w((lambda *s: _rng.normal(s) * 0.05)(D, D) * s), 'w_merge': _w((lambda *s: _rng.normal(s) * 0.05)(2 * D, D) * s)}

def reference(x, w_q, w_k, w_v, w_ao, w_up, dw, w_dn, w_merge):
    B, T, D = x.shape
    K = dw.shape[0]
    xa = _layernorm(x, axis=-1)
    q = jnp.einsum('btd,de->bte', xa, w_q)
    k = jnp.einsum('btd,de->bte', xa, w_k)
    v = jnp.einsum('btd,de->bte', xa, w_v)
    logits = jnp.einsum('btd,bsd->bts', q, k) * float(D) ** (-0.5)
    attn = _softmax(logits, axis=-1)
    ya = jnp.einsum('bts,bsd->btd', attn, v)
    ya = jnp.einsum('btd,de->bte', ya, w_ao)
    xc = _layernorm(x, axis=-1)
    h = _gelu(jnp.einsum('btd,de->bte', xc, w_up))
    u = h[..., :D].copy()
    g = _layernorm(h[..., D:], axis=-1)
    pad = K // 2
    gp = jnp.pad(g, ((0, 0), (pad, pad), (0, 0)))
    conv = jnp.zeros_like(g)
    for i in range(K):
        conv = conv + gp[:, i:i + T, :] * dw[i][None, None, :]
    yc = jnp.einsum('btd,de->bte', u * conv, w_dn)
    merged = jnp.concatenate([ya, yc], axis=-1)
    out = jnp.einsum('btf,fd->btd', merged, w_merge)
    return x + out
```

```python
import functools

import jax
import jax.numpy as jnp
from jax import lax
import jax.experimental.pallas as pl
import jax.experimental.pallas.tpu as pltpu

F32, BF16, U32 = jnp.float32, jnp.bfloat16, jnp.uint32

T, D, KW = 4000, 512, 31
QS = 1008
QR = 144
NB = 7
NT = 8
XROWS = 3 * QS + NT * 128
GOFF = 16
EPS = 1e-5
LOG2E = 1.4426950408889634

SL_U = 16 * NT
SL_M = SL_U + 16
SL_L = SL_M + 4
SL_OFF = SL_L + 4
SL_DUMMY = SL_OFF + 4
PR_RAW = 31
PR_LEFT = 36
PR_DUMMY = 40


def _enc_a(a11, a12, a21, a22):
  return [a11 + a22, a21 + a22, a11, a22, a11 + a12, a21 - a11, a12 - a22]


def _enc_b(b11, b12, b21, b22):
  return [b11 + b22, b11, b12 - b22, b21 - b11, b22, b11 + b12, b21 + b22]


_A_TERMS = ([(0, 0, 1), (1, 1, 1)], [(1, 0, 1), (1, 1, 1)], [(0, 0, 1)], [(1, 1, 1)],
            [(0, 0, 1), (0, 1, 1)], [(1, 0, 1), (0, 0, -1)], [(0, 1, 1), (1, 1, -1)])
_B_TERMS = ([(0, 0, 1), (1, 1, 1)], [(0, 0, 1)], [(0, 1, 1), (1, 1, -1)],
            [(1, 0, 1), (0, 0, -1)], [(1, 1, 1)], [(0, 0, 1), (0, 1, 1)],
            [(1, 0, 1), (1, 1, 1)])
_USE = ([((0, 0), 1), ((1, 1), 1)], [((1, 0), 1), ((1, 1), -1)],
        [((0, 1), 1), ((1, 1), 1)], [((0, 0), 1), ((1, 0), 1)],
        [((0, 0), -1), ((0, 1), 1)], [((1, 1), 1)], [((0, 0), 1)])


def _lin(terms):
  acc = None
  for v, s in terms:
    if acc is None:
      acc = v
    else:
      acc = acc + v if s > 0 else acc - v
  return acc


def _encode2(blk, terms, enc, store):
  for o in range(7):
    q = [[_lin([(blk[2 * r + i][2 * c + j], s) for r, c, s in terms[o]])
          for j in range(2)] for i in range(2)]
    for p, v in enumerate(enc(q[0][0], q[0][1], q[1][0], q[1][1])):
      store(7 * o + p, v)


def _decode_outer(inner):
  c = {}
  for o in range(7):
    quad = inner(o)
    for qi, v in quad.items():
      for qo, s in _USE[o]:
        key = (2 * qo[0] + qi[0], 2 * qo[1] + qi[1])
        if key not in c:
          c[key] = v
        else:
          c[key] = c[key] + v if s > 0 else c[key] - v
  return c


def _decode_inner(m):
  return {(0, 0): m[0] + m[3] - m[4] + m[6], (0, 1): m[2] + m[4],
          (1, 0): m[1] + m[3], (1, 1): m[0] - m[1] + m[2] + m[5]}


def _layernorm(v):
  mean = jnp.sum(v, axis=-1, keepdims=True) * (1.0 / D)
  d = v - mean
  var = jnp.sum(d * d, axis=-1, keepdims=True) * (1.0 / D)
  return d * lax.rsqrt(var + EPS)


def _gelu(v):
  c1 = 0.7978845608028654
  inner = v * (c1 + (c1 * 0.044715) * (v * v))
  h = 0.5 * v
  return h + h * jnp.tanh(inner)


def _dot(a, b):
  return jnp.dot(a, b, preferred_element_type=F32)


def _dot_nt(a, b):
  return lax.dot_general(a, b, (((1,), (1,)), ((), ())), preferred_element_type=F32)


def _ldb(ref, *idx):
  return pltpu.bitcast(ref.bitcast(U32)[idx], BF16)


def _run(rounds, pieces, rows, span=1.0):
  if not rounds:
    for fn, _ in pieces:
      fn()
    return
  per = rows // 8
  total = int(len(rounds) * per * span)
  j = 0
  for k, rnd in enumerate(rounds):
    res = rnd()
    while j < len(pieces) and (j * total) // len(pieces) < (k + 1) * per:
      r = ((j * total) // len(pieces) - k * per) * 8
      fn, anchor = pieces[j]
      anchor(res[r:r + 8, 0:128])
      fn()
      j += 1


def _merge(*lists):
  keyed = []
  for n, l in enumerate(lists):
    keyed += [((i + 0.5) / len(l), n, i, v) for i, v in enumerate(l)]
  return [v for _, _, _, v in sorted(keyed, key=lambda e: e[:3])]


def _kernel(x_hbm, wq_hbm, wk_hbm, wv_hbm, wao_hbm, wup_hbm, dw_hbm, wdn_hbm, wm_hbm,
            o_hbm, xb, ae, ke, ve, gb, dwb, wqk, wvom, wup, stage, w_sem, x_sem, o_sem):
  nbatch = x_hbm.shape[0]

  def x_copies(b, part):
    cps = []
    for a in range(4):
      lo, hi = (0, 256) if part == 0 else (256, min(QS, T - a * QS))
      rows = pl.ds(a * QS + lo, hi - lo)
      cps.append(pltpu.make_async_copy(
          x_hbm.at[b, rows, :], xb.at[b, rows, :], x_sem.at[b * 8 + part * 4 + a]))
    return cps

  def o_copies(b, j, par, last=False):
    cps = []
    for a in range(4):
      n = min(QR, T - (a * QS + (NB - 1) * QR)) if last else QR
      cps.append(pltpu.make_async_copy(
          stage.at[par, a, pl.ds(0, n), :],
          o_hbm.at[b, pl.ds(a * QS + j * QR, n), :], o_sem.at[par * 4 + a]))
    return cps

  def encode_b(src, dst, t, g):
    rows = slice(16 * g, 16 * g + 16)
    blk = [[src[i * 128 + 16 * g:i * 128 + 16 * g + 16, j * 128:j * 128 + 128].astype(F32)
            for j in range(4)] for i in range(4)]

    def store(p, v):
      dst[t, p, rows, :] = v.astype(BF16)
    _encode2(blk, _B_TERMS, _enc_b, store)

  def weights(wq, wk, wv, wao, wdn, wm, dw, tmp):
    srcs = (wq_hbm, wk_hbm, wv_hbm, wao_hbm, wm_hbm, wdn_hbm, wup_hbm, dw_hbm)
    dsts = (wq, wk, wv, wao, wm, wdn, wup, dw)
    cps = [pltpu.make_async_copy(s, d, w_sem.at[i])
           for i, (s, d) in enumerate(zip(srcs, dsts))]
    for cp in cps:
      cp.start()
    for cp in x_copies(0, 0) + x_copies(0, 1):
      cp.start()
    for b in range(nbatch):
      xb[b, T:XROWS, :] = jnp.zeros((XROWS - T, D), BF16)
    for c in range(4):
      gb[c, 0:GOFF, :] = jnp.zeros((GOFF, 128), F32)
    cps[0].wait()
    cps[1].wait()
    wqk[...] = (_dot_nt(wq[...], wk[...]) * (LOG2E * D ** -0.5)).astype(BF16)
    cps[2].wait()
    cps[3].wait()
    cps[4].wait()
    wvom[...] = _dot(_dot(wv[...], wao[...]).astype(BF16), wm[0:D, :]).astype(BF16)
    cps[5].wait()
    tmp[...] = _dot(wdn[...], wm[D:2 * D, :])
    cps[6].wait()
    cps[7].wait()
    for g in range(8):
      encode_b(wup, ke, NT, g)
    for g in range(8):
      encode_b(tmp, ve, NT, g)
    taps = dw[...].astype(F32)
    for c in range(4):
      for k in range(KW):
        dwb[c, k] = jnp.broadcast_to(taps[k:k + 1, c * 128:c * 128 + 128], (8, 128))

  sq = pltpu.VMEM((D, D), BF16)
  pl.run_scoped(weights, sq, sq, sq, sq, sq, pltpu.VMEM((2 * D, D), BF16),
                pltpu.VMEM((KW, D), BF16), pltpu.VMEM((D, D), F32))

  def phase1(b, z, xa0, xa1, k0, k1, v0, v1, g0, g1):
    xas, ks, vs, gs = (xa0, xa1), (k0, k1), (v0, v1), (g0, g1)

    def anchor(ref):
      def put(v):
        ref[pl.ds(pl.multiple_of(D + z, 8), 8), 0:128] = v
      return put

    def norm_piece(t, par, g):
      blk = []
      for a in range(4):
        r0 = pl.multiple_of(a * QS + 16 * g + 128 * t, 16)
        xa = _layernorm(xb[b, pl.ds(r0, 16), :].astype(F32))
        xas[par][a * 128 + 16 * g:a * 128 + 16 * g + 16, :] = xa.astype(BF16)
        blk.append([xa[:, k * 128:k * 128 + 128] for k in range(4)])
      rows = pl.ds(pl.multiple_of(128 * t + 16 * g, 16), 16)

      def store(p, v):
        ae[p, rows, :] = v.astype(BF16)
      _encode2(blk, _A_TERMS, _enc_a, store)

    def gate_piece(t, par, a, g):
      v = _layernorm(_gelu(gs[par][a * 128 + 8 * g:a * 128 + 8 * g + 8, :]))
      rows = pl.ds(pl.multiple_of(GOFF + a * QS + 8 * g + 128 * t, 8), 8)
      for c in range(4):
        gb[c, rows, :] = v[:, c * 128:c * 128 + 128]

    def step(t, par, dots, post, norm):
      rounds = []
      if dots:
        def proj(dst, n, fn):
          def rnd():
            res = fn()
            dst[0:D, n * 128:n * 128 + 128] = res
            return res
          return rnd
        xa = xas[par]
        for n in range(4):
          cols = slice(n * 128, n * 128 + 128)
          rounds.append(proj(gs[par], n, lambda cols=cols: _dot(
              xa[...], wup[:, D + cols.start:D + cols.stop])))
        for n in range(4):
          cols = slice(n * 128, n * 128 + 128)
          rounds.append(proj(ks[par], n, lambda cols=cols: _dot_nt(wqk[...], xa[cols, :])))
        for n in range(4):
          cols = slice(n * 128, n * 128 + 128)
          rounds.append(proj(vs[par], n, lambda cols=cols: _dot(xa[...], wvom[:, cols])))
      lists = []
      if post:
        q = 1 - par
        lists.append([(functools.partial(gate_piece, t - 1, q, a, g), anchor(gs[q]))
                      for a in range(4) for g in range(16)])
        lists.append([(functools.partial(encode_b, ks[q], ke, t - 1, g), anchor(ks[q]))
                      for g in range(8)])
        lists.append([(functools.partial(encode_b, vs[q], ve, t - 1, g), anchor(vs[q]))
                      for g in range(8)])
      if norm:
        def xanchor(v):
          xb[nbatch, pl.ds(pl.multiple_of(z, 16), 16), 0:128] = jnp.concatenate(
              [v, v], axis=0).astype(BF16)
        lists.append([(functools.partial(norm_piece, t + 1, 1 - par, g), xanchor)
                      for g in range(8)])
      _run(rounds, _merge(*lists), D, span=0.95)

    step(-1, 1, False, False, True)
    step(0, 0, True, False, True)
    for cp in x_copies(b, 1):
      cp.wait()

    def pair(i, carry):
      step(2 * i + 1, 1, True, True, True)
      step(2 * i + 2, 0, True, True, True)
      return carry
    lax.fori_loop(0, (NT - 2) // 2, pair, None)
    step(NT - 1, 1, True, True, False)
    step(NT, 0, False, True, False)

  def phase2(b, z, sb, pr0, pr1, pr2, pe_a, pe_b, pe_z, oacc, ofin, cv):
    prs = [(pr0, pr1)[t % 2] for t in range(NT)] + [pr2]
    left = [PR_LEFT + t // 2 for t in range(NT)] + [PR_LEFT]

    def anchor(ref, slot):
      def put(v):
        ref[slot + z, 0:8, :] = v
      return put

    def s_prod(m, t, o, p):
      lhs = _ldb(ae, 7 * o + p, pl.ds(pl.multiple_of(m * (QR // 2), 8), QR // 2), slice(None))
      return _dot(lhs, _ldb(ke, t, 7 * o + p))

    raw = [(o, p) for o in (5, 6) for p in (0, 2, 4)]

    def s_round_a(m, t, o):
      m2, m4, m6, m7 = [s_prod(m, t, o, p) for p in (1, 3, 5, 6)]
      pr = prs[t]
      pr[3 * o] = m4 + m7
      pr[3 * o + 1] = m2 + m4
      pr[3 * o + 2] = m6 - m2
      return m7

    def s_round_b(m, t, o):
      m1, m3, m5 = [s_prod(m, t, o, p) for p in (0, 2, 4)]
      extra = s_prod(m, t, *raw[o])
      pr = prs[t]
      pr[21 + 2 * o] = m1 - m5
      pr[22 + 2 * o] = m3 + m5
      pr[PR_RAW + o] = extra
      return extra

    def z_prod(p):
      res = _dot(_ldb(pe_z, p), _ldb(ve, NT, p))
      ofin[p] = oacc[p] + res
      return res

    def left_round(m, tiles, z_too):
      res = None
      for t in tiles:
        res = s_prod(m, t, *raw[5])
        prs[t][left[t]] = res
      if z_too:
        res = z_prod(48)
      return res

    def z_round(k):
      return [z_prod(p) for p in range(4 * k, 4 * k + 4)][-1]

    def pv_round(second, p):
      pe = pe_b if second else pe_a
      lhs = jnp.concatenate([_ldb(pe, i, p) for i in range(4)], axis=1)
      rhs = jnp.concatenate([_ldb(ve, 4 * second + i, p) for i in range(4)], axis=0)
      res = _dot(lhs, rhs)
      oacc[p] = oacc[p] + res if second else res
      return res

    def comb_piece(t, r):
      rows = slice(r, r + 8)
      pr = prs[t]

      def inner(o):
        q, rr, w = [pr[3 * o + i, rows, :] for i in range(3)]
        if o < 5:
          xx, yy = pr[21 + 2 * o, rows, :], pr[22 + 2 * o, rows, :]
        else:
          slots = [PR_RAW + i if i < 5 else left[t]
                   for i in range(3 * (o - 5), 3 * (o - 5) + 3)]
          m1, m3, m5 = [pr[s, rows, :] for s in slots]
          xx, yy = m1 - m5, m3 + m5
        return {(0, 0): xx + q, (0, 1): yy, (1, 0): rr, (1, 1): xx + yy + w}
      c = _decode_outer(inner)
      if t == NT:
        for (a, k), v in c.items():
          sb[SL_U + 4 * a + k, rows, :] = v
        return
      if t == NT - 1:
        lane = lax.broadcasted_iota(jnp.int32, (8, 128), 1)
      for a in range(4):
        vs = [c[(a, k)] for k in range(4)]
        if t == NT - 1:
          vs = [jnp.where(lane < min(QS, T - k * QS) - 128 * t, v, -jnp.inf)
                for k, v in enumerate(vs)]
        for k in range(4):
          sb[16 * t + 4 * a + k, rows, :] = vs[k]
        mx = jnp.maximum(jnp.maximum(vs[0], vs[1]), jnp.maximum(vs[2], vs[3]))
        if t > 0:
          m_old = sb[SL_M + a, rows, :]
          mx = jnp.maximum(mx, m_old)
        e = [jnp.exp2(v - mx) for v in vs]
        ls = (e[0] + e[1]) + (e[2] + e[3])
        if t > 0:
          ls = ls + sb[SL_L + a, rows, :] * jnp.exp2(m_old - mx)
        if t < NT - 1:
          sb[SL_M + a, rows, :] = mx
          sb[SL_L + a, rows, :] = ls
        else:
          m_row = jnp.max(mx, axis=-1, keepdims=True)
          l_row = jnp.sum(ls * jnp.exp2(mx - m_row), axis=-1, keepdims=True)
          sb[SL_OFF + a, rows, :] = jnp.broadcast_to(m_row + jnp.log2(l_row), (8, 128))

    def prep_piece(t, r):
      rows = slice(r, r + 16)
      blk = []
      for a in range(4):
        if t < NT:
          off = sb[SL_OFF + a, rows, :]
          blk.append([jnp.exp2(sb[16 * t + 4 * a + k, rows, :] - off) for k in range(4)])
        else:
          blk.append([_gelu(sb[SL_U + 4 * a + k, rows, :]) * cv[4 * a + k, rows, :]
                      for k in range(4)])

      def store(p, v):
        if t == NT:
          pe_z[p, rows, :] = v.astype(BF16)
        else:
          (pe_a if t < 4 else pe_b)[t % 4, p, rows, :] = v.astype(BF16)
      _encode2(blk, _A_TERMS, _enc_a, store)

    def conv_piece(j, a, c, r):
      base = GOFF - KW // 2 + a * QS + r + j * QR
      acc = [None, None]
      for k in range(KW):
        w = dwb[c, k]
        for h in range(2):
          v = gb[c, pl.ds(base + 8 * h + k, 8), :] * w
          acc[h] = v if acc[h] is None else acc[h] + v
      for h in range(2):
        cv[4 * a + c, r + 8 * h:r + 8 * h + 8, :] = acc[h]

    def out_piece(j, par, r):
      halves = []
      for h in range(2):
        rows = slice(r + 8 * h, r + 8 * h + 8)
        halves.append(_decode_outer(
            lambda o: _decode_inner([ofin[7 * o + p, rows, :] for p in range(7)])))
      for a in range(4):
        xr = pl.ds(pl.multiple_of(a * QS + r + j * QR, 16), 16)
        for k in range(4):
          cols = slice(k * 128, k * 128 + 128)
          y = jnp.concatenate([halves[0][(a, k)], halves[1][(a, k)]], axis=0)
          stage[par, a, r:r + 16, cols] = (xb[b, xr, cols].astype(F32) + y).astype(BF16)

    def ganchor(v):
      gb[4, pl.ds(pl.multiple_of(z, 8), 8), :] = v

    def iteration(m, do_s, do_p, do_z):
      part = functools.partial
      par = m % 2
      convs = [(part(conv_piece, m - 1, a, c, r), ganchor)
               for a in range(4) for c in range(4) for r in range(0, QR, 16)]
      outs = [(part(out_piece, m - 2, par, r), anchor(ofin, 49)) for r in range(0, QR, 16)]
      pv_split = [0, 12, 24, 36, 49]
      for j in range(NT + 1):
        s_rounds, v_rounds = [], []
        if do_s:
          if j in (0, 4):
            s_rounds.append(part(left_round, m, range(j, j + 4), False))
          for o in range(7):
            s_rounds.append(part(s_round_a, m, j, o))
            if o < 5:
              s_rounds.append(part(s_round_b, m, j, o))
        if do_z and j < 4:
          v_rounds = [part(pv_round, 1, p) for p in range(pv_split[j], pv_split[j + 1])]
        if do_z and j == 4:
          anchor(oacc, 49)(jnp.zeros((8, 128), F32))
          v_rounds = [part(z_round, k) for k in range(12)]
        if j == 4 and (do_s or do_z):
          v_rounds.append(part(left_round, m, [NT] if do_s else [], do_z))
        if do_p and j > 4:
          if j == 5:
            pe_a[4 + z, 0, 0:16, :] = jnp.zeros((16, 128), BF16)
          v_rounds = [part(pv_round, 0, p) for p in range(pv_split[j - 5], pv_split[j - 4])]
        t = j - 1 if j > 0 else NT
        main = []
        for r in range(0, QR, 8):
          if r % 16 == 0 and (do_p if j > 0 else do_z):
            main.append((part(prep_piece, t, r), anchor(sb, SL_DUMMY)))
          if do_s if j > 0 else do_p:
            main.append((part(comb_piece, t, r), anchor(prs[t], PR_DUMMY)))
        lists = [main]
        if do_p and j > 0:
          n = len(convs) // NT
          lists.append(convs[(j - 1) * n:j * n])
        if do_z and j > 4:
          lists.append(outs[(9 * (j - 5)) // 4:(9 * (j - 4)) // 4])
        _run(_merge(s_rounds, v_rounds), _merge(*lists), QR, span=0.95)

    iteration(0, True, False, False)

    @pl.when(b > 0)
    def _():
      for cp in o_copies(b - 1, NB - 2, 1) + o_copies(b - 1, NB - 1, 0, last=True):
        cp.wait()
    iteration(1, True, True, False)

    def steady(m, carry):
      @pl.when(m >= 4)
      def _():
        for cp in o_copies(b, m - 4, m % 2):
          cp.wait()
      iteration(m, True, True, True)
      for cp in o_copies(b, m - 2, m % 2):
        cp.start()
      return carry
    lax.fori_loop(2, NB, steady, None)
    for cp in o_copies(b, NB - 4, NB % 2):
      cp.wait()
    iteration(NB, False, True, True)
    for cp in o_copies(b, NB - 2, NB % 2):
      cp.start()
    for cp in o_copies(b, NB - 3, (NB + 1) % 2):
      cp.wait()
    iteration(NB + 1, False, False, True)
    for cp in o_copies(b, NB - 1, (NB + 1) % 2, last=True):
      cp.start()

  def batch(b, carry):
    z = lax.shift_right_logical(b, 8)
    for cp in x_copies(b, 0):
      cp.wait()
    st = pltpu.VMEM((D + 8, D), F32)
    pl.run_scoped(functools.partial(phase1, b, z), sq, sq, st, st, st, st, st, st)

    @pl.when(b + 1 < nbatch)
    def _():
      for cp in x_copies(b + 1, 0) + x_copies(b + 1, 1):
        cp.start()
    blocks = lambda n: pltpu.VMEM((n, QR, 128), F32)
    pl.run_scoped(
        functools.partial(phase2, b, z),
        blocks(SL_DUMMY + 1), blocks(PR_DUMMY + 1), blocks(PR_DUMMY + 1), blocks(PR_DUMMY + 1),
        pltpu.VMEM((5, 49, QR, 128), BF16), pltpu.VMEM((4, 49, QR, 128), BF16),
        pltpu.VMEM((49, QR, 128), BF16), blocks(50), blocks(50), blocks(16))
    return carry

  lax.fori_loop(0, nbatch, batch, None)
  for cp in o_copies(nbatch - 1, NB - 2, 1) + o_copies(nbatch - 1, NB - 1, 0, last=True):
    cp.wait()


@jax.jit
def pallas_standalone__conformer_family_branchformer__speech_kernel(
    x: jax.Array,
    w_q: jax.Array,
    w_k: jax.Array,
    w_v: jax.Array,
    w_ao: jax.Array,
    w_up: jax.Array,
    dw: jax.Array,
    w_dn: jax.Array,
    w_merge: jax.Array,
):
  nbatch = x.shape[0]
  assert x.shape[1:] == (T, D) and dw.shape == (KW, D)
  any_spec = pl.BlockSpec(memory_space=pl.ANY)
  return pl.pallas_call(
      _kernel,
      out_shape=jax.ShapeDtypeStruct(x.shape, x.dtype),
      in_specs=[any_spec] * 9,
      out_specs=any_spec,
      scratch_shapes=[
          pltpu.VMEM((nbatch + 1, XROWS, D), BF16),
          pltpu.VMEM((49, NT * 128, 128), BF16),
          pltpu.VMEM((NT + 1, 49, 128, 128), BF16),
          pltpu.VMEM((NT + 1, 49, 128, 128), BF16),
          pltpu.VMEM((5, GOFF + XROWS, 128), F32),
          pltpu.VMEM((4, KW, 8, 128), F32),
          pltpu.VMEM((D, D), BF16),
          pltpu.VMEM((D, D), BF16),
          pltpu.VMEM((D, 2 * D), BF16),
          pltpu.VMEM((2, 4, QR, D), BF16),
          pltpu.SemaphoreType.DMA((8,)),
          pltpu.SemaphoreType.DMA((8 * nbatch,)),
          pltpu.SemaphoreType.DMA((8,)),
      ],
      compiler_params=pltpu.CompilerParams(vmem_limit_bytes=126 * 1024 * 1024),
      name="branchformer",
  )(x, w_q, w_k, w_v, w_ao, w_up, dw, w_dn, w_merge)
```

```python
import functools

import jax
import jax.numpy as jnp
from jax import lax
import jax.experimental.pallas as pl
import jax.experimental.pallas.tpu as pltpu

F32, BF16, U32 = jnp.float32, jnp.bfloat16, jnp.uint32

T, D, KW = 4000, 512, 31
QS = 1008
QR = 144
NB = 7
NT = 8
XROWS = 3 * QS + NT * 128
GOFF = 16
EPS = 1e-5
LOG2E = 1.4426950408889634

_DEV = None
CONV_TAPS = 16
SPAN = 0.95

SL_U = 16 * NT
SL_M = SL_U + 16
SL_L = SL_M + 4
SL_OFF = SL_L + 4
SL_DUMMY = SL_OFF + 4
PR_RAW = 31
PR_LEFT = 36
PR_DUMMY = 40


def _enc_a(a11, a12, a21, a22):
  return [a11 + a22, a21 + a22, a11, a22, a11 + a12, a21 - a11, a12 - a22]


def _enc_b(b11, b12, b21, b22):
  return [b11 + b22, b11, b12 - b22, b21 - b11, b22, b11 + b12, b21 + b22]


_A_TERMS = ([(0, 0, 1), (1, 1, 1)], [(1, 0, 1), (1, 1, 1)], [(0, 0, 1)], [(1, 1, 1)],
            [(0, 0, 1), (0, 1, 1)], [(1, 0, 1), (0, 0, -1)], [(0, 1, 1), (1, 1, -1)])
_B_TERMS = ([(0, 0, 1), (1, 1, 1)], [(0, 0, 1)], [(0, 1, 1), (1, 1, -1)],
            [(1, 0, 1), (0, 0, -1)], [(1, 1, 1)], [(0, 0, 1), (0, 1, 1)],
            [(1, 0, 1), (1, 1, 1)])
_USE = ([((0, 0), 1), ((1, 1), 1)], [((1, 0), 1), ((1, 1), -1)],
        [((0, 1), 1), ((1, 1), 1)], [((0, 0), 1), ((1, 0), 1)],
        [((0, 0), -1), ((0, 1), 1)], [((1, 1), 1)], [((0, 0), 1)])


def _lin(terms):
  acc = None
  for v, s in terms:
    if acc is None:
      acc = v
    else:
      acc = acc + v if s > 0 else acc - v
  return acc


def _encode2(blk, terms, enc, store, outer=range(7)):
  for o in outer:
    q = [[_lin([(blk[2 * r + i][2 * c + j], s) for r, c, s in terms[o]])
          for j in range(2)] for i in range(2)]
    for p, v in enumerate(enc(q[0][0], q[0][1], q[1][0], q[1][1])):
      store(7 * o + p, v)
  return v


_A_STEPS = (([(0, 0), (1, 1)], (2, 0, 3)), ([(1, 0)], (1, 5)), ([(0, 1)], (4, 6)))
_B_STEPS = (([(0, 0), (1, 1)], (1, 0, 4)), ([(0, 1)], (2, 5)), ([(1, 0)], (3, 6)))


def _encode_steps(fetch, steps, terms, enc, store):
  blk = [[None] * 4 for _ in range(4)]

  def step(quads, outer):
    for r, c in quads:
      for i in range(2):
        for j in range(2):
          blk[2 * r + i][2 * c + j] = fetch(2 * r + i, 2 * c + j)
    return _encode2(blk, terms, enc, store, outer)
  return [functools.partial(step, *st) for st in steps]


def _decode_outer(inner):
  c = {}
  for o in range(7):
    quad = inner(o)
    for qi, v in quad.items():
      for qo, s in _USE[o]:
        key = (2 * qo[0] + qi[0], 2 * qo[1] + qi[1])
        if key not in c:
          c[key] = v
        else:
          c[key] = c[key] + v if s > 0 else c[key] - v
  return c


def _decode_inner(m):
  return {(0, 0): m[0] + m[3] - m[4] + m[6], (0, 1): m[2] + m[4],
          (1, 0): m[1] + m[3], (1, 1): m[0] - m[1] + m[2] + m[5]}


def _layernorm(v):
  mean = jnp.sum(v, axis=-1, keepdims=True) * (1.0 / D)
  d = v - mean
  var = jnp.sum(d * d, axis=-1, keepdims=True) * (1.0 / D)
  return d * lax.rsqrt(var + EPS)


def _gelu(v):
  c1 = 0.7978845608028654
  inner = v * (c1 + (c1 * 0.044715) * (v * v))
  h = 0.5 * v
  return h + h * jnp.tanh(inner)


def _dot(a, b):
  return jnp.dot(a, b, preferred_element_type=F32)


def _dot_nt(a, b):
  return lax.dot_general(a, b, (((1,), (1,)), ((), ())), preferred_element_type=F32)


def _ldb(ref, *idx):
  return pltpu.bitcast(ref.bitcast(U32)[idx], BF16)


def _run(rounds, pieces, rows, span=1.0):
  if not rounds:
    for fn, _, _, _ in pieces:
      fn()
    return
  per = rows // 8
  total = len(rounds) * per * span / max(1, sum(p[2] for p in pieces))
  j, done, last = 0, 0, {}
  for k, rnd in enumerate(rounds):
    res = rnd()
    while j < len(pieces) and int(done * total) < (k + 1) * per:
      r = (int(done * total) - k * per) * 8
      fn, anchor, cost, chain = pieces[j]
      pin = res[r:r + 8, 0:128]
      anchor(pin + last[chain] if chain in last else pin)
      tok = fn()
      if chain is not None:
        last[chain] = tok[0:8, 0:128]
      j += 1
      done += cost


def _merge(*lists, cost=lambda v: 1):
  keyed = []
  for n, l in enumerate(lists):
    total, done = sum(cost(v) for v in l), 0
    for i, v in enumerate(l):
      keyed.append(((done + 0.5 * cost(v)) / total, n, i, v))
      done += cost(v)
  return [v for _, _, _, v in sorted(keyed, key=lambda e: e[:3])]


def _merge_groups(*lists):
  merged = _merge(*lists, cost=lambda g: sum(p[2] for p in g))
  return [p for g in merged for p in g]


def _kernel(x_hbm, wq_hbm, wk_hbm, wv_hbm, wao_hbm, wup_hbm, dw_hbm, wdn_hbm, wm_hbm,
            o_hbm, xb, ae, ke, ve, gb, dwb, wqk, wvom, wup, stage, w_sem, x_sem, o_sem):
  nbatch = x_hbm.shape[0]

  def x_copies(b, part):
    cps = []
    for a in range(4):
      lo, hi = (0, 256) if part == 0 else (256, min(QS, T - a * QS))
      rows = pl.ds(a * QS + lo, hi - lo)
      cps.append(pltpu.make_async_copy(
          x_hbm.at[b, rows, :], xb.at[b, rows, :], x_sem.at[b * 8 + part * 4 + a]))
    return cps

  def o_copies(b, j, par, last=False):
    cps = []
    for a in range(4):
      n = min(QR, T - (a * QS + (NB - 1) * QR)) if last else QR
      cps.append(pltpu.make_async_copy(
          stage.at[par, a, pl.ds(0, n), :],
          o_hbm.at[b, pl.ds(a * QS + j * QR, n), :], o_sem.at[par * 4 + a]))
    return cps

  def block_fetch(src, g):
    def fetch(i, j):
      return src[i * 128 + 16 * g:i * 128 + 16 * g + 16, j * 128:j * 128 + 128].astype(F32)
    return fetch

  def encode_b(src, dst, t, g):
    def store(p, v):
      dst[t, p, 16 * g:16 * g + 16, :] = v.astype(BF16)
    return _encode_steps(block_fetch(src, g), _B_STEPS, _B_TERMS, _enc_b, store)

  def weights(wq, wk, wv, wao, wdn, wm, dw, tmp):
    srcs = (wq_hbm, wk_hbm, wv_hbm, wao_hbm, wm_hbm, wdn_hbm, wup_hbm, dw_hbm)
    dsts = (wq, wk, wv, wao, wm, wdn, wup, dw)
    cps = [pltpu.make_async_copy(s, d, w_sem.at[i])
           for i, (s, d) in enumerate(zip(srcs, dsts))]
    for cp in cps:
      cp.start()
    for cp in x_copies(0, 0) + x_copies(0, 1):
      cp.start()
    for b in range(nbatch):
      xb[b, T:XROWS, :] = jnp.zeros((XROWS - T, D), BF16)
    for c in range(4):
      gb[c, 0:GOFF, :] = jnp.zeros((GOFF, 128), F32)
    cps[0].wait()
    cps[1].wait()
    wqk[...] = (_dot_nt(wq[...], wk[...]) * (LOG2E * D ** -0.5)).astype(BF16)
    cps[2].wait()
    cps[3].wait()
    cps[4].wait()
    wvom[...] = _dot(_dot(wv[...], wao[...]).astype(BF16), wm[0:D, :]).astype(BF16)
    cps[5].wait()
    tmp[...] = _dot(wdn[...], wm[D:2 * D, :])
    cps[6].wait()
    cps[7].wait()
    for src, dst in ((wup, ke), (tmp, ve)):
      for g in range(8):
        for fn in encode_b(src, dst, NT, g):
          fn()
    taps = dw[...].astype(F32)
    for c in range(4):
      for k in range(KW):
        dwb[c, k] = jnp.broadcast_to(taps[k:k + 1, c * 128:c * 128 + 128], (8, 128))

  sq = pltpu.VMEM((D, D), BF16)
  if _DEV is None: pl.run_scoped(weights, sq, sq, sq, sq, sq, pltpu.VMEM((2 * D, D), BF16),
                pltpu.VMEM((KW, D), BF16), pltpu.VMEM((D, D), F32))

  def phase1(b, z, xa0, xa1, xf, k0, k1, v0, v1, g0, g1):
    xas, ks, vs, gs = (xa0, xa1), (k0, k1), (v0, v1), (g0, g1)

    def anchor(ref):
      def put(v):
        ref[pl.ds(pl.multiple_of(D + z, 8), 8), 0:128] = v
      return put

    def norm_piece(t, par, a, g):
      r0 = pl.multiple_of(a * QS + 16 * g + 128 * t, 16)
      xa = _layernorm(xb[b, pl.ds(r0, 16), :].astype(F32))
      rows = slice(a * 128 + 16 * g, a * 128 + 16 * g + 16)
      xas[par][rows, :] = xa.astype(BF16)
      xf[rows, :] = xa

    def encode_a(t, g):
      rows = pl.ds(pl.multiple_of(128 * t + 16 * g, 16), 16)

      def store(p, v):
        ae[p, rows, :] = v.astype(BF16)
      return _encode_steps(block_fetch(xf, g), _A_STEPS, _A_TERMS, _enc_a, store)

    def gate_piece(t, par, a, g):
      v = _layernorm(_gelu(gs[par][a * 128 + 8 * g:a * 128 + 8 * g + 8, :]))
      rows = pl.ds(pl.multiple_of(GOFF + a * QS + 8 * g + 128 * t, 8), 8)
      for c in range(4):
        gb[c, rows, :] = v[:, c * 128:c * 128 + 128]
      return v

    def step(t, par, dots, post, norm):
      rounds = []
      if dots:
        def proj(dst, n, fn):
          def rnd():
            res = fn()
            dst[0:D, n * 128:n * 128 + 128] = res
            return res
          return rnd
        xa = xas[par]
        for n in range(4):
          cols = slice(n * 128, n * 128 + 128)
          rounds.append(proj(gs[par], n, lambda cols=cols: _dot(
              xa[...], wup[:, D + cols.start:D + cols.stop])))
        for n in range(4):
          cols = slice(n * 128, n * 128 + 128)
          rounds.append(proj(ks[par], n, lambda cols=cols: _dot_nt(wqk[...], xa[cols, :])))
        for n in range(4):
          cols = slice(n * 128, n * 128 + 128)
          rounds.append(proj(vs[par], n, lambda cols=cols: _dot(xa[...], wvom[:, cols])))
      lists = []
      if post:
        q = 1 - par
        lists.append([[(functools.partial(gate_piece, t - 1, q, a, g), anchor(gs[q]), 30, None)]
                      for a in range(4) for g in range(16)])
        for src, dst in ((ks[q], ke), (vs[q], ve)):
          lists.append([[(fn, anchor(src), c, 1) for fn, c in
                         zip(encode_b(src, dst, t - 1, g), (35, 25, 25))] for g in range(8)])
      if norm:
        def xanchor(v):
          xb[nbatch, pl.ds(pl.multiple_of(z, 16), 16), 0:128] = jnp.concatenate(
              [v, v], axis=0).astype(BF16)
        norms = [[(functools.partial(norm_piece, t + 1, 1 - par, a, g), xanchor, 30, None)]
                 for g in range(8) for a in range(4)]
        encs = [[(fn, anchor(xf), c, 1) for fn, c in zip(encode_a(t + 1, g), (35, 25, 25))]
                for g in range(8)]
        lists.append(norms + encs)
      _run(rounds, _merge_groups(*lists), D, span=0.95)

    step(-1, 1, False, False, True)
    step(0, 0, True, False, True)
    for cp in x_copies(b, 1):
      cp.wait()

    def pair(i, carry):
      step(2 * i + 1, 1, True, True, True)
      step(2 * i + 2, 0, True, True, True)
      return carry
    lax.fori_loop(0, (NT - 2) // 2, pair, None)
    step(NT - 1, 1, True, True, False)
    step(NT, 0, False, True, False)

  def phase2(b, z, sb, pr0, pr1, pr2, pe_a, pe_b, pe_z, oacc, ofin, cv):
    prs = [(pr0, pr1)[t % 2] for t in range(NT)] + [pr2]
    left = [PR_LEFT + t // 2 for t in range(NT)] + [PR_LEFT]

    def anchor(ref, slot):
      def put(v):
        ref[slot + z, 0:8, :] = v
      return put

    def s_prod(m, t, o, p):
      lhs = _ldb(ae, 7 * o + p, pl.ds(pl.multiple_of(m * (QR // 2), 8), QR // 2), slice(None))
      return _dot(lhs, _ldb(ke, t, 7 * o + p))

    raw = [(o, p) for o in (5, 6) for p in (0, 2, 4)]

    def s_round_a(m, t, o):
      m2, m4, m6, m7 = [s_prod(m, t, o, p) for p in (1, 3, 5, 6)]
      pr = prs[t]
      pr[3 * o] = m4 + m7
      pr[3 * o + 1] = m2 + m4
      pr[3 * o + 2] = m6 - m2
      return m7

    def s_round_b(m, t, o):
      m1, m3, m5 = [s_prod(m, t, o, p) for p in (0, 2, 4)]
      extra = s_prod(m, t, *raw[o])
      pr = prs[t]
      pr[21 + 2 * o] = m1 - m5
      pr[22 + 2 * o] = m3 + m5
      pr[PR_RAW + o] = extra
      return extra

    def z_prod(p):
      res = _dot(_ldb(pe_z, p), _ldb(ve, NT, p))
      ofin[p] = oacc[p] + res
      return res

    def left_round(m, tiles, z_too):
      res = None
      for t in tiles:
        res = s_prod(m, t, *raw[5])
        prs[t][left[t]] = res
      if z_too:
        res = z_prod(48)
      return res

    def z_round(k):
      return [z_prod(p) for p in range(4 * k, 4 * k + 4)][-1]

    def pv_round(second, p):
      pe = pe_b if second else pe_a
      lhs = jnp.concatenate([_ldb(pe, i, p) for i in range(4)], axis=1)
      rhs = jnp.concatenate([_ldb(ve, 4 * second + i, p) for i in range(4)], axis=0)
      res = _dot(lhs, rhs)
      oacc[p] = oacc[p] + res if second else res
      return res

    def comb_piece(t, r, i):
      rows = slice(r, r + 8)
      pr = prs[t]

      def inner(o):
        if o < 5:
          xx, yy = pr[21 + 2 * o, rows, :], pr[22 + 2 * o, rows, :]
        else:
          slots = [PR_RAW + n if n < 5 else left[t]
                   for n in range(3 * (o - 5), 3 * (o - 5) + 3)]
          m1, m3, m5 = [pr[n, rows, :] for n in slots]
          xx, yy = m1 - m5, m3 + m5
        if i == 0:
          return {(0, 0): xx + pr[3 * o, rows, :], (0, 1): yy}
        return {(1, 0): pr[3 * o + 1, rows, :], (1, 1): xx + yy + pr[3 * o + 2, rows, :]}
      c = _decode_outer(inner)
      if t == NT:
        for (a, k), v in c.items():
          sb[SL_U + 4 * a + k, rows, :] = _gelu(v)
        return c[(i, 0)]
      if t == NT - 1:
        lane = lax.broadcasted_iota(jnp.int32, (8, 128), 1)
      for a in (i, i + 2):
        vs = [c[(a, k)] for k in range(4)]
        if t == NT - 1:
          vs = [jnp.where(lane < min(QS, T - k * QS) - 128 * t, v, -jnp.inf)
                for k, v in enumerate(vs)]
        for k in range(4):
          sb[16 * t + 4 * a + k, rows, :] = vs[k]
        mx = jnp.maximum(jnp.maximum(vs[0], vs[1]), jnp.maximum(vs[2], vs[3]))
        if t > 0:
          m_old = sb[SL_M + a, rows, :]
          mx = jnp.maximum(mx, m_old)
        e = [jnp.exp2(v - mx) for v in vs]
        ls = (e[0] + e[1]) + (e[2] + e[3])
        if t > 0:
          ls = ls + sb[SL_L + a, rows, :] * jnp.exp2(m_old - mx)
        sb[SL_M + a, rows, :] = mx
        sb[SL_L + a, rows, :] = ls
      return mx

    def norm_const_piece(r):
      rows = slice(r, r + 24)
      for a in range(4):
        mx = sb[SL_M + a, rows, :]
        m_row = jnp.max(mx, axis=-1, keepdims=True)
        l_row = jnp.sum(sb[SL_L + a, rows, :] * jnp.exp2(mx - m_row), axis=-1, keepdims=True)
        off = jnp.broadcast_to(m_row + jnp.log2(l_row), (24, 128))
        sb[SL_OFF + a, rows, :] = off
      return off

    def prep_steps(t, r):
      rows = slice(r, r + 16)

      def fetch(a, k):
        if t < NT:
          return jnp.exp2(sb[16 * t + 4 * a + k, rows, :] - sb[SL_OFF + a, rows, :])
        return sb[SL_U + 4 * a + k, rows, :] * cv[4 * a + k, rows, :]

      def store(p, v):
        if t == NT:
          pe_z[p, rows, :] = v.astype(BF16)
        else:
          (pe_a if t < 4 else pe_b)[t % 4, p, rows, :] = v.astype(BF16)
      return _encode_steps(fetch, _A_STEPS, _A_TERMS, _enc_a, store)

    def conv_steps(j, a, c, r):
      base = GOFF - KW // 2 + a * QS + r + j * QR
      acc = [None, None]

      def step(k0, k1):
        for k in range(k0, k1):
          w = dwb[c, k]
          for h in range(2):
            v = gb[c, pl.ds(base + 8 * h + k, 8), :] * w
            acc[h] = v if acc[h] is None else acc[h] + v
        if k1 == KW:
          for h in range(2):
            cv[4 * a + c, r + 8 * h:r + 8 * h + 8, :] = acc[h]
        return acc[1]
      return [functools.partial(step, k0, min(KW, k0 + CONV_TAPS))
              for k0 in range(0, KW, CONV_TAPS)]

    def out_piece(j, par, r):
      halves = []
      for h in range(2):
        rows = slice(r + 8 * h, r + 8 * h + 8)
        halves.append(_decode_outer(
            lambda o: _decode_inner([ofin[7 * o + p, rows, :] for p in range(7)])))
      for a in range(4):
        xr = pl.ds(pl.multiple_of(a * QS + r + j * QR, 16), 16)
        for k in range(4):
          cols = slice(k * 128, k * 128 + 128)
          y = jnp.concatenate([halves[0][(a, k)], halves[1][(a, k)]], axis=0)
          y = xb[b, xr, cols].astype(F32) + y
          stage[par, a, r:r + 16, cols] = y.astype(BF16)
      return y

    def ganchor(v):
      gb[4, pl.ds(pl.multiple_of(z, 8), 8), :] = v

    def zanchor(v):
      anchor(sb, SL_DUMMY)(v)
      anchor(cv, 16)(v)

    def iteration(m, do_s, do_p, do_z):
      part = functools.partial
      par = m % 2
      convs = [[(fn, ganchor, CONV_TAPS * 1.4, 0) for fn in conv_steps(m - 1, a, c, r)]
               for a in range(4) for c in range(4) for r in range(0, QR, 16)]
      outs = [[(part(out_piece, m - 2, par, r), anchor(ofin, 49), 90, 1)]
              for r in range(0, QR, 16)]
      pv_split = [0, 12, 24, 36, 49]
      for j in range(NT + 1):
        s_rounds, v_rounds = [], []
        if do_s:
          if j in (0, 4):
            s_rounds.append(part(left_round, m, range(j, j + 4), False))
          for o in range(7):
            s_rounds.append(part(s_round_a, m, j, o))
            if o < 5:
              s_rounds.append(part(s_round_b, m, j, o))
        if do_z and j < 4:
          v_rounds = [part(pv_round, 1, p) for p in range(pv_split[j], pv_split[j + 1])]
        if do_z and j == 4:
          anchor(oacc, 49)(jnp.zeros((8, 128), F32))
          v_rounds = [part(z_round, k) for k in range(12)]
        if j == 4 and (do_s or do_z):
          v_rounds.append(part(left_round, m, [NT] if do_s else [], do_z))
        if do_p and j > 4:
          if j == 5:
            pe_a[4 + z, 0, 0:16, :] = jnp.zeros((16, 128), BF16)
          v_rounds = [part(pv_round, 0, p) for p in range(pv_split[j - 5], pv_split[j - 4])]
        t = j - 1 if j > 0 else NT
        main = []
        for r in range(0, QR, 8):
          if r % 16 == 0 and (do_p if j > 0 else do_z):
            pin = anchor(sb, SL_DUMMY) if j > 0 else zanchor
            main.append([(fn, pin, c, 1) for fn, c in zip(prep_steps(t, r), (50, 32, 32))])
          if do_s if j > 0 else do_p:
            main += [[(part(comb_piece, t, r, i), anchor(prs[t], PR_DUMMY), 30 if j > 0 else 36, 1)]
                     for i in range(2)]
        lists = [main]
        if do_p and j > 0:
          n = len(convs) // NT
          lists.append(convs[(j - 1) * n:j * n])
        if do_p and j == 0:
          lists.append([[(part(norm_const_piece, r), anchor(sb, SL_DUMMY), 40, 0)]
                        for r in range(0, QR, 24)])
        if do_z and j > 4:
          lists.append(outs[(9 * (j - 5)) // 4:(9 * (j - 4)) // 4])
        _run(_merge(s_rounds, v_rounds), _merge_groups(*lists), QR, span=SPAN)

    if _DEV is not None:
      lax.fori_loop(2, NB, lambda m, c: iteration(m, *_DEV), None)
      return
    iteration(0, True, False, False)

    @pl.when(b > 0)
    def _():
      for cp in o_copies(b - 1, NB - 2, 1) + o_copies(b - 1, NB - 1, 0, last=True):
        cp.wait()
    iteration(1, True, True, False)

    def steady(m, carry):
      @pl.when(m >= 4)
      def _():
        for cp in o_copies(b, m - 4, m % 2):
          cp.wait()
      iteration(m, True, True, True)
      for cp in o_copies(b, m - 2, m % 2):
        cp.start()
      return carry
    lax.fori_loop(2, NB, steady, None)
    for cp in o_copies(b, NB - 4, NB % 2):
      cp.wait()
    iteration(NB, False, True, True)
    for cp in o_copies(b, NB - 2, NB % 2):
      cp.start()
    for cp in o_copies(b, NB - 3, (NB + 1) % 2):
      cp.wait()
    iteration(NB + 1, False, False, True)
    for cp in o_copies(b, NB - 1, (NB + 1) % 2, last=True):
      cp.start()

  def batch(b, carry):
    z = lax.shift_right_logical(b, 8)
    for cp in x_copies(b, 0):
      cp.wait()
    st = pltpu.VMEM((D + 8, D), F32)
    if _DEV is None or _DEV == 'p1': pl.run_scoped(functools.partial(phase1, b, z), sq, sq, st, st, st, st, st, st, st)

    @pl.when(b + 1 < nbatch)
    def _():
      for cp in x_copies(b + 1, 0) + x_copies(b + 1, 1):
        cp.start()
    blocks = lambda n: pltpu.VMEM((n, QR, 128), F32)
    if _DEV == 'p1':
      @pl.when(z > 0)
      def _():
        stage[0, 0, :, 0:128] = ae[z, 0:QR, :] + ke[z, z, 0:16, :].sum() + ve[z, z, 0:16, :].sum()
    if _DEV != 'p1': pl.run_scoped(
        functools.partial(phase2, b, z),
        blocks(SL_DUMMY + 1), blocks(PR_DUMMY + 1), blocks(PR_DUMMY + 1), blocks(PR_DUMMY + 1),
        pltpu.VMEM((5, 49, QR, 128), BF16), pltpu.VMEM((4, 49, QR, 128), BF16),
        pltpu.VMEM((49, QR, 128), BF16), blocks(50), blocks(50), blocks(17))
    return carry

  lax.fori_loop(0, nbatch, batch, None)
  for cp in o_copies(nbatch - 1, NB - 2, 1) + o_copies(nbatch - 1, NB - 1, 0, last=True):
    cp.wait()


@jax.jit
def pallas_standalone__conformer_family_branchformer__speech_kernel(
    x: jax.Array,
    w_q: jax.Array,
    w_k: jax.Array,
    w_v: jax.Array,
    w_ao: jax.Array,
    w_up: jax.Array,
    dw: jax.Array,
    w_dn: jax.Array,
    w_merge: jax.Array,
):
  nbatch = x.shape[0]
  assert x.shape[1:] == (T, D) and dw.shape == (KW, D)
  any_spec = pl.BlockSpec(memory_space=pl.ANY)
  return pl.pallas_call(
      _kernel,
      out_shape=jax.ShapeDtypeStruct(x.shape, x.dtype),
      in_specs=[any_spec] * 9,
      out_specs=any_spec,
      scratch_shapes=[
          pltpu.VMEM((nbatch + 1, XROWS, D), BF16),
          pltpu.VMEM((49, NT * 128, 128), BF16),
          pltpu.VMEM((NT + 1, 49, 128, 128), BF16),
          pltpu.VMEM((NT + 1, 49, 128, 128), BF16),
          pltpu.VMEM((5, GOFF + XROWS, 128), F32),
          pltpu.VMEM((4, KW, 8, 128), F32),
          pltpu.VMEM((D, D), BF16),
          pltpu.VMEM((D, D), BF16),
          pltpu.VMEM((D, 2 * D), BF16),
          pltpu.VMEM((2, 4, QR, D), BF16),
          pltpu.SemaphoreType.DMA((8,)),
          pltpu.SemaphoreType.DMA((8 * nbatch,)),
          pltpu.SemaphoreType.DMA((8,)),
      ],
      compiler_params=pltpu.CompilerParams(vmem_limit_bytes=126 * 1024 * 1024),
      name="branchformer",
  )(x, w_q, w_k, w_v, w_ao, w_up, dw, w_dn, w_merge)
```

```python
import functools

import jax
import jax.numpy as jnp
from jax import lax
import jax.experimental.pallas as pl
import jax.experimental.pallas.tpu as pltpu

F32, BF16, U32 = jnp.float32, jnp.bfloat16, jnp.uint32

T, D, KW = 4000, 512, 31
QS = 1008
QR = 144
NB = 7
NT = 8
XROWS = 3 * QS + NT * 128
GOFF = 16
EPS = 1e-5
LOG2E = 1.4426950408889634

_DEV = None
_NOCONV = False
CONV_N, CONV_SH = 3, 2
SPAN = 0.95

SL_U = 16 * NT
SL_M = SL_U + 16
SL_L = SL_M + 4
SL_OFF = SL_L + 4
SL_DUMMY = SL_OFF + 4
PR_RAW = 31
PR_LEFT = 36
PR_DUMMY = 40


def _enc_a(a11, a12, a21, a22):
  return [a11 + a22, a21 + a22, a11, a22, a11 + a12, a21 - a11, a12 - a22]


def _enc_b(b11, b12, b21, b22):
  return [b11 + b22, b11, b12 - b22, b21 - b11, b22, b11 + b12, b21 + b22]


_A_TERMS = ([(0, 0, 1), (1, 1, 1)], [(1, 0, 1), (1, 1, 1)], [(0, 0, 1)], [(1, 1, 1)],
            [(0, 0, 1), (0, 1, 1)], [(1, 0, 1), (0, 0, -1)], [(0, 1, 1), (1, 1, -1)])
_B_TERMS = ([(0, 0, 1), (1, 1, 1)], [(0, 0, 1)], [(0, 1, 1), (1, 1, -1)],
            [(1, 0, 1), (0, 0, -1)], [(1, 1, 1)], [(0, 0, 1), (0, 1, 1)],
            [(1, 0, 1), (1, 1, 1)])
_USE = ([((0, 0), 1), ((1, 1), 1)], [((1, 0), 1), ((1, 1), -1)],
        [((0, 1), 1), ((1, 1), 1)], [((0, 0), 1), ((1, 0), 1)],
        [((0, 0), -1), ((0, 1), 1)], [((1, 1), 1)], [((0, 0), 1)])


def _lin(terms):
  acc = None
  for v, s in terms:
    if acc is None:
      acc = v
    else:
      acc = acc + v if s > 0 else acc - v
  return acc


def _encode2(blk, terms, enc, store, outer=range(7)):
  for o in outer:
    q = [[_lin([(blk[2 * r + i][2 * c + j], s) for r, c, s in terms[o]])
          for j in range(2)] for i in range(2)]
    for p, v in enumerate(enc(q[0][0], q[0][1], q[1][0], q[1][1])):
      store(7 * o + p, v)
  return v


_A_STEPS = (([(0, 0), (1, 1)], (2, 0, 3)), ([(1, 0)], (1, 5)), ([(0, 1)], (4, 6)))
_B_STEPS = (([(0, 0), (1, 1)], (1, 0, 4)), ([(0, 1)], (2, 5)), ([(1, 0)], (3, 6)))


def _encode_steps(fetch, steps, terms, enc, store):
  blk = [[None] * 4 for _ in range(4)]

  def step(quads, outer):
    for r, c in quads:
      for i in range(2):
        for j in range(2):
          blk[2 * r + i][2 * c + j] = fetch(2 * r + i, 2 * c + j)
    return _encode2(blk, terms, enc, store, outer)
  return [functools.partial(step, *st) for st in steps]


def _decode_outer(inner):
  c = {}
  for o in range(7):
    quad = inner(o)
    for qi, v in quad.items():
      for qo, s in _USE[o]:
        key = (2 * qo[0] + qi[0], 2 * qo[1] + qi[1])
        if key not in c:
          c[key] = v
        else:
          c[key] = c[key] + v if s > 0 else c[key] - v
  return c


def _decode_inner(m):
  return {(0, 0): m[0] + m[3] - m[4] + m[6], (0, 1): m[2] + m[4],
          (1, 0): m[1] + m[3], (1, 1): m[0] - m[1] + m[2] + m[5]}


def _layernorm(v):
  mean = jnp.sum(v, axis=-1, keepdims=True) * (1.0 / D)
  d = v - mean
  var = jnp.sum(d * d, axis=-1, keepdims=True) * (1.0 / D)
  return d * lax.rsqrt(var + EPS)


def _gelu(v):
  c1 = 0.7978845608028654
  inner = v * (c1 + (c1 * 0.044715) * (v * v))
  h = 0.5 * v
  return h + h * jnp.tanh(inner)


def _dot(a, b):
  return jnp.dot(a, b, preferred_element_type=F32)


def _dot_nt(a, b):
  return lax.dot_general(a, b, (((1,), (1,)), ((), ())), preferred_element_type=F32)


def _ldb(ref, *idx):
  return pltpu.bitcast(ref.bitcast(U32)[idx], BF16)


def _run(rounds, pieces, rows, span=1.0):
  if not rounds:
    for fn, _, _, _ in pieces:
      fn()
    return
  per = rows // 8
  total = len(rounds) * per * span / max(1, sum(p[2] for p in pieces))
  j, done, last = 0, 0, {}
  for k, rnd in enumerate(rounds):
    res = rnd()
    while j < len(pieces) and int(done * total) < (k + 1) * per:
      r = (int(done * total) - k * per) * 8
      fn, anchor, cost, chain = pieces[j]
      pin = res[r:r + 8, 0:128]
      anchor(pin + last[chain] if chain in last else pin)
      tok = fn()
      if chain is not None:
        last[chain] = tok[0:8, 0:128]
      j += 1
      done += cost


def _merge(*lists, cost=lambda v: 1):
  keyed = []
  for n, l in enumerate(lists):
    total, done = max(1, sum(cost(v) for v in l)), 0
    for i, v in enumerate(l):
      keyed.append(((done + 0.5 * cost(v)) / total, n, i, v))
      done += cost(v)
  return [v for _, _, _, v in sorted(keyed, key=lambda e: e[:3])]


def _merge_groups(*lists):
  merged = _merge(*lists, cost=lambda g: sum(p[2] for p in g))
  return [p for g in merged for p in g]


def _kernel(x_hbm, wq_hbm, wk_hbm, wv_hbm, wao_hbm, wup_hbm, dw_hbm, wdn_hbm, wm_hbm,
            o_hbm, xb, ae, ke, ve, gb, dwb, wqk, wvom, wup, stage, w_sem, x_sem, o_sem):
  nbatch = x_hbm.shape[0]

  def x_copies(b, part):
    cps = []
    if _DEV is not None: return cps
    for a in range(4):
      lo, hi = (0, 256) if part == 0 else (256, min(QS, T - a * QS))
      rows = pl.ds(a * QS + lo, hi - lo)
      cps.append(pltpu.make_async_copy(
          x_hbm.at[b, rows, :], xb.at[b, rows, :], x_sem.at[b * 8 + part * 4 + a]))
    return cps

  def o_copies(b, j, par, last=False):
    cps = []
    for a in range(4):
      n = min(QR, T - (a * QS + (NB - 1) * QR)) if last else QR
      cps.append(pltpu.make_async_copy(
          stage.at[par, a, pl.ds(0, n), :],
          o_hbm.at[b, pl.ds(a * QS + j * QR, n), :], o_sem.at[par * 4 + a]))
    return cps

  def block_fetch(src, g):
    def fetch(i, j):
      return src[i * 128 + 16 * g:i * 128 + 16 * g + 16, j * 128:j * 128 + 128].astype(F32)
    return fetch

  def encode_b(src, dst, t, g):
    def store(p, v):
      dst[t, p, 16 * g:16 * g + 16, :] = v.astype(BF16)
    return _encode_steps(block_fetch(src, g), _B_STEPS, _B_TERMS, _enc_b, store)

  def weights(wq, wk, wv, wao, wdn, wm, dw, tmp):
    srcs = (wq_hbm, wk_hbm, wv_hbm, wao_hbm, wm_hbm, wdn_hbm, wup_hbm, dw_hbm)
    dsts = (wq, wk, wv, wao, wm, wdn, wup, dw)
    cps = [pltpu.make_async_copy(s, d, w_sem.at[i])
           for i, (s, d) in enumerate(zip(srcs, dsts))]
    for cp in cps:
      cp.start()
    for cp in x_copies(0, 0) + x_copies(0, 1):
      cp.start()
    for b in range(nbatch):
      xb[b, T:XROWS, :] = jnp.zeros((XROWS - T, D), BF16)
    for c in range(4):
      gb[c, 0:GOFF, :] = jnp.zeros((GOFF, 128), F32)
    cps[0].wait()
    cps[1].wait()
    wqk[...] = (_dot_nt(wq[...], wk[...]) * (LOG2E * D ** -0.5)).astype(BF16)
    cps[2].wait()
    cps[3].wait()
    cps[4].wait()
    wvom[...] = _dot(_dot(wv[...], wao[...]).astype(BF16), wm[0:D, :]).astype(BF16)
    cps[5].wait()
    tmp[...] = _dot(wdn[...], wm[D:2 * D, :])
    cps[6].wait()
    cps[7].wait()
    for src, dst in ((wup, ke), (tmp, ve)):
      for g in range(8):
        for fn in encode_b(src, dst, NT, g):
          fn()
    taps = dw[...].astype(F32)
    for c in range(4):
      for k in range(KW):
        dwb[c, k] = jnp.broadcast_to(taps[k:k + 1, c * 128:c * 128 + 128], (8, 128))

  sq = pltpu.VMEM((D, D), BF16)
  if _DEV is None: pl.run_scoped(weights, sq, sq, sq, sq, sq, pltpu.VMEM((2 * D, D), BF16),
                pltpu.VMEM((KW, D), BF16), pltpu.VMEM((D, D), F32))

  def phase1(b, z, xa0, xa1, xf, k0, k1, v0, v1, g0, g1):
    xas, ks, vs, gs = (xa0, xa1), (k0, k1), (v0, v1), (g0, g1)

    def anchor(ref):
      def put(v):
        ref[pl.ds(pl.multiple_of(D + z, 8), 8), 0:128] = v
      return put

    def norm_piece(t, par, a, g):
      r0 = pl.multiple_of(a * QS + 16 * g + 128 * t, 16)
      xa = _layernorm(xb[b, pl.ds(r0, 16), :].astype(F32))
      rows = slice(a * 128 + 16 * g, a * 128 + 16 * g + 16)
      xas[par][rows, :] = xa.astype(BF16)
      xf[rows, :] = xa

    def encode_a(t, g):
      rows = pl.ds(pl.multiple_of(128 * t + 16 * g, 16), 16)

      def store(p, v):
        ae[p, rows, :] = v.astype(BF16)
      return _encode_steps(block_fetch(xf, g), _A_STEPS, _A_TERMS, _enc_a, store)

    def gate_piece(t, par, a, g):
      v = _layernorm(_gelu(gs[par][a * 128 + 8 * g:a * 128 + 8 * g + 8, :]))
      rows = pl.ds(pl.multiple_of(GOFF + a * QS + 8 * g + 128 * t, 8), 8)
      for c in range(4):
        gb[c, rows, :] = v[:, c * 128:c * 128 + 128]
      return v

    def step(t, par, dots, post, norm):
      rounds = []
      if dots:
        def proj(dst, n, fn):
          def rnd():
            res = fn()
            dst[0:D, n * 128:n * 128 + 128] = res
            return res
          return rnd
        xa = xas[par]
        for n in range(4):
          cols = slice(n * 128, n * 128 + 128)
          rounds.append(proj(gs[par], n, lambda cols=cols: _dot(
              xa[...], wup[:, D + cols.start:D + cols.stop])))
        for n in range(4):
          cols = slice(n * 128, n * 128 + 128)
          rounds.append(proj(ks[par], n, lambda cols=cols: _dot_nt(wqk[...], xa[cols, :])))
        for n in range(4):
          cols = slice(n * 128, n * 128 + 128)
          rounds.append(proj(vs[par], n, lambda cols=cols: _dot(xa[...], wvom[:, cols])))
      lists = []
      if post:
        q = 1 - par
        lists.append([[(functools.partial(gate_piece, t - 1, q, a, g), anchor(gs[q]), 30, None)]
                      for a in range(4) for g in range(16)])
        for src, dst in ((ks[q], ke), (vs[q], ve)):
          lists.append([[(fn, anchor(src), c, 1) for fn, c in
                         zip(encode_b(src, dst, t - 1, g), (35, 25, 25))] for g in range(8)])
      if norm:
        def xanchor(v):
          xb[nbatch, pl.ds(pl.multiple_of(z, 16), 16), 0:128] = jnp.concatenate(
              [v, v], axis=0).astype(BF16)
        norms = [[(functools.partial(norm_piece, t + 1, 1 - par, a, g), xanchor, 30, None)]
                 for g in range(8) for a in range(4)]
        encs = [[(fn, anchor(xf), c, 1) for fn, c in zip(encode_a(t + 1, g), (35, 25, 25))]
                for g in range(8)]
        lists.append(norms + encs)
      _run(rounds, _merge_groups(*lists), D, span=0.95)

    step(-1, 1, False, False, True)
    step(0, 0, True, False, True)
    for cp in x_copies(b, 1):
      cp.wait()

    def pair(i, carry):
      step(2 * i + 1, 1, True, True, True)
      step(2 * i + 2, 0, True, True, True)
      return carry
    lax.fori_loop(0, (NT - 2) // 2, pair, None)
    step(NT - 1, 1, True, True, False)
    step(NT, 0, False, True, False)

  def phase2(b, z, sb, pr0, pr1, pr2, pe_a, pe_b, pe_z, oacc, ofin, cv):
    prs = [(pr0, pr1)[t % 2] for t in range(NT)] + [pr2]
    left = [PR_LEFT + t // 2 for t in range(NT)] + [PR_LEFT]

    def anchor(ref, slot):
      def put(v):
        ref[slot + z, 0:8, :] = v
      return put

    def s_prod(m, t, o, p):
      lhs = _ldb(ae, 7 * o + p, pl.ds(pl.multiple_of(m * (QR // 2), 8), QR // 2), slice(None))
      return _dot(lhs, _ldb(ke, t, 7 * o + p))

    raw = [(o, p) for o in (5, 6) for p in (0, 2, 4)]

    def s_round_a(m, t, o):
      m2, m4, m6, m7 = [s_prod(m, t, o, p) for p in (1, 3, 5, 6)]
      pr = prs[t]
      pr[3 * o] = m4 + m7
      pr[3 * o + 1] = m2 + m4
      pr[3 * o + 2] = m6 - m2
      return m7

    def s_round_b(m, t, o):
      m1, m3, m5 = [s_prod(m, t, o, p) for p in (0, 2, 4)]
      extra = s_prod(m, t, *raw[o])
      pr = prs[t]
      pr[21 + 2 * o] = m1 - m5
      pr[22 + 2 * o] = m3 + m5
      pr[PR_RAW + o] = extra
      return extra

    def z_prod(p):
      res = _dot(_ldb(pe_z, p), _ldb(ve, NT, p))
      oacc[p] = res
      return res

    def left_round(m, tiles, z_too):
      res = None
      for t in tiles:
        res = s_prod(m, t, *raw[5])
        prs[t][left[t]] = res
      if z_too:
        res = z_prod(48)
      return res

    def z_round(k):
      return [z_prod(p) for p in range(4 * k, 4 * k + 4)][-1]

    def pv_round(second, p):
      pe = pe_b if second else pe_a
      lhs = jnp.concatenate([_ldb(pe, 49 * i + p) for i in range(4)], axis=1)
      rhs = jnp.concatenate([_ldb(ve, 4 * second + i, p) for i in range(4)], axis=0)
      res = _dot(lhs, rhs)
      (ofin if second else oacc)[p] = oacc[p] + res
      return res

    def comb_piece(t, r, i):
      rows = slice(r, r + 8)
      pr = prs[t]

      def inner(o):
        if o < 5:
          xx, yy = pr[21 + 2 * o, rows, :], pr[22 + 2 * o, rows, :]
        else:
          slots = [PR_RAW + n if n < 5 else left[t]
                   for n in range(3 * (o - 5), 3 * (o - 5) + 3)]
          m1, m3, m5 = [pr[n, rows, :] for n in slots]
          xx, yy = m1 - m5, m3 + m5
        if i == 0:
          return {(0, 0): xx + pr[3 * o, rows, :], (0, 1): yy}
        return {(1, 0): pr[3 * o + 1, rows, :], (1, 1): xx + yy + pr[3 * o + 2, rows, :]}
      c = _decode_outer(inner)
      if t == NT:
        for (a, k), v in c.items():
          sb[SL_U + 4 * a + k, rows, :] = _gelu(v)
        return c[(i, 0)]
      if t == NT - 1:
        lane = lax.broadcasted_iota(jnp.int32, (8, 128), 1)
      for a in (i, i + 2):
        vs = [c[(a, k)] for k in range(4)]
        if t == NT - 1:
          vs = [jnp.where(lane < min(QS, T - k * QS) - 128 * t, v, -jnp.inf)
                for k, v in enumerate(vs)]
        for k in range(4):
          sb[16 * t + 4 * a + k, rows, :] = vs[k]
        mx = jnp.maximum(jnp.maximum(vs[0], vs[1]), jnp.maximum(vs[2], vs[3]))
        if t > 0:
          m_old = sb[SL_M + a, rows, :]
          mx = jnp.maximum(mx, m_old)
        e = [jnp.exp2(v - mx) for v in vs]
        ls = (e[0] + e[1]) + (e[2] + e[3])
        if t > 0:
          ls = ls + sb[SL_L + a, rows, :] * jnp.exp2(m_old - mx)
        sb[SL_M + a, rows, :] = mx
        sb[SL_L + a, rows, :] = ls
      return mx

    def norm_const_steps(r):
      rows = slice(r, r + 8)
      off = []

      def compute():
        for a in range(4):
          mx = sb[SL_M + a, rows, :]
          m_row = jnp.max(mx, axis=-1, keepdims=True)
          l_row = jnp.sum(sb[SL_L + a, rows, :] * jnp.exp2(mx - m_row), axis=-1, keepdims=True)
          off.append(jnp.broadcast_to(m_row + jnp.log2(l_row), (8, 128)))

      def store():
        for a in range(4):
          sb[SL_OFF + a, rows, :] = off[a]
      return compute, store

    def prep_steps(t, r):
      rows = slice(r, r + 16)

      def fetch(a, k):
        if t < NT:
          return jnp.exp2(sb[16 * t + 4 * a + k, rows, :] - sb[SL_OFF + a, rows, :])
        return sb[SL_U + 4 * a + k, rows, :] * cv[4 * a + k, rows, :]

      def store(p, v):
        if t == NT:
          pe_z[p, rows, :] = v.astype(BF16)
        else:
          (pe_a if t < 4 else pe_b)[49 * (t % 4) + p, rows, :] = v.astype(BF16)
      return _encode_steps(fetch, _A_STEPS, _A_TERMS, _enc_a, store)

    def conv_steps(j, a, c, r):
      base = GOFF - KW // 2 + a * QS + r + j * QR
      acc = [None] * CONV_N

      def step(shifts):
        for sh in shifts:
          taps = range(sh, KW, 8)
          g = [gb[c, pl.ds(base + sh + 8 * i, 8), :] for i in range(CONV_N + len(taps) - 1)]
          for q, k in enumerate(taps):
            w = dwb[c, k]
            for h in range(CONV_N):
              v = g[h + q] * w
              acc[h] = v if acc[h] is None else acc[h] + v
        if shifts[-1] == 7:
          for h in range(CONV_N):
            cv[4 * a + c, r + 8 * h:r + 8 * h + 8, :] = acc[h]
        return acc[-1]
      return [functools.partial(step, range(s0, s0 + CONV_SH)) for s0 in range(0, 8, CONV_SH)]

    def out_piece(j, par, r):
      halves = []
      for h in range(2):
        rows = slice(r + 8 * h, r + 8 * h + 8)
        halves.append(_decode_outer(
            lambda o: _decode_inner([ofin[7 * o + p, rows, :] for p in range(7)])))
      for a in range(4):
        xr = pl.ds(pl.multiple_of(a * QS + r + j * QR, 16), 16)
        for k in range(4):
          cols = slice(k * 128, k * 128 + 128)
          y = jnp.concatenate([halves[0][(a, k)], halves[1][(a, k)]], axis=0)
          y = xb[b, xr, cols].astype(F32) + y
          stage[par, a, r:r + 16, cols] = y.astype(BF16)
      return y

    def ganchor(v):
      gb[4, pl.ds(pl.multiple_of(z, 8), 8), :] = v

    def zanchor(v):
      anchor(sb, SL_DUMMY)(v)
      anchor(cv, 16)(v)

    def iteration(m, do_s, do_p, do_o):
      part = functools.partial
      par = m % 2
      convs = [[(fn, ganchor, CONV_N * CONV_SH * 2.8, 0) for fn in conv_steps(m, a, c, r)]
               for a in range(4) for c in range(4) for r in range(0, QR, 8 * CONV_N)]
      outs = [[(part(out_piece, m - 2, par, r), anchor(ofin, 49), 90, 1)]
              for r in range(0, QR, 16)]
      first, zk = [[] for _ in range(5)], 0
      for j, (n_b, n_z) in enumerate(((12, 0), (9, 3), (9, 3), (10, 3), (9, 3))):
        p0 = sum((0, 12, 9, 9, 10)[:j + 1])
        bs = [part(pv_round, 1, p) for p in range(p0, p0 + n_b)] if do_o else []
        zs = [part(z_round, k) for k in range(zk, zk + n_z)] if do_p else []
        zk += n_z
        first[j] = bs + zs if j == 4 else _merge(bs, zs)
      pv_split = [0, 12, 24, 36, 49]
      for j in range(NT + 1):
        s_rounds, v_rounds = [], []
        if do_s:
          if j in (0, 4):
            s_rounds.append(part(left_round, m, range(j, j + 4), False))
          for o in range(7):
            s_rounds.append(part(s_round_a, m, j, o))
            if o < 5:
              s_rounds.append(part(s_round_b, m, j, o))
        if j < 5:
          v_rounds = first[j]
        if j == 4 and (do_s or do_p):
          v_rounds.append(part(left_round, m, [NT] if do_s else [], do_p))
        if do_p and j > 4:
          if j == 5:
            anchor(oacc, 49)(jnp.zeros((8, 128), F32))
            pe_a[4 * 49 + z, 0:16, :] = jnp.zeros((16, 128), BF16)
          v_rounds = [part(pv_round, 0, p) for p in range(pv_split[j - 5], pv_split[j - 4])]
        t = j - 1 if j > 0 else NT
        main = []
        for r in range(0, QR, 8):
          combs = [[(part(comb_piece, t, r, i), anchor(prs[t], PR_DUMMY), 30 if j else 36, 1)]
                   for i in range(2)]
          if j > 0:
            if do_p and r % 16 == 0:
              main.append([(fn, anchor(sb, SL_DUMMY), c, 1)
                           for fn, c in zip(prep_steps(t, r), (50, 32, 32))])
            if do_s:
              main += combs
          elif do_p:
            main += combs
            if r % 16 == 8:
              main.append([(fn, zanchor, c, 1)
                           for fn, c in zip(prep_steps(t, r - 8), (40, 28, 28))])
        lists = [main]
        if do_s and j > 0:
          n = len(convs) // NT
          lists.append(convs[(j - 1) * n:j * n])
        if do_p and j == 0:
          steps = [norm_const_steps(r) for r in range(0, QR, 8)]
          seq = []
          for n in range(len(steps) + 3):
            if n < len(steps):
              seq.append([(steps[n][0], anchor(sb, SL_DUMMY), 10, None)])
            if n >= 3:
              seq.append([(steps[n - 3][1], lambda v: None, 1, None)])
          lists.append(seq)
        if do_o and j > 4:
          lists.append(outs[(9 * (j - 5)) // 4:(9 * (j - 4)) // 4])
        _run(_merge(s_rounds, v_rounds), _merge_groups(*lists), QR, span=SPAN)

    if _DEV is not None:
      lax.fori_loop(2, NB, lambda m, c: iteration(m, *_DEV), None)
      return
    iteration(0, True, False, False)

    @pl.when(b > 0)
    def _():
      for cp in o_copies(b - 1, NB - 2, 1) + o_copies(b - 1, NB - 1, 0, last=True):
        cp.wait()
    iteration(1, True, True, False)

    def steady(m, carry):
      @pl.when(m >= 4)
      def _():
        for cp in o_copies(b, m - 4, m % 2):
          cp.wait()
      iteration(m, True, True, True)
      for cp in o_copies(b, m - 2, m % 2):
        cp.start()
      return carry
    lax.fori_loop(2, NB, steady, None)
    for cp in o_copies(b, NB - 4, NB % 2):
      cp.wait()
    iteration(NB, False, True, True)
    for cp in o_copies(b, NB - 2, NB % 2):
      cp.start()
    for cp in o_copies(b, NB - 3, (NB + 1) % 2):
      cp.wait()
    iteration(NB + 1, False, False, True)
    for cp in o_copies(b, NB - 1, (NB + 1) % 2, last=True):
      cp.start()

  def batch(b, carry):
    z = lax.shift_right_logical(b, 8)
    for cp in x_copies(b, 0):
      cp.wait()
    st = pltpu.VMEM((D + 8, D), F32)
    if _DEV is None or _DEV == 'p1': pl.run_scoped(functools.partial(phase1, b, z), sq, sq, st, st, st, st, st, st, st)

    @pl.when(b + 1 < nbatch)
    def _():
      for cp in x_copies(b + 1, 0) + x_copies(b + 1, 1):
        cp.start()
    blocks = lambda n: pltpu.VMEM((n, QR, 128), F32)
    if _DEV == 'p1':
      @pl.when(z > 0)
      def _():
        stage[0, 0, :, 0:128] = ae[z, 0:QR, :] + ke[z, z, 0:16, :].sum() + ve[z, z, 0:16, :].sum()
    if _DEV != 'p1': pl.run_scoped(
        functools.partial(phase2, b, z),
        blocks(SL_DUMMY + 1), blocks(PR_DUMMY + 1), blocks(PR_DUMMY + 1), blocks(PR_DUMMY + 1),
        pltpu.VMEM((4 * 49 + 1, QR, 128), BF16), pltpu.VMEM((4 * 49, QR, 128), BF16),
        pltpu.VMEM((49, QR, 128), BF16), blocks(50), blocks(50), blocks(17))
    return carry

  lax.fori_loop(0, nbatch, batch, None)
  if _DEV is not None:
    for cp in o_copies(0, 0, 0):
      cp.start(); cp.wait()
    return
  for cp in o_copies(nbatch - 1, NB - 2, 1) + o_copies(nbatch - 1, NB - 1, 0, last=True):
    cp.wait()


@jax.jit
def pallas_standalone__conformer_family_branchformer__speech_kernel(
    x: jax.Array,
    w_q: jax.Array,
    w_k: jax.Array,
    w_v: jax.Array,
    w_ao: jax.Array,
    w_up: jax.Array,
    dw: jax.Array,
    w_dn: jax.Array,
    w_merge: jax.Array,
):
  nbatch = x.shape[0]
  assert x.shape[1:] == (T, D) and dw.shape == (KW, D)
  any_spec = pl.BlockSpec(memory_space=pl.ANY)
  return pl.pallas_call(
      _kernel,
      out_shape=jax.ShapeDtypeStruct(x.shape, x.dtype),
      in_specs=[any_spec] * 9,
      out_specs=any_spec,
      scratch_shapes=[
          pltpu.VMEM((nbatch + 1, XROWS, D), BF16),
          pltpu.VMEM((49, NT * 128, 128), BF16),
          pltpu.VMEM((NT + 1, 49, 128, 128), BF16),
          pltpu.VMEM((NT + 1, 49, 128, 128), BF16),
          pltpu.VMEM((5, GOFF + XROWS, 128), F32),
          pltpu.VMEM((4, KW, 8, 128), F32),
          pltpu.VMEM((D, D), BF16),
          pltpu.VMEM((D, D), BF16),
          pltpu.VMEM((D, 2 * D), BF16),
          pltpu.VMEM((2, 4, QR, D), BF16),
          pltpu.SemaphoreType.DMA((8,)),
          pltpu.SemaphoreType.DMA((8 * nbatch,)),
          pltpu.SemaphoreType.DMA((8,)),
      ],
      compiler_params=pltpu.CompilerParams(vmem_limit_bytes=126 * 1024 * 1024),
      name="branchformer",
  )(x, w_q, w_k, w_v, w_ao, w_up, dw, w_dn, w_merge)
```

```python
import functools

import jax
import jax.numpy as jnp
from jax import lax
import jax.experimental.pallas as pl
import jax.experimental.pallas.tpu as pltpu

F32, BF16, U32 = jnp.float32, jnp.bfloat16, jnp.uint32

T, D, KW = 4000, 512, 31
QS = 1008
QR = 144
NB = 7
NT = 8
XROWS = 3 * QS + NT * 128
AE_ROWS = 7104
GOFF = 16
EPS = 1e-5
LOG2E = 1.4426950408889634

_DEV = None
CONV_N = 3
CONV_SH = 2
SPAN = 0.99
CW, CCH, OCH = 2.8, 0, 1
PC = (50, 32, 32)
CC = 30

SL_U = 16 * NT
SL_M = SL_U + 16
SL_L = SL_M + 4
SL_OFF = SL_L + 4
SL_DUMMY = SL_OFF + 4
PR_RAW = 31
PR_LEFT = 36
PR_DUMMY = 40


def _enc_a(a11, a12, a21, a22):
  return [a11 + a22, a21 + a22, a11, a22, a11 + a12, a21 - a11, a12 - a22]


def _enc_b(b11, b12, b21, b22):
  return [b11 + b22, b11, b12 - b22, b21 - b11, b22, b11 + b12, b21 + b22]


_A_TERMS = ([(0, 0, 1), (1, 1, 1)], [(1, 0, 1), (1, 1, 1)], [(0, 0, 1)], [(1, 1, 1)],
            [(0, 0, 1), (0, 1, 1)], [(1, 0, 1), (0, 0, -1)], [(0, 1, 1), (1, 1, -1)])
_B_TERMS = ([(0, 0, 1), (1, 1, 1)], [(0, 0, 1)], [(0, 1, 1), (1, 1, -1)],
            [(1, 0, 1), (0, 0, -1)], [(1, 1, 1)], [(0, 0, 1), (0, 1, 1)],
            [(1, 0, 1), (1, 1, 1)])
_USE = ([((0, 0), 1), ((1, 1), 1)], [((1, 0), 1), ((1, 1), -1)],
        [((0, 1), 1), ((1, 1), 1)], [((0, 0), 1), ((1, 0), 1)],
        [((0, 0), -1), ((0, 1), 1)], [((1, 1), 1)], [((0, 0), 1)])


def _lin(terms):
  acc = None
  for v, s in terms:
    if acc is None:
      acc = v
    else:
      acc = acc + v if s > 0 else acc - v
  return acc


def _encode2(blk, terms, enc, store, outer=range(7)):
  for o in outer:
    q = [[_lin([(blk[2 * r + i][2 * c + j], s) for r, c, s in terms[o]])
          for j in range(2)] for i in range(2)]
    for p, v in enumerate(enc(q[0][0], q[0][1], q[1][0], q[1][1])):
      store(7 * o + p, v)
  return v


_A_STEPS = (([(0, 0), (1, 1)], (2, 0, 3)), ([(1, 0)], (1, 5)), ([(0, 1)], (4, 6)))
_B_STEPS = (([(0, 0), (1, 1)], (1, 0, 4)), ([(0, 1)], (2, 5)), ([(1, 0)], (3, 6)))


def _encode_steps(fetch, steps, terms, enc, store):
  blk = [[None] * 4 for _ in range(4)]

  def step(quads, outer):
    for r, c in quads:
      for i in range(2):
        for j in range(2):
          blk[2 * r + i][2 * c + j] = fetch(2 * r + i, 2 * c + j)
    return _encode2(blk, terms, enc, store, outer)
  return [functools.partial(step, *st) for st in steps]


def _decode_outer(inner):
  c = {}
  for o in range(7):
    quad = inner(o)
    for qi, v in quad.items():
      for qo, s in _USE[o]:
        key = (2 * qo[0] + qi[0], 2 * qo[1] + qi[1])
        if key not in c:
          c[key] = v
        else:
          c[key] = c[key] + v if s > 0 else c[key] - v
  return c


def _decode_inner(m):
  return {(0, 0): m[0] + m[3] - m[4] + m[6], (0, 1): m[2] + m[4],
          (1, 0): m[1] + m[3], (1, 1): m[0] - m[1] + m[2] + m[5]}


def _layernorm(v):
  mean = jnp.sum(v, axis=-1, keepdims=True) * (1.0 / D)
  d = v - mean
  var = jnp.sum(d * d, axis=-1, keepdims=True) * (1.0 / D)
  return d * lax.rsqrt(var + EPS)


def _gelu(v):
  c1 = 0.7978845608028654
  inner = v * (c1 + (c1 * 0.044715) * (v * v))
  h = 0.5 * v
  return h + h * jnp.tanh(inner)


def _dot(a, b):
  return jnp.dot(a, b, preferred_element_type=F32)


def _dot_nt(a, b):
  return lax.dot_general(a, b, (((1,), (1,)), ((), ())), preferred_element_type=F32)


def _ldb(ref, *idx):
  return pltpu.bitcast(ref.bitcast(U32)[idx], BF16)


def _run(rounds, pieces, rows, span=1.0):
  if not rounds:
    for fn, _, _, _ in pieces:
      fn()
    return
  per = rows // 8
  total = len(rounds) * per * span / max(1, sum(p[2] for p in pieces))
  j, done, last = 0, 0, {}
  for k, rnd in enumerate(rounds):
    res = rnd()
    while j < len(pieces) and int(done * total) < (k + 1) * per:
      r = (int(done * total) - k * per) * 8
      fn, anchor, cost, chain = pieces[j]
      pin = res[r:r + 8, 0:128]
      anchor(pin + last[chain] if chain in last else pin)
      tok = fn()
      if chain is not None:
        last[chain] = tok[0:8, 0:128]
      j += 1
      done += cost


def _merge(*lists, cost=lambda v: 1):
  keyed = []
  for n, l in enumerate(lists):
    total, done = max(1, sum(cost(v) for v in l)), 0
    for i, v in enumerate(l):
      keyed.append(((done + 0.5 * cost(v)) / total, n, i, v))
      done += cost(v)
  return [v for _, _, _, v in sorted(keyed, key=lambda e: e[:3])]


def _merge_groups(*lists):
  merged = _merge(*lists, cost=lambda g: sum(p[2] for p in g))
  return [p for g in merged for p in g]


def _kernel(x_hbm, wq_hbm, wk_hbm, wv_hbm, wao_hbm, wup_hbm, dw_hbm, wdn_hbm, wm_hbm,
            o_hbm, xb, ae, ke, ve, gb, dwb, wqk, wvom, wup, stage, w_sem, x_sem, o_sem):
  nbatch = x_hbm.shape[0]

  def x_copies(b, part):
    cps = []
    if _DEV is not None: return cps
    for a in range(4):
      lo, hi = (0, 256) if part == 0 else (256, min(QS, T - a * QS))
      rows = pl.ds(a * QS + lo, hi - lo)
      cps.append(pltpu.make_async_copy(
          x_hbm.at[b, rows, :], xb.at[b, rows, :], x_sem.at[b * 8 + part * 4 + a]))
    return cps

  def o_copies(b, j, par, last=False):
    cps = []
    for a in range(4):
      n = min(QR, T - (a * QS + (NB - 1) * QR)) if last else QR
      cps.append(pltpu.make_async_copy(
          stage.at[par, a, pl.ds(0, n), :],
          o_hbm.at[b, pl.ds(a * QS + j * QR, n), :], o_sem.at[par * 4 + a]))
    return cps

  def block_fetch(src, g):
    def fetch(i, j):
      return src[i * 128 + 16 * g:i * 128 + 16 * g + 16, j * 128:j * 128 + 128].astype(F32)
    return fetch

  def encode_b(src, dst, t, g):
    def store(p, v):
      dst[t, p, 16 * g:16 * g + 16, :] = v.astype(BF16)
    return _encode_steps(block_fetch(src, g), _B_STEPS, _B_TERMS, _enc_b, store)

  def weights(wq, wk, wv, wao, wdn, wm, dw, tmp):
    srcs = (wq_hbm, wk_hbm, wv_hbm, wao_hbm, wm_hbm, wdn_hbm, wup_hbm, dw_hbm)
    dsts = (wq, wk, wv, wao, wm, wdn, wup, dw)
    cps = [pltpu.make_async_copy(s, d, w_sem.at[i])
           for i, (s, d) in enumerate(zip(srcs, dsts))]
    for cp in cps:
      cp.start()
    for cp in x_copies(0, 0) + x_copies(0, 1):
      cp.start()
    for b in range(nbatch):
      xb[b, T:XROWS, :] = jnp.zeros((XROWS - T, D), BF16)
    for c in range(4):
      gb[c, 0:GOFF, :] = jnp.zeros((GOFF, 128), F32)
    cps[0].wait()
    cps[1].wait()
    wqk[...] = (_dot_nt(wq[...], wk[...]) * (LOG2E * D ** -0.5)).astype(BF16)
    cps[2].wait()
    cps[3].wait()
    cps[4].wait()
    wvom[...] = _dot(_dot(wv[...], wao[...]).astype(BF16), wm[0:D, :]).astype(BF16)
    cps[5].wait()
    tmp[...] = _dot(wdn[...], wm[D:2 * D, :])
    cps[6].wait()
    cps[7].wait()
    for src, dst in ((wup, ke), (tmp, ve)):
      for g in range(8):
        for fn in encode_b(src, dst, NT, g):
          fn()
    taps = dw[...].astype(F32)
    for c in range(4):
      for k in range(KW):
        dwb[c, k] = jnp.broadcast_to(taps[k:k + 1, c * 128:c * 128 + 128], (8, 128))

  sq = pltpu.VMEM((D, D), BF16)
  if _DEV is None: pl.run_scoped(weights, sq, sq, sq, sq, sq, pltpu.VMEM((2 * D, D), BF16),
                pltpu.VMEM((KW, D), BF16), pltpu.VMEM((D, D), F32))

  def phase1(b, z, xa0, xa1, xf, k0, k1, v0, v1, g0, g1):
    xas, ks, vs, gs = (xa0, xa1), (k0, k1), (v0, v1), (g0, g1)

    def anchor(ref):
      def put(v):
        ref[pl.ds(pl.multiple_of(D + z, 8), 8), 0:128] = v
      return put

    def norm_piece(t, par, a, g):
      r0 = pl.multiple_of(a * QS + 16 * g + 128 * t, 16)
      xa = _layernorm(xb[b, pl.ds(r0, 16), :].astype(F32))
      rows = slice(a * 128 + 16 * g, a * 128 + 16 * g + 16)
      xas[par][rows, :] = xa.astype(BF16)
      xf[rows, :] = xa

    def encode_a(t, g):
      pos = 128 * t + 16 * g
      j, r = pos // QR, pos % QR

      def store(p, v):
        ae[j, pl.ds(pl.multiple_of(p * QR + r, 16), 16), :] = v.astype(BF16)
      return _encode_steps(block_fetch(xf, g), _A_STEPS, _A_TERMS, _enc_a, store)

    def gate_piece(t, par, a, g):
      v = _layernorm(_gelu(gs[par][a * 128 + 8 * g:a * 128 + 8 * g + 8, :]))
      rows = pl.ds(pl.multiple_of(GOFF + a * QS + 8 * g + 128 * t, 8), 8)
      for c in range(4):
        gb[c, rows, :] = v[:, c * 128:c * 128 + 128]
      return v

    def step(t, par, dots, post, norm):
      rounds = []
      if dots:
        def proj(dst, n, fn):
          def rnd():
            res = fn()
            dst[0:D, n * 128:n * 128 + 128] = res
            return res
          return rnd
        xa = xas[par]
        for n in range(4):
          cols = slice(n * 128, n * 128 + 128)
          rounds.append(proj(gs[par], n, lambda cols=cols: _dot(
              xa[...], wup[:, D + cols.start:D + cols.stop])))
        for n in range(4):
          cols = slice(n * 128, n * 128 + 128)
          rounds.append(proj(ks[par], n, lambda cols=cols: _dot_nt(wqk[...], xa[cols, :])))
        for n in range(4):
          cols = slice(n * 128, n * 128 + 128)
          rounds.append(proj(vs[par], n, lambda cols=cols: _dot(xa[...], wvom[:, cols])))
      lists = []
      if post:
        q = 1 - par
        lists.append([[(functools.partial(gate_piece, t - 1, q, a, g), anchor(gs[q]), 30, None)]
                      for a in range(4) for g in range(16)])
        for src, dst in ((ks[q], ke), (vs[q], ve)):
          lists.append([[(fn, anchor(src), c, 1) for fn, c in
                         zip(encode_b(src, dst, t - 1, g), (35, 25, 25))] for g in range(8)])
      if norm:
        def xanchor(v):
          xb[0, pl.ds(pl.multiple_of(XROWS + z, 16), 16), 0:128] = jnp.concatenate(
              [v, v], axis=0).astype(BF16)
        norms = [[(functools.partial(norm_piece, t + 1, 1 - par, a, g), xanchor, 30, None)]
                 for g in range(8) for a in range(4)]
        encs = [[(fn, anchor(xf), c, 1) for fn, c in zip(encode_a(t + 1, g), (35, 25, 25))]
                for g in range(8)]
        lists.append(norms + encs)
      _run(rounds, _merge_groups(*lists), D, span=0.95)

    step(-1, 1, False, False, True)
    step(0, 0, True, False, True)
    for cp in x_copies(b, 1):
      cp.wait()

    def pair(i, carry):
      step(2 * i + 1, 1, True, True, True)
      step(2 * i + 2, 0, True, True, True)
      return carry
    lax.fori_loop(0, (NT - 2) // 2, pair, None)
    step(NT - 1, 1, True, True, False)
    step(NT, 0, False, True, False)

  def phase2(b, z, sb, pr0, pr1, pr2, pe_a, pe_b, pe_z, oacc, ofin, cv, gw):
    prs = [(pr0, pr1)[t % 2] for t in range(NT)] + [pr2]
    left = [PR_LEFT + t // 2 for t in range(NT)] + [PR_LEFT]

    def anchor(ref, slot):
      def put(v):
        ref[slot + z, 0:8, :] = v
      return put

    def s_prod(m, t, o, p):
      lhs = _ldb(ae, m, pl.ds((7 * o + p) * (QR // 2), QR // 2), slice(None))
      return _dot(lhs, _ldb(ke, t, 7 * o + p))

    raw = [(o, p) for o in (5, 6) for p in (0, 2, 4)]

    def s_round_a(m, t, o):
      m2, m4, m6, m7 = [s_prod(m, t, o, p) for p in (1, 3, 5, 6)]
      pr = prs[t]
      pr[3 * o] = m4 + m7
      pr[3 * o + 1] = m2 + m4
      pr[3 * o + 2] = m6 - m2
      return m7

    def s_round_b(m, t, o):
      m1, m3, m5 = [s_prod(m, t, o, p) for p in (0, 2, 4)]
      extra = s_prod(m, t, *raw[o])
      pr = prs[t]
      pr[21 + 2 * o] = m1 - m5
      pr[22 + 2 * o] = m3 + m5
      pr[PR_RAW + o] = extra
      return extra

    def z_prod(p):
      res = _dot(_ldb(pe_z, p), _ldb(ve, NT, p))
      oacc[p] = res
      return res

    def left_round(m, tiles, z_too):
      res = None
      for t in tiles:
        res = s_prod(m, t, *raw[5])
        prs[t][left[t]] = res
      if z_too:
        res = z_prod(48)
      return res

    def z_round(k):
      return [z_prod(p) for p in range(4 * k, 4 * k + 4)][-1]

    def pv_round(second, p):
      pe = pe_b if second else pe_a
      lhs = jnp.concatenate([_ldb(pe, 49 * i + p) for i in range(4)], axis=1)
      rhs = jnp.concatenate([_ldb(ve, 4 * second + i, p) for i in range(4)], axis=0)
      res = _dot(lhs, rhs)
      (ofin if second else oacc)[p] = oacc[p] + res
      return res

    def comb_piece(t, r, i):
      rows = slice(r, r + 8)
      pr = prs[t]

      def inner(o):
        if o < 5:
          xx, yy = pr[21 + 2 * o, rows, :], pr[22 + 2 * o, rows, :]
        else:
          slots = [PR_RAW + n if n < 5 else left[t]
                   for n in range(3 * (o - 5), 3 * (o - 5) + 3)]
          m1, m3, m5 = [pr[n, rows, :] for n in slots]
          xx, yy = m1 - m5, m3 + m5
        if i == 0:
          return {(0, 0): xx + pr[3 * o, rows, :], (0, 1): yy}
        return {(1, 0): pr[3 * o + 1, rows, :], (1, 1): xx + yy + pr[3 * o + 2, rows, :]}
      c = _decode_outer(inner)
      if t == NT:
        for (a, k), v in c.items():
          sb[SL_U + 4 * a + k, rows, :] = _gelu(v)
        return c[(i, 0)]
      if t == NT - 1:
        lane = lax.broadcasted_iota(jnp.int32, (8, 128), 1)
      for a in (i, i + 2):
        vs = [c[(a, k)] for k in range(4)]
        if t == NT - 1:
          vs = [jnp.where(lane < min(QS, T - k * QS) - 128 * t, v, -jnp.inf)
                for k, v in enumerate(vs)]
        for k in range(4):
          sb[16 * t + 4 * a + k, rows, :] = vs[k]
        mx = jnp.maximum(jnp.maximum(vs[0], vs[1]), jnp.maximum(vs[2], vs[3]))
        if t > 0:
          m_old = sb[SL_M + a, rows, :]
          mx = jnp.maximum(mx, m_old)
        e = [jnp.exp2(v - mx) for v in vs]
        ls = (e[0] + e[1]) + (e[2] + e[3])
        if t > 0:
          ls = ls + sb[SL_L + a, rows, :] * jnp.exp2(m_old - mx)
        sb[SL_M + a, rows, :] = mx
        sb[SL_L + a, rows, :] = ls
      return mx

    def norm_const_steps(r):
      rows = slice(r, r + 8)
      off = []

      def compute():
        for a in range(4):
          mx = sb[SL_M + a, rows, :]
          m_row = jnp.max(mx, axis=-1, keepdims=True)
          l_row = jnp.sum(sb[SL_L + a, rows, :] * jnp.exp2(mx - m_row), axis=-1, keepdims=True)
          off.append(jnp.broadcast_to(m_row + jnp.log2(l_row), (8, 128)))

      def store():
        for a in range(4):
          sb[SL_OFF + a, rows, :] = off[a]
      return compute, store

    def prep_steps(t, r):
      rows = slice(r, r + 16)

      def fetch(a, k):
        if t < NT:
          return jnp.exp2(sb[16 * t + 4 * a + k, rows, :] - sb[SL_OFF + a, rows, :])
        return sb[SL_U + 4 * a + k, rows, :] * cv[4 * a + k, rows, :]

      def store(p, v):
        if t == NT:
          pe_z[p, rows, :] = v.astype(BF16)
        else:
          (pe_a if t < 4 else pe_b)[49 * (t % 4) + p, rows, :] = v.astype(BF16)
      return _encode_steps(fetch, _A_STEPS, _A_TERMS, _enc_a, store)

    def window_piece(j, a, c):
      v = gb[c, pl.ds(pl.multiple_of(a * QS + j * QR, 16), QR + 2 * GOFF), :]
      gw[4 * a + c] = v
      return v

    def conv_steps(a, c, r):
      base = GOFF - KW // 2 + r
      acc = [None] * CONV_N

      def step(shifts):
        for sh in shifts:
          taps = range(sh, KW, 8)
          g = [gw[4 * a + c, pl.ds(base + sh + 8 * i, 8), :] for i in range(CONV_N + len(taps) - 1)]
          for q, k in enumerate(taps):
            w = dwb[c, k]
            for h in range(CONV_N):
              v = g[h + q] * w
              acc[h] = v if acc[h] is None else acc[h] + v
        if shifts[-1] == 7:
          for h in range(CONV_N):
            cv[4 * a + c, r + 8 * h:r + 8 * h + 8, :] = acc[h]
        return acc[-1]
      return [functools.partial(step, range(s0, s0 + CONV_SH)) for s0 in range(0, 8, CONV_SH)]

    def out_piece(j, par, r):
      halves = []
      for h in range(2):
        rows = slice(r + 8 * h, r + 8 * h + 8)
        halves.append(_decode_outer(
            lambda o: _decode_inner([ofin[7 * o + p, rows, :] for p in range(7)])))
      for a in range(4):
        xr = pl.ds(pl.multiple_of(a * QS + r + j * QR, 16), 16)
        for k in range(4):
          cols = slice(k * 128, k * 128 + 128)
          y = jnp.concatenate([halves[0][(a, k)], halves[1][(a, k)]], axis=0)
          y = xb[b, xr, cols].astype(F32) + y
          stage[par, a, r:r + 16, cols] = y.astype(BF16)
      return y

    def ganchor(v):
      gb[3, pl.ds(pl.multiple_of(GOFF + XROWS + z, 8), 8), :] = v

    def zanchor(v):
      anchor(sb, SL_DUMMY)(v)
      anchor(cv, 16)(v)

    def iteration(m, do_s, do_p, do_o):
      part = functools.partial
      par = m % 2
      convs = [[(fn, anchor(gw, 16), CONV_N * CONV_SH * CW, CCH) for fn in conv_steps(a, c, r)]
               for a in range(4) for c in range(4) for r in range(0, QR, 8 * CONV_N)]
      outs = [[(part(out_piece, m - 2, par, r), anchor(ofin, 49), 90, OCH)]
              for r in range(0, QR, 16)]
      first, zk = [[] for _ in range(5)], 0
      for j, (n_b, n_z) in enumerate(((12, 0), (9, 3), (9, 3), (10, 3), (9, 3))):
        p0 = sum((0, 12, 9, 9, 10)[:j + 1])
        bs = [part(pv_round, 1, p) for p in range(p0, p0 + n_b)] if do_o else []
        zs = [part(z_round, k) for k in range(zk, zk + n_z)] if do_p else []
        zk += n_z
        first[j] = bs + zs if j == 4 else _merge(bs, zs)
      pv_split = [0, 12, 24, 36, 49]
      for j in range(NT + 1):
        s_rounds, v_rounds = [], []
        if do_s:
          if j in (0, 4):
            s_rounds.append(part(left_round, m, range(j, j + 4), False))
          for o in range(7):
            s_rounds.append(part(s_round_a, m, j, o))
            if o < 5:
              s_rounds.append(part(s_round_b, m, j, o))
        if j < 5:
          v_rounds = first[j]
        if j == 4 and (do_s or do_p):
          v_rounds.append(part(left_round, m, [NT] if do_s else [], do_p))
        if do_p and j > 4:
          if j == 5:
            anchor(oacc, 49)(jnp.zeros((8, 128), F32))
            pe_a[4 * 49 + z, 0:16, :] = jnp.zeros((16, 128), BF16)
          v_rounds = [part(pv_round, 0, p) for p in range(pv_split[j - 5], pv_split[j - 4])]
        t = j - 1 if j > 0 else NT
        main = []
        for r in range(0, QR, 8):
          combs = [[(part(comb_piece, t, r, i), anchor(prs[t], PR_DUMMY), CC if j else 36, 1)]
                   for i in range(2)]
          if j > 0:
            if do_p and r % 16 == 0:
              main.append([(fn, anchor(sb, SL_DUMMY), c, 1)
                           for fn, c in zip(prep_steps(t, r), PC)])
            if do_s:
              main += combs
          elif do_p:
            main += combs
            if r % 16 == 8:
              main.append([(fn, zanchor, c, 1)
                           for fn, c in zip(prep_steps(t, r - 8), (40, 28, 28))])
        lists = [main]
        if do_s and do_p and not do_o:
          if j > 4:
            n = len(convs) // 4
            lists.append(convs[(j - 5) * n:(j - 4) * n])
        elif do_s and j > 0:
          n = len(convs) // NT
          lists.append(convs[(j - 1) * n:j * n])
        if do_s and j == 0:
          lists.append([[(part(window_piece, m, a, c), ganchor, 16, None)]
                        for a in range(4) for c in range(4)])
        if do_p and j == 0:
          steps = [norm_const_steps(r) for r in range(0, QR, 8)]
          seq = []
          for n in range(len(steps) + 3):
            if n < len(steps):
              seq.append([(steps[n][0], anchor(sb, SL_DUMMY), 10, None)])
            if n >= 3:
              seq.append([(steps[n - 3][1], lambda v: None, 1, None)])
          lists.append(seq)
        if do_o and j > 4:
          lists.append(outs[(9 * (j - 5)) // 4:(9 * (j - 4)) // 4])
        _run(_merge(s_rounds, v_rounds), _merge_groups(*lists), QR, span=SPAN)

    if _DEV is not None:
      lax.fori_loop(2, NB, lambda m, c: iteration(m, *_DEV), None)
      return
    iteration(0, True, False, False)

    @pl.when(b > 0)
    def _():
      for cp in o_copies(b - 1, NB - 2, 1) + o_copies(b - 1, NB - 1, 0, last=True):
        cp.wait()
    iteration(1, True, True, False)

    def steady(m, carry):
      @pl.when(m >= 4)
      def _():
        for cp in o_copies(b, m - 4, m % 2):
          cp.wait()
      iteration(m, True, True, True)
      for cp in o_copies(b, m - 2, m % 2):
        cp.start()
      return carry
    lax.fori_loop(2, NB, steady, None)
    for cp in o_copies(b, NB - 4, NB % 2):
      cp.wait()
    iteration(NB, False, True, True)
    for cp in o_copies(b, NB - 2, NB % 2):
      cp.start()
    for cp in o_copies(b, NB - 3, (NB + 1) % 2):
      cp.wait()
    iteration(NB + 1, False, False, True)
    for cp in o_copies(b, NB - 1, (NB + 1) % 2, last=True):
      cp.start()

  def batch(b, carry):
    z = lax.shift_right_logical(b, 8)
    for cp in x_copies(b, 0):
      cp.wait()
    st = pltpu.VMEM((D + 8, D), F32)
    if _DEV is None or _DEV == 'p1': pl.run_scoped(functools.partial(phase1, b, z), sq, sq, st, st, st, st, st, st, st)

    @pl.when(b + 1 < nbatch)
    def _():
      for cp in x_copies(b + 1, 0) + x_copies(b + 1, 1):
        cp.start()
    blocks = lambda n: pltpu.VMEM((n, QR, 128), F32)
    if _DEV == 'p1':
      @pl.when(z > 0)
      def _():
        stage[0, 0, :, 0:128] = ae[z, 0:QR, :] + ke[z, z, 0:16, :].sum() + ve[z, z, 0:16, :].sum()
    if _DEV != 'p1': pl.run_scoped(
        functools.partial(phase2, b, z),
        blocks(SL_DUMMY + 1), blocks(PR_DUMMY + 1), blocks(PR_DUMMY + 1), blocks(PR_DUMMY + 1),
        pltpu.VMEM((4 * 49 + 1, QR, 128), BF16), pltpu.VMEM((4 * 49, QR, 128), BF16),
        pltpu.VMEM((49, QR, 128), BF16), blocks(50), blocks(50), blocks(17),
        pltpu.VMEM((17, QR + 2 * GOFF, 128), F32))
    return carry

  lax.fori_loop(0, nbatch, batch, None)
  if _DEV is not None:
    for cp in o_copies(0, 0, 0):
      cp.start(); cp.wait()
    return
  for cp in o_copies(nbatch - 1, NB - 2, 1) + o_copies(nbatch - 1, NB - 1, 0, last=True):
    cp.wait()


@jax.jit
def pallas_standalone__conformer_family_branchformer__speech_kernel(
    x: jax.Array,
    w_q: jax.Array,
    w_k: jax.Array,
    w_v: jax.Array,
    w_ao: jax.Array,
    w_up: jax.Array,
    dw: jax.Array,
    w_dn: jax.Array,
    w_merge: jax.Array,
):
  nbatch = x.shape[0]
  assert x.shape[1:] == (T, D) and dw.shape == (KW, D)
  any_spec = pl.BlockSpec(memory_space=pl.ANY)
  return pl.pallas_call(
      _kernel,
      out_shape=jax.ShapeDtypeStruct(x.shape, x.dtype),
      in_specs=[any_spec] * 9,
      out_specs=any_spec,
      scratch_shapes=[
          pltpu.VMEM((nbatch, XROWS + 16, D), BF16),
          pltpu.VMEM((NB + 1, AE_ROWS, 128), BF16),
          pltpu.VMEM((NT + 1, 49, 128, 128), BF16),
          pltpu.VMEM((NT + 1, 49, 128, 128), BF16),
          pltpu.VMEM((4, GOFF + XROWS + 32, 128), F32),
          pltpu.VMEM((4, KW, 8, 128), F32),
          pltpu.VMEM((D, D), BF16),
          pltpu.VMEM((D, D), BF16),
          pltpu.VMEM((D, 2 * D), BF16),
          pltpu.VMEM((2, 4, QR, D), BF16),
          pltpu.SemaphoreType.DMA((8,)),
          pltpu.SemaphoreType.DMA((8 * nbatch,)),
          pltpu.SemaphoreType.DMA((8,)),
      ],
      compiler_params=pltpu.CompilerParams(vmem_limit_bytes=126 * 1024 * 1024),
      name="branchformer",
  )(x, w_q, w_k, w_v, w_ao, w_up, dw, w_dn, w_merge)
```

```python
import functools

import jax
import jax.numpy as jnp
from jax import lax
import jax.experimental.pallas as pl
import jax.experimental.pallas.tpu as pltpu

F32, BF16, U32 = jnp.float32, jnp.bfloat16, jnp.uint32

T, D, KW = 4000, 512, 31
QS = 1008
QR = 144
NB = 7
NT = 8
XROWS = 3 * QS + NT * 128
AE_ROWS = 7104
GOFF = 16
EPS = 1e-5
LOG2E = 1.4426950408889634

_DEV = None
_SCOPES = False


def _scope(name):
  import contextlib
  return jax.named_scope(name) if _SCOPES else contextlib.nullcontext()


CONV_N = 3
CONV_SH = 2
SPAN = 0.99
CW, CCH, OCH = 2.8, 0, 1
PC = (50, 32, 32)
CC = 30
ENC_COST = (35, 25, 25)
P1SPAN = 0.98

SL_U = 16 * NT
SL_M = SL_U + 16
SL_L = SL_M + 4
SL_OFF = SL_L + 4
SL_DUMMY = SL_OFF + 4
PR_RAW = 31
PR_LEFT = 36
PR_DUMMY = 40


def _enc_a(a11, a12, a21, a22):
  return [a11 + a22, a21 + a22, a11, a22, a11 + a12, a21 - a11, a12 - a22]


def _enc_b(b11, b12, b21, b22):
  return [b11 + b22, b11, b12 - b22, b21 - b11, b22, b11 + b12, b21 + b22]


_A_TERMS = ([(0, 0, 1), (1, 1, 1)], [(1, 0, 1), (1, 1, 1)], [(0, 0, 1)], [(1, 1, 1)],
            [(0, 0, 1), (0, 1, 1)], [(1, 0, 1), (0, 0, -1)], [(0, 1, 1), (1, 1, -1)])
_B_TERMS = ([(0, 0, 1), (1, 1, 1)], [(0, 0, 1)], [(0, 1, 1), (1, 1, -1)],
            [(1, 0, 1), (0, 0, -1)], [(1, 1, 1)], [(0, 0, 1), (0, 1, 1)],
            [(1, 0, 1), (1, 1, 1)])
_USE = ([((0, 0), 1), ((1, 1), 1)], [((1, 0), 1), ((1, 1), -1)],
        [((0, 1), 1), ((1, 1), 1)], [((0, 0), 1), ((1, 0), 1)],
        [((0, 0), -1), ((0, 1), 1)], [((1, 1), 1)], [((0, 0), 1)])


def _lin(terms):
  acc = None
  for v, s in terms:
    if acc is None:
      acc = v
    else:
      acc = acc + v if s > 0 else acc - v
  return acc


def _encode2(blk, terms, enc, store, outer=range(7)):
  for o in outer:
    q = [[_lin([(blk[2 * r + i][2 * c + j], s) for r, c, s in terms[o]])
          for j in range(2)] for i in range(2)]
    for p, v in enumerate(enc(q[0][0], q[0][1], q[1][0], q[1][1])):
      store(7 * o + p, v)
  return v


_A_STEPS = (([(0, 0), (1, 1)], (2, 0, 3)), ([(1, 0)], (1, 5)), ([(0, 1)], (4, 6)))
_B_STEPS = (([(0, 0), (1, 1)], (1, 0, 4)), ([(0, 1)], (2, 5)), ([(1, 0)], (3, 6)))


def _encode_steps(fetch, steps, terms, enc, store):
  blk = [[None] * 4 for _ in range(4)]

  def step(quads, outer):
    for r, c in quads:
      for i in range(2):
        for j in range(2):
          blk[2 * r + i][2 * c + j] = fetch(2 * r + i, 2 * c + j)
    return _encode2(blk, terms, enc, store, outer)
  return [functools.partial(step, *st) for st in steps]


def _decode_outer(inner):
  c = {}
  for o in range(7):
    quad = inner(o)
    for qi, v in quad.items():
      for qo, s in _USE[o]:
        key = (2 * qo[0] + qi[0], 2 * qo[1] + qi[1])
        if key not in c:
          c[key] = v
        else:
          c[key] = c[key] + v if s > 0 else c[key] - v
  return c


def _decode_inner(m):
  return {(0, 0): m[0] + m[3] - m[4] + m[6], (0, 1): m[2] + m[4],
          (1, 0): m[1] + m[3], (1, 1): m[0] - m[1] + m[2] + m[5]}


def _layernorm(v):
  mean = jnp.sum(v, axis=-1, keepdims=True) * (1.0 / D)
  d = v - mean
  var = jnp.sum(d * d, axis=-1, keepdims=True) * (1.0 / D)
  return d * lax.rsqrt(var + EPS)


def _gelu(v):
  c1 = 0.7978845608028654
  inner = v * (c1 + (c1 * 0.044715) * (v * v))
  h = 0.5 * v
  return h + h * jnp.tanh(inner)


def _dot(a, b):
  return jnp.dot(a, b, preferred_element_type=F32)


def _dot_nt(a, b):
  return lax.dot_general(a, b, (((1,), (1,)), ((), ())), preferred_element_type=F32)


def _ldb(ref, *idx):
  return pltpu.bitcast(ref.bitcast(U32)[idx], BF16)


def _run(rounds, pieces, rows, span=1.0):
  if not rounds:
    for fn, _, _, _ in pieces:
      fn()
    return
  per = rows // 8
  total = len(rounds) * per * span / max(1, sum(p[2] for p in pieces))
  j, done, last = 0, 0, {}
  for k, rnd in enumerate(rounds):
    res = rnd()
    while j < len(pieces) and int(done * total) < (k + 1) * per:
      r = (int(done * total) - k * per) * 8
      fn, anchor, cost, chain = pieces[j]
      pin = res[r:r + 8, 0:128]
      anchor(pin + last[chain] if chain in last else pin)
      tok = fn()
      if chain is not None:
        last[chain] = tok[0:8, 0:128]
      j += 1
      done += cost


def _merge(*lists, cost=lambda v: 1):
  keyed = []
  for n, l in enumerate(lists):
    total, done = max(1, sum(cost(v) for v in l)), 0
    for i, v in enumerate(l):
      keyed.append(((done + 0.5 * cost(v)) / total, n, i, v))
      done += cost(v)
  return [v for _, _, _, v in sorted(keyed, key=lambda e: e[:3])]


def _merge_groups(*lists):
  merged = _merge(*lists, cost=lambda g: sum(p[2] for p in g))
  return [p for g in merged for p in g]


def _kernel(x_hbm, wq_hbm, wk_hbm, wv_hbm, wao_hbm, wup_hbm, dw_hbm, wdn_hbm, wm_hbm,
            o_hbm, xb, ae, ke, ve, gb, dwb, wqk, wvom, wup, wdm, taps, stage, xa0, xa1, xf,
            w_sem, x_sem, o_sem):
  nbatch = x_hbm.shape[0]
  xas = (xa0, xa1)

  def x_copies(b, part):
    cps = []
    if _DEV is not None: return cps
    for a in range(4):
      lo, hi = (0, 256) if part == 0 else (256, min(QS, T - a * QS))
      rows = pl.ds(a * QS + lo, hi - lo)
      cps.append(pltpu.make_async_copy(
          x_hbm.at[b, rows, :], xb.at[b, rows, :], x_sem.at[b * 8 + part * 4 + a]))
    return cps

  def o_copies(b, j, par, last=False):
    cps = []
    for a in range(4):
      n = min(QR, T - (a * QS + (NB - 1) * QR)) if last else QR
      cps.append(pltpu.make_async_copy(
          stage.at[par, a, pl.ds(0, n), :],
          o_hbm.at[b, pl.ds(a * QS + j * QR, n), :], o_sem.at[par * 4 + a]))
    return cps

  def block_fetch(src, g):
    def fetch(i, j):
      return src[i * 128 + 16 * g:i * 128 + 16 * g + 16, j * 128:j * 128 + 128].astype(F32)
    return fetch

  def encode_b(src, dst, t, g):
    def store(p, v):
      dst[t, p, 16 * g:16 * g + 16, :] = v.astype(BF16)
    return _encode_steps(block_fetch(src, g), _B_STEPS, _B_TERMS, _enc_b, store)

  def stage_anchor(ref, z):
    def put(v):
      if ref.dtype == BF16:
        ref[pl.ds(pl.multiple_of(D + z, 16), 16), 0:128] = jnp.concatenate(
            [v, v], axis=0).astype(BF16)
      else:
        ref[pl.ds(pl.multiple_of(D + z, 8), 8), 0:128] = v
    return put

  def norm_pieces(b, z, t, par):
    def norm(a, g):
      r0 = pl.multiple_of(a * QS + 16 * g + 128 * t, 16)
      xa = _layernorm(xb[b, pl.ds(r0, 16), :].astype(F32))
      rows = slice(a * 128 + 16 * g, a * 128 + 16 * g + 16)
      xas[par][rows, :] = xa.astype(BF16)
      xf[rows, :] = xa

    def encode_a(g):
      pos = 128 * t + 16 * g
      j, r = pos // QR, pos % QR

      def store(p, v):
        ae[j, pl.ds(pl.multiple_of(p * QR + r, 16), 16), :] = v.astype(BF16)
      return _encode_steps(block_fetch(xf, g), _A_STEPS, _A_TERMS, _enc_a, store)

    def xanchor(v):
      xb[0, pl.ds(pl.multiple_of(XROWS + z, 16), 16), 0:128] = jnp.concatenate(
          [v, v], axis=0).astype(BF16)
    norms = [[(functools.partial(norm, a, g), xanchor, 30, None)]
             for g in range(8) for a in range(4)]
    encs = [[(fn, stage_anchor(xf, z), c, 1) for fn, c in zip(encode_a(g), ENC_COST)]
            for g in range(8)]
    return norms, encs

  def enc_pieces(src, dst, t, z):
    return [[(fn, stage_anchor(src, z), c, 1)
             for fn, c in zip(encode_b(src, dst, t, g), ENC_COST)] for g in range(8)]

  def col_rounds(dst, fn, post=lambda v: v):
    def rnd(cols):
      res = fn(cols)
      dst[0:D, cols] = post(res)
      return res
    return [functools.partial(rnd, slice(n * 128, n * 128 + 128)) for n in range(4)]

  def weights(wq, wk, wv, wao, wdn, wm, t1):
    srcs = (wq_hbm, wk_hbm, wv_hbm, wao_hbm, wm_hbm, wdn_hbm, wup_hbm, dw_hbm)
    dsts = (wq, wk, wv, wao, wm, wdn, wup.at[0:D, :], taps)
    cps = [pltpu.make_async_copy(s, d, w_sem.at[i])
           for i, (s, d) in enumerate(zip(srcs, dsts))]

    def hand_over(done, nxt):
      for cp in done:
        cp.wait()
      for cp in nxt:
        cp.start()
    hand_over([], cps[0:2])
    for b in range(nbatch):
      xb[b, T:XROWS, :] = jnp.zeros((XROWS - T, D), BF16)
    for c in range(4):
      gb[c, 0:GOFF, :] = jnp.zeros((GOFF, 128), F32)
    to_bf16 = lambda v: v.astype(BF16)
    hand_over(cps[0:2], cps[2:4])
    _run(col_rounds(wqk, lambda c: _dot_nt(wq[...], wk[c, :]),
                    lambda v: to_bf16(v * (LOG2E * D ** -0.5))), [], D)
    hand_over(cps[2:4], cps[4:5])
    _run(col_rounds(t1, lambda c: _dot(wv[...], wao[:, c]), to_bf16), [], D)
    hand_over(cps[4:5], cps[5:6] + x_copies(0, 0))
    _run(col_rounds(wvom, lambda c: _dot(t1[...], wm[0:D, c]), to_bf16), [], D)
    hand_over(cps[5:6] + x_copies(0, 0), cps[6:8])
    norms, encs = norm_pieces(0, None, 0, 0)
    _run(col_rounds(wdm, lambda c: _dot(wdn[...], wm[D:2 * D, c])),
         [(fn, lambda v: None, c, None) for fn, _, c, _ in _merge_groups(norms)], D, span=0.7)
    _run([], _merge_groups(encs), D)
    hand_over(cps[6:8], x_copies(0, 1))

  sq = pltpu.VMEM((D, D), BF16)
  if _DEV is None:
   with _scope('w'):
    pl.run_scoped(weights, sq, sq, sq, sq, sq, pltpu.VMEM((2 * D, D), BF16), sq)

  def phase1(b, z, ks, vs, gs):
    def gate_piece(t, a, g):
      v = _layernorm(_gelu(gs[a * 128 + 8 * g:a * 128 + 8 * g + 8, :]))
      rows = pl.ds(pl.multiple_of(GOFF + a * QS + 8 * g + 128 * t, 8), 8)
      for c in range(4):
        gb[c, rows, :] = v[:, c * 128:c * 128 + 128]

    def spread_taps():
      rows = taps[...].astype(F32)
      for c in range(4):
        for k in range(KW):
          dwb[c, k] = jnp.broadcast_to(rows[k:k + 1, c * 128:c * 128 + 128], (8, 128))

    def step(t, par, first, last):
      xa = xas[par]
      gates = [[(functools.partial(gate_piece, t, a, g), stage_anchor(gs, z), 30, None)]
               for a in range(4) for g in range(16)]
      keys = enc_pieces(ks, ke, t, z)
      if first:
        prev_k = enc_pieces(wup, ke, NT, z) + [[(spread_taps, lambda v: None, 40, None)]]
        prev_v = enc_pieces(wdm, ve, NT, z)
      else:
        prev_k = enc_pieces(ks, ke, t - 1, z)[4:]
        prev_v = enc_pieces(vs, ve, t - 1, z)
      norms, encs = ([], []) if last else norm_pieces(b, z, t + 1, 1 - par)
      _run(col_rounds(gs, lambda c: _dot(xa[...], wup[0:D, D + c.start:D + c.stop])),
           _merge_groups(prev_k + prev_v[:6], norms[:24]), D, span=P1SPAN)
      _run(col_rounds(ks, lambda c: _dot_nt(wqk[...], xa[c, :])),
           _merge_groups(prev_v[6:] + encs[:4], norms[24:] + gates[:32]), D, span=P1SPAN)
      _run(col_rounds(vs, lambda c: _dot(xa[...], wvom[:, c])),
           _merge_groups((keys if last else encs[4:] + keys[:4]), gates[32:]), D,
           span=P1SPAN - 0.1)

    step(0, 0, True, False)
    for cp in x_copies(b, 1):
      cp.wait()

    def pair(i, carry):
      step(2 * i + 1, 1, False, False)
      step(2 * i + 2, 0, False, False)
      return carry
    lax.fori_loop(0, (NT - 2) // 2, pair, None)
    step(NT - 1, 1, False, True)
    _run([], _merge_groups(enc_pieces(vs, ve, NT - 1, z)), D)

  def phase2(b, z, sb, pr0, pr1, pr2, pe_a, pe_b, pe_z, oacc, ofin, cv, gw):
    prs = [(pr0, pr1)[t % 2] for t in range(NT)] + [pr2]
    left = [PR_LEFT + t // 2 for t in range(NT)] + [PR_LEFT]

    def anchor(ref, slot):
      def put(v):
        ref[slot + z, 0:8, :] = v
      return put

    def s_prod(m, t, o, p):
      lhs = _ldb(ae, m, pl.ds((7 * o + p) * (QR // 2), QR // 2), slice(None))
      return _dot(lhs, _ldb(ke, t, 7 * o + p))

    raw = [(o, p) for o in (5, 6) for p in (0, 2, 4)]

    def s_round_a(m, t, o):
      m2, m4, m6, m7 = [s_prod(m, t, o, p) for p in (1, 3, 5, 6)]
      pr = prs[t]
      pr[3 * o] = m4 + m7
      pr[3 * o + 1] = m2 + m4
      pr[3 * o + 2] = m6 - m2
      return m7

    def s_round_b(m, t, o):
      m1, m3, m5 = [s_prod(m, t, o, p) for p in (0, 2, 4)]
      extra = s_prod(m, t, *raw[o])
      pr = prs[t]
      pr[21 + 2 * o] = m1 - m5
      pr[22 + 2 * o] = m3 + m5
      pr[PR_RAW + o] = extra
      return extra

    def z_prod(p):
      res = _dot(_ldb(pe_z, p), _ldb(ve, NT, p))
      oacc[p] = res
      return res

    def left_round(m, tiles, z_too):
      res = None
      for t in tiles:
        res = s_prod(m, t, *raw[5])
        prs[t][left[t]] = res
      if z_too:
        res = z_prod(48)
      return res

    def z_round(k):
      return [z_prod(p) for p in range(4 * k, 4 * k + 4)][-1]

    def pv_round(second, p):
      pe = pe_b if second else pe_a
      lhs = jnp.concatenate([_ldb(pe, 49 * i + p) for i in range(4)], axis=1)
      rhs = jnp.concatenate([_ldb(ve, 4 * second + i, p) for i in range(4)], axis=0)
      res = _dot(lhs, rhs)
      (ofin if second else oacc)[p] = oacc[p] + res
      return res

    def comb_piece(t, r, i):
      rows = slice(r, r + 8)
      pr = prs[t]

      def inner(o):
        if o < 5:
          xx, yy = pr[21 + 2 * o, rows, :], pr[22 + 2 * o, rows, :]
        else:
          slots = [PR_RAW + n if n < 5 else left[t]
                   for n in range(3 * (o - 5), 3 * (o - 5) + 3)]
          m1, m3, m5 = [pr[n, rows, :] for n in slots]
          xx, yy = m1 - m5, m3 + m5
        if i == 0:
          return {(0, 0): xx + pr[3 * o, rows, :], (0, 1): yy}
        return {(1, 0): pr[3 * o + 1, rows, :], (1, 1): xx + yy + pr[3 * o + 2, rows, :]}
      c = _decode_outer(inner)
      if t == NT:
        for (a, k), v in c.items():
          sb[SL_U + 4 * a + k, rows, :] = _gelu(v)
        return c[(i, 0)]
      if t == NT - 1:
        lane = lax.broadcasted_iota(jnp.int32, (8, 128), 1)
      for a in (i, i + 2):
        vs = [c[(a, k)] for k in range(4)]
        if t == NT - 1:
          vs = [jnp.where(lane < min(QS, T - k * QS) - 128 * t, v, -jnp.inf)
                for k, v in enumerate(vs)]
        for k in range(4):
          sb[16 * t + 4 * a + k, rows, :] = vs[k]
        mx = jnp.maximum(jnp.maximum(vs[0], vs[1]), jnp.maximum(vs[2], vs[3]))
        if t > 0:
          m_old = sb[SL_M + a, rows, :]
          mx = jnp.maximum(mx, m_old)
        e = [jnp.exp2(v - mx) for v in vs]
        ls = (e[0] + e[1]) + (e[2] + e[3])
        if t > 0:
          ls = ls + sb[SL_L + a, rows, :] * jnp.exp2(m_old - mx)
        sb[SL_M + a, rows, :] = mx
        sb[SL_L + a, rows, :] = ls
      return mx

    def norm_const_steps(r):
      rows = slice(r, r + 8)
      off = []

      def compute():
        for a in range(4):
          mx = sb[SL_M + a, rows, :]
          m_row = jnp.max(mx, axis=-1, keepdims=True)
          l_row = jnp.sum(sb[SL_L + a, rows, :] * jnp.exp2(mx - m_row), axis=-1, keepdims=True)
          off.append(jnp.broadcast_to(m_row + jnp.log2(l_row), (8, 128)))

      def store():
        for a in range(4):
          sb[SL_OFF + a, rows, :] = off[a]
      return compute, store

    def prep_steps(t, r):
      rows = slice(r, r + 16)

      def fetch(a, k):
        if t < NT:
          return jnp.exp2(sb[16 * t + 4 * a + k, rows, :] - sb[SL_OFF + a, rows, :])
        return sb[SL_U + 4 * a + k, rows, :] * cv[4 * a + k, rows, :]

      def store(p, v):
        if t == NT:
          pe_z[p, rows, :] = v.astype(BF16)
        else:
          (pe_a if t < 4 else pe_b)[49 * (t % 4) + p, rows, :] = v.astype(BF16)
      return _encode_steps(fetch, _A_STEPS, _A_TERMS, _enc_a, store)

    def window_piece(j, a, c):
      v = gb[c, pl.ds(pl.multiple_of(a * QS + j * QR, 16), QR + 2 * GOFF), :]
      gw[4 * a + c] = v
      return v

    def conv_steps(a, c, r):
      base = GOFF - KW // 2 + r
      acc = [None] * CONV_N

      def step(shifts):
        for sh in shifts:
          taps = range(sh, KW, 8)
          g = [gw[4 * a + c, pl.ds(base + sh + 8 * i, 8), :] for i in range(CONV_N + len(taps) - 1)]
          for q, k in enumerate(taps):
            w = dwb[c, k]
            for h in range(CONV_N):
              v = g[h + q] * w
              acc[h] = v if acc[h] is None else acc[h] + v
        if shifts[-1] == 7:
          for h in range(CONV_N):
            cv[4 * a + c, r + 8 * h:r + 8 * h + 8, :] = acc[h]
        return acc[-1]
      return [functools.partial(step, range(s0, s0 + CONV_SH)) for s0 in range(0, 8, CONV_SH)]

    def out_piece(j, par, r):
      halves = []
      for h in range(2):
        rows = slice(r + 8 * h, r + 8 * h + 8)
        halves.append(_decode_outer(
            lambda o: _decode_inner([ofin[7 * o + p, rows, :] for p in range(7)])))
      for a in range(4):
        xr = pl.ds(pl.multiple_of(a * QS + r + j * QR, 16), 16)
        for k in range(4):
          cols = slice(k * 128, k * 128 + 128)
          y = jnp.concatenate([halves[0][(a, k)], halves[1][(a, k)]], axis=0)
          y = xb[b, xr, cols].astype(F32) + y
          stage[par, a, r:r + 16, cols] = y.astype(BF16)
      return y

    def ganchor(v):
      gb[3, pl.ds(pl.multiple_of(GOFF + XROWS + z, 8), 8), :] = v

    def zanchor(v):
      anchor(sb, SL_DUMMY)(v)
      anchor(cv, 16)(v)

    def iteration(m, do_s, do_p, do_o):
      part = functools.partial
      par = m % 2
      convs = [[(fn, anchor(gw, 16), CONV_N * CONV_SH * CW, CCH) for fn in conv_steps(a, c, r)]
               for a in range(4) for c in range(4) for r in range(0, QR, 8 * CONV_N)]
      outs = [[(part(out_piece, m - 2, par, r), anchor(ofin, 49), 90, OCH)]
              for r in range(0, QR, 16)]
      if do_o and not do_p:
        norms, encs = norm_pieces(jnp.minimum(b + 1, nbatch - 1), z, 0, 0)
        next_rows = norms + encs
      first, zk = [[] for _ in range(5)], 0
      for j, (n_b, n_z) in enumerate(((12, 0), (9, 3), (9, 3), (10, 3), (9, 3))):
        p0 = sum((0, 12, 9, 9, 10)[:j + 1])
        bs = [part(pv_round, 1, p) for p in range(p0, p0 + n_b)] if do_o else []
        zs = [part(z_round, k) for k in range(zk, zk + n_z)] if do_p else []
        zk += n_z
        first[j] = bs + zs if j == 4 else _merge(bs, zs)
      pv_split = [0, 12, 24, 36, 49]
      for j in range(NT + 1):
        s_rounds, v_rounds = [], []
        if do_s:
          if j in (0, 4):
            s_rounds.append(part(left_round, m, range(j, j + 4), False))
          for o in range(7):
            s_rounds.append(part(s_round_a, m, j, o))
            if o < 5:
              s_rounds.append(part(s_round_b, m, j, o))
        if j < 5:
          v_rounds = first[j]
        if j == 4 and (do_s or do_p):
          v_rounds.append(part(left_round, m, [NT] if do_s else [], do_p))
        if do_p and j > 4:
          if j == 5:
            anchor(oacc, 49)(jnp.zeros((8, 128), F32))
            pe_a[4 * 49 + z, 0:16, :] = jnp.zeros((16, 128), BF16)
          v_rounds = [part(pv_round, 0, p) for p in range(pv_split[j - 5], pv_split[j - 4])]
        t = j - 1 if j > 0 else NT
        main = []
        for r in range(0, QR, 8):
          combs = [[(part(comb_piece, t, r, i), anchor(prs[t], PR_DUMMY), CC if j else 36, 1)]
                   for i in range(2)]
          if j > 0:
            if do_p and r % 16 == 0:
              main.append([(fn, anchor(sb, SL_DUMMY), c, 1)
                           for fn, c in zip(prep_steps(t, r), PC)])
            if do_s:
              main += combs
          elif do_p:
            main += combs
            if r % 16 == 8:
              main.append([(fn, zanchor, c, 1)
                           for fn, c in zip(prep_steps(t, r - 8), (40, 28, 28))])
        lists = [main]
        if do_s and do_p and not do_o:
          if j > 4:
            n = len(convs) // 4
            lists.append(convs[(j - 5) * n:(j - 4) * n])
        elif do_s and j > 0:
          n = len(convs) // NT
          lists.append(convs[(j - 1) * n:j * n])
        if do_s and j == 0:
          lists.append([[(part(window_piece, m, a, c), ganchor, 16, None)]
                        for a in range(4) for c in range(4)])
        if do_p and j == 0:
          steps = [norm_const_steps(r) for r in range(0, QR, 8)]
          seq = []
          for n in range(len(steps) + 3):
            if n < len(steps):
              seq.append([(steps[n][0], anchor(sb, SL_DUMMY), 10, None)])
            if n >= 3:
              seq.append([(steps[n - 3][1], lambda v: None, 1, None)])
          lists.append(seq)
        if do_o and not do_p and j < 5:
          lists.append(next_rows[8 * j:8 * j + 8])
        if do_o and j > 4:
          lists.append(outs[(9 * (j - 5)) // 4:(9 * (j - 4)) // 4])
        _run(_merge(s_rounds, v_rounds), _merge_groups(*lists), QR, span=SPAN)

    if _DEV is not None:
      lax.fori_loop(2, NB, lambda m, c: iteration(m, *_DEV), None)
      return
    with _scope('it0'):
      iteration(0, True, False, False)

    @pl.when(b > 0)
    def _():
      for cp in o_copies(b - 1, NB - 2, 1) + o_copies(b - 1, NB - 1, 0, last=True):
        cp.wait()
    with _scope('it1'):
      iteration(1, True, True, False)

    def steady(m, carry):
      @pl.when(m >= 4)
      def _():
        for cp in o_copies(b, m - 4, m % 2):
          cp.wait()
      with _scope('steady'):
        iteration(m, True, True, True)
      for cp in o_copies(b, m - 2, m % 2):
        cp.start()
      return carry
    lax.fori_loop(2, NB, steady, None)
    for cp in o_copies(b, NB - 4, NB % 2):
      cp.wait()
    with _scope('it7'):
      iteration(NB, False, True, True)
    for cp in o_copies(b, NB - 2, NB % 2):
      cp.start()
    for cp in o_copies(b, NB - 3, (NB + 1) % 2):
      cp.wait()

    @pl.when(b + 1 < nbatch)
    def _():
      for cp in x_copies(b + 1, 0):
        cp.wait()
    with _scope('it8'):
      iteration(NB + 1, False, False, True)
    for cp in o_copies(b, NB - 1, (NB + 1) % 2, last=True):
      cp.start()

  def batch(b, carry):
    z = lax.shift_right_logical(b, 8)
    st = pltpu.VMEM((D + 8, D), F32)

    if _DEV is None or _DEV == 'p1':
     with _scope('p1'):
      pl.run_scoped(functools.partial(phase1, b, z), st, st, st)

    @pl.when(b + 1 < nbatch)
    def _():
      for cp in x_copies(b + 1, 0) + x_copies(b + 1, 1):
        cp.start()
    blocks = lambda n: pltpu.VMEM((n, QR, 128), F32)
    if _DEV == 'p1':
      @pl.when(z > 0)
      def _():
        stage[0, 0, :, 0:128] = gb[z, 0:QR, :].astype(BF16) + ae[z, 0:QR, :] + ke[z, z, 0:16, :].sum() + ve[z, z, 0:16, :].sum()
    if _DEV != 'p1': pl.run_scoped(
        functools.partial(phase2, b, z),
        blocks(SL_DUMMY + 1), blocks(PR_DUMMY + 1), blocks(PR_DUMMY + 1), blocks(PR_DUMMY + 1),
        pltpu.VMEM((4 * 49 + 1, QR, 128), BF16), pltpu.VMEM((4 * 49, QR, 128), BF16),
        pltpu.VMEM((49, QR, 128), BF16), blocks(50), blocks(50), blocks(17),
        pltpu.VMEM((17, QR + 2 * GOFF, 128), F32))
    return carry

  lax.fori_loop(0, nbatch, batch, None)
  if _DEV is not None:
    for cp in o_copies(0, 0, 0):
      cp.start(); cp.wait()
    return
  for cp in o_copies(nbatch - 1, NB - 2, 1) + o_copies(nbatch - 1, NB - 1, 0, last=True):
    cp.wait()


@jax.jit
def pallas_standalone__conformer_family_branchformer__speech_kernel(
    x: jax.Array,
    w_q: jax.Array,
    w_k: jax.Array,
    w_v: jax.Array,
    w_ao: jax.Array,
    w_up: jax.Array,
    dw: jax.Array,
    w_dn: jax.Array,
    w_merge: jax.Array,
):
  nbatch = x.shape[0]
  assert x.shape[1:] == (T, D) and dw.shape == (KW, D)
  any_spec = pl.BlockSpec(memory_space=pl.ANY)
  return pl.pallas_call(
      _kernel,
      out_shape=jax.ShapeDtypeStruct(x.shape, x.dtype),
      in_specs=[any_spec] * 9,
      out_specs=any_spec,
      scratch_shapes=[
          pltpu.VMEM((nbatch, XROWS + 16, D), BF16),
          pltpu.VMEM((NB + 1, AE_ROWS, 128), BF16),
          pltpu.VMEM((NT + 1, 49, 128, 128), BF16),
          pltpu.VMEM((NT + 1, 49, 128, 128), BF16),
          pltpu.VMEM((4, GOFF + XROWS + 32, 128), F32),
          pltpu.VMEM((4, KW, 8, 128), F32),
          pltpu.VMEM((D, D), BF16),
          pltpu.VMEM((D, D), BF16),
          pltpu.VMEM((D + 16, 2 * D), BF16),
          pltpu.VMEM((D + 8, D), F32),
          pltpu.VMEM((KW, D), BF16),
          pltpu.VMEM((2, 4, QR, D), BF16),
          pltpu.VMEM((D, D), BF16),
          pltpu.VMEM((D, D), BF16),
          pltpu.VMEM((D + 8, D), F32),
          pltpu.SemaphoreType.DMA((8,)),
          pltpu.SemaphoreType.DMA((8 * nbatch,)),
          pltpu.SemaphoreType.DMA((8,)),
      ],
      compiler_params=pltpu.CompilerParams(vmem_limit_bytes=126 * 1024 * 1024),
      name="branchformer",
  )(x, w_q, w_k, w_v, w_ao, w_up, dw, w_dn, w_merge)
```

```python
import functools

import jax
import jax.numpy as jnp
from jax import lax
import jax.experimental.pallas as pl
import jax.experimental.pallas.tpu as pltpu

F32, BF16, U32 = jnp.float32, jnp.bfloat16, jnp.uint32

T, D, KW = 4000, 512, 31
QS = 1008
QR = 144
NB = 7
NT = 8
XROWS = 3 * QS + NT * 128
AE_ROWS = 7104
GOFF = 16
EPS = 1e-5
LOG2E = 1.4426950408889634

_DEV = None
_SCOPES = False
_FLAGS = None


def _scope(name):
  import contextlib
  return jax.named_scope(name) if _SCOPES else contextlib.nullcontext()


CONV_N = 3
CONV_SH = 2
SPAN = 0.99
CW, CCH, OCH = 2.8, 0, 1
PC = (50, 32, 32)
CC = 30
FPAD, WPAD, GPAD = 8, 0, 0
NC, NCH, UC = 10, 0, 50
ZC = (30, 24, 24)
P1UNROLL = False
P1S3 = 0.75
WSTART = ([0, 1], [2], [3], [4], [5], [])
ENC_COST = (35, 25, 25)
P1SPAN = 0.85

SL_U = 16 * NT
SL_M = SL_U + 16
SL_L = SL_M + 4
SL_OFF = SL_L + 4
SL_DUMMY = SL_OFF + 4
PR_RAW = 31
PR_LEFT = 36
PR_DUMMY = 40


def _enc_a(a11, a12, a21, a22):
  return [a11 + a22, a21 + a22, a11, a22, a11 + a12, a21 - a11, a12 - a22]


def _enc_b(b11, b12, b21, b22):
  return [b11 + b22, b11, b12 - b22, b21 - b11, b22, b11 + b12, b21 + b22]


_A_TERMS = ([(0, 0, 1), (1, 1, 1)], [(1, 0, 1), (1, 1, 1)], [(0, 0, 1)], [(1, 1, 1)],
            [(0, 0, 1), (0, 1, 1)], [(1, 0, 1), (0, 0, -1)], [(0, 1, 1), (1, 1, -1)])
_B_TERMS = ([(0, 0, 1), (1, 1, 1)], [(0, 0, 1)], [(0, 1, 1), (1, 1, -1)],
            [(1, 0, 1), (0, 0, -1)], [(1, 1, 1)], [(0, 0, 1), (0, 1, 1)],
            [(1, 0, 1), (1, 1, 1)])
_USE = ([((0, 0), 1), ((1, 1), 1)], [((1, 0), 1), ((1, 1), -1)],
        [((0, 1), 1), ((1, 1), 1)], [((0, 0), 1), ((1, 0), 1)],
        [((0, 0), -1), ((0, 1), 1)], [((1, 1), 1)], [((0, 0), 1)])


def _lin(terms):
  acc = None
  for v, s in terms:
    if acc is None:
      acc = v
    else:
      acc = acc + v if s > 0 else acc - v
  return acc


def _encode2(blk, terms, enc, store, outer=range(7)):
  for o in outer:
    q = [[_lin([(blk[2 * r + i][2 * c + j], s) for r, c, s in terms[o]])
          for j in range(2)] for i in range(2)]
    for p, v in enumerate(enc(q[0][0], q[0][1], q[1][0], q[1][1])):
      store(7 * o + p, v)
  return v


_A_STEPS = (([(0, 0), (1, 1)], (2, 0, 3)), ([(1, 0)], (1, 5)), ([(0, 1)], (4, 6)))
_B_STEPS = (([(0, 0), (1, 1)], (1, 0, 4)), ([(0, 1)], (2, 5)), ([(1, 0)], (3, 6)))


def _encode_steps(fetch, steps, terms, enc, store):
  blk = [[None] * 4 for _ in range(4)]

  def step(quads, outer):
    for r, c in quads:
      for i in range(2):
        for j in range(2):
          blk[2 * r + i][2 * c + j] = fetch(2 * r + i, 2 * c + j)
    return _encode2(blk, terms, enc, store, outer)
  return [functools.partial(step, *st) for st in steps]


def _decode_outer(inner):
  c = {}
  for o in range(7):
    quad = inner(o)
    for qi, v in quad.items():
      for qo, s in _USE[o]:
        key = (2 * qo[0] + qi[0], 2 * qo[1] + qi[1])
        if key not in c:
          c[key] = v
        else:
          c[key] = c[key] + v if s > 0 else c[key] - v
  return c


def _decode_inner(m):
  return {(0, 0): m[0] + m[3] - m[4] + m[6], (0, 1): m[2] + m[4],
          (1, 0): m[1] + m[3], (1, 1): m[0] - m[1] + m[2] + m[5]}


def _layernorm(v):
  mean = jnp.sum(v, axis=-1, keepdims=True) * (1.0 / D)
  d = v - mean
  var = jnp.sum(d * d, axis=-1, keepdims=True) * (1.0 / D)
  return d * lax.rsqrt(var + EPS)


def _gelu(v):
  c1 = 0.7978845608028654
  inner = v * (c1 + (c1 * 0.044715) * (v * v))
  h = 0.5 * v
  return h + h * jnp.tanh(inner)


def _dot(a, b):
  return jnp.dot(a, b, preferred_element_type=F32)


def _dot_nt(a, b):
  return lax.dot_general(a, b, (((1,), (1,)), ((), ())), preferred_element_type=F32)


def _aligned(i, n):
  return i if isinstance(i, int) else pl.multiple_of(i, n)


def _ldb(ref, *idx):
  return pltpu.bitcast(ref.bitcast(U32)[idx], BF16)


def _run(rounds, pieces, rows, span=1.0):
  if not rounds:
    for fn, _, _, _ in pieces:
      fn()
    return
  per = rows // 8
  total = len(rounds) * per * span / max(1, sum(p[2] for p in pieces))
  j, done, last = 0, 0, {}
  for k, rnd in enumerate(rounds):
    res = rnd()
    while j < len(pieces) and int(done * total) < (k + 1) * per:
      r = (int(done * total) - k * per) * 8
      fn, anchor, cost, chain = pieces[j]
      pin = res[r:r + 8, 0:128]
      anchor(pin + last[chain] if chain in last else pin)
      tok = fn()
      if chain is not None:
        last[chain] = tok[0:8, 0:128]
      j += 1
      done += cost


def _merge(*lists, cost=lambda v: 1):
  keyed = []
  for n, l in enumerate(lists):
    total, done = max(1, sum(cost(v) for v in l)), 0
    for i, v in enumerate(l):
      keyed.append(((done + 0.5 * cost(v)) / total, n, i, v))
      done += cost(v)
  return [v for _, _, _, v in sorted(keyed, key=lambda e: e[:3])]


def _merge_groups(*lists):
  merged = _merge(*lists, cost=lambda g: sum(p[2] for p in g))
  return [p for g in merged for p in g]


def _kernel(x_hbm, wq_hbm, wk_hbm, wv_hbm, wao_hbm, wup_hbm, dw_hbm, wdn_hbm, wm_hbm,
            o_hbm, xb, ae, ke, ve, gb, dwb, wqk, wvom, wup, wdm, taps, stage, xa0, xa1, xf,
            w_sem, x_sem, o_sem):
  nbatch = x_hbm.shape[0]
  xas = (xa0, xa1)

  def x_copies(b, part):
    cps = []
    if _DEV is not None and _DEV != 'w': return cps
    for a in range(4):
      lo, hi = (0, 256) if part == 0 else (256, min(QS, T - a * QS))
      rows = pl.ds(a * QS + lo, hi - lo)
      cps.append(pltpu.make_async_copy(
          x_hbm.at[b, rows, :], xb.at[b, rows, :], x_sem.at[b * 8 + part * 4 + a]))
    return cps

  def o_copies(b, j, par, last=False):
    cps = []
    for a in range(4):
      n = min(QR, T - (a * QS + (NB - 1) * QR)) if last else QR
      cps.append(pltpu.make_async_copy(
          stage.at[par, a, pl.ds(0, n), :],
          o_hbm.at[b, pl.ds(a * QS + j * QR, n), :], o_sem.at[par * 4 + a]))
    return cps

  def block_fetch(src, g):
    def fetch(i, j):
      return src[i * 128 + 16 * g:i * 128 + 16 * g + 16, j * 128:j * 128 + 128].astype(F32)
    return fetch

  def encode_b(src, dst, t, g):
    def store(p, v):
      dst[t, p, 16 * g:16 * g + 16, :] = v.astype(BF16)
    return _encode_steps(block_fetch(src, g), _B_STEPS, _B_TERMS, _enc_b, store)

  def stage_anchor(ref, z):
    def put(v):
      if ref.dtype == BF16:
        ref[pl.ds(pl.multiple_of(D + z, 16), 16), 0:128] = jnp.concatenate(
            [v, v], axis=0).astype(BF16)
      else:
        ref[pl.ds(pl.multiple_of(D + z, 8), 8), 0:128] = v
    return put

  def norm_pieces(b, z, t, par):
    def norm(a, g):
      r0 = _aligned(a * QS + 16 * g + 128 * t, 16)
      xa = _layernorm(xb[b, pl.ds(r0, 16), :].astype(F32))
      rows = slice(a * 128 + 16 * g, a * 128 + 16 * g + 16)
      xas[par][rows, :] = xa.astype(BF16)
      xf[rows, :] = xa

    def encode_a(g):
      pos = 128 * t + 16 * g
      j, r = pos // QR, pos % QR

      def store(p, v):
        ae[j, pl.ds(_aligned(p * QR + r, 16), 16), :] = v.astype(BF16)
      return _encode_steps(block_fetch(xf, g), _A_STEPS, _A_TERMS, _enc_a, store)

    def xanchor(v):
      xb[0, pl.ds(pl.multiple_of(XROWS + z, 16), 16), 0:128] = jnp.concatenate(
          [v, v], axis=0).astype(BF16)
    norms = [[(functools.partial(norm, a, g), xanchor, 30, None)]
             for g in range(8) for a in range(4)]
    encs = [[(fn, stage_anchor(xf, z), c, 1) for fn, c in zip(encode_a(g), ENC_COST)]
            for g in range(8)]
    return norms, encs

  def enc_pieces(src, dst, t, z):
    return [[(fn, stage_anchor(src, z), c, 1)
             for fn, c in zip(encode_b(src, dst, t, g), ENC_COST)] for g in range(8)]

  def col_rounds(dst, fn, post=lambda v: v):
    def rnd(cols):
      res = fn(cols)
      dst[0:D, cols] = post(res)
      return res
    return [functools.partial(rnd, slice(n * 128, n * 128 + 128)) for n in range(4)]

  def weights(wq, wk, wv, wao, wdn, wm, t1):
    srcs = (wq_hbm, wk_hbm, wv_hbm, wao_hbm, wm_hbm, wdn_hbm, wup_hbm, dw_hbm)
    dsts = (wq, wk, wv, wao, wm, wdn, wup.at[0:D, :], taps)
    cps = [pltpu.make_async_copy(s, d, w_sem.at[i])
           for i, (s, d) in enumerate(zip(srcs, dsts))]

    groups = [cps[0:2], cps[2:4], cps[4:5], cps[5:6] + x_copies(0, 0), cps[6:8], x_copies(0, 1)]

    def need(i):
      for cp in groups[i]:
        cp.wait()
      for g in WSTART[i + 1]:
        for cp in groups[g]:
          cp.start()
    for g in WSTART[0]:
      for cp in groups[g]:
        cp.start()
    for b in range(nbatch):
      xb[b, T:XROWS, :] = jnp.zeros((XROWS - T, D), BF16)
    for c in range(4):
      gb[c, 0:GOFF, :] = jnp.zeros((GOFF, 128), F32)
    to_bf16 = lambda v: v.astype(BF16)
    need(0)
    _run(col_rounds(wqk, lambda c: _dot_nt(wq[...], wk[c, :]),
                    lambda v: to_bf16(v * (LOG2E * D ** -0.5))), [], D)
    need(1)
    _run(col_rounds(t1, lambda c: _dot(wv[...], wao[:, c]), to_bf16), [], D)
    need(2)
    _run(col_rounds(wvom, lambda c: _dot(t1[...], wm[0:D, c]), to_bf16), [], D)
    need(3)
    norms, encs = norm_pieces(0, None, 0, 0)
    _run(col_rounds(wdm, lambda c: _dot(wdn[...], wm[D:2 * D, c])),
         [(fn, lambda v: None, c, None) for fn, _, c, _ in _merge_groups(norms)], D, span=0.7)
    _run([], _merge_groups(encs), D)
    need(4)

  sq = pltpu.VMEM((D, D), BF16)
  if _DEV is None or _DEV == 'w':
   with _scope('w'):
    pl.run_scoped(weights, sq, sq, sq, sq, sq, pltpu.VMEM((2 * D, D), BF16), sq)

  def phase1(b, z, ks, vs, gs):
    def gate_piece(t, a, g):
      v = _layernorm(_gelu(gs[a * 128 + 8 * g:a * 128 + 8 * g + 8, :]))
      rows = pl.ds(_aligned(GOFF + a * QS + 8 * g + 128 * t, 8), 8)
      for c in range(4):
        gb[c, rows, :] = v[:, c * 128:c * 128 + 128]

    def spread_taps():
      rows = taps[...].astype(F32)
      for c in range(4):
        for k in range(KW):
          dwb[c, k] = jnp.broadcast_to(rows[k:k + 1, c * 128:c * 128 + 128], (8, 128))

    def step(t, par, first, last):
      xa = xas[par]
      gates = [[(functools.partial(gate_piece, t, a, g), stage_anchor(gs, z), 30, None)]
               for a in range(4) for g in range(16)]
      keys = enc_pieces(ks, ke, t, z)
      if first:
        prev_k = enc_pieces(wup, ke, NT, z) + [[(spread_taps, lambda v: None, 40, None)]]
        prev_v = enc_pieces(wdm, ve, NT, z)
      else:
        prev_k = enc_pieces(ks, ke, t - 1, z)[4:]
        prev_v = enc_pieces(vs, ve, t - 1, z)
      norms, encs = ([], []) if last else norm_pieces(b, z, t + 1, 1 - par)
      _run(col_rounds(gs, lambda c: _dot(xa[...], wup[0:D, D + c.start:D + c.stop])),
           _merge_groups(prev_k + prev_v[:6], norms[:24]), D, span=P1SPAN)
      _run(col_rounds(ks, lambda c: _dot_nt(wqk[...], xa[c, :])),
           _merge_groups(prev_v[6:] + encs[:4], norms[24:] + gates[:32]), D, span=P1SPAN)
      _run(col_rounds(vs, lambda c: _dot(xa[...], wvom[:, c])),
           _merge_groups((keys if last else encs[4:] + keys[:4]), gates[32:]), D,
           span=P1S3)

    step(0, 0, True, False)
    for cp in x_copies(b, 1):
      cp.wait()

    def pair(i, carry):
      step(2 * i + 1, 1, False, False)
      step(2 * i + 2, 0, False, False)
      return carry
    if P1UNROLL:
      for i in range((NT - 2) // 2):
        pair(i, None)
    else:
      lax.fori_loop(0, (NT - 2) // 2, pair, None)
    step(NT - 1, 1, False, True)
    _run([], _merge_groups(enc_pieces(vs, ve, NT - 1, z)), D)

  def phase2(b, z, sb, pr0, pr1, pr2, pe_a, pe_b, pe_z, oacc, ofin, cv, gw):
    prs = [(pr0, pr1)[t % 2] for t in range(NT)] + [pr2]
    left = [PR_LEFT + t // 2 for t in range(NT)] + [PR_LEFT]

    def anchor(ref, slot):
      def put(v):
        ref[slot + z, 0:8, :] = v
      return put

    def s_prod(m, t, o, p):
      lhs = _ldb(ae, m, pl.ds((7 * o + p) * (QR // 2), QR // 2), slice(None))
      return _dot(lhs, _ldb(ke, t, 7 * o + p, slice(0, 64), slice(None)))

    raw = [(o, p) for o in (5, 6) for p in (0, 2, 4)]

    def s_round_a(m, t, o):
      m2, m4, m6, m7 = [s_prod(m, t, o, p) for p in (1, 3, 5, 6)]
      pr = prs[t]
      pr[3 * o, 0:QR, :] = m4 + m7
      pr[3 * o + 1, 0:QR, :] = m2 + m4
      pr[3 * o + 2, 0:QR, :] = m6 - m2
      return m7

    def s_round_b(m, t, o):
      m1, m3, m5 = [s_prod(m, t, o, p) for p in (0, 2, 4)]
      extra = s_prod(m, t, *raw[o])
      pr = prs[t]
      pr[21 + 2 * o, 0:QR, :] = m1 - m5
      pr[22 + 2 * o, 0:QR, :] = m3 + m5
      pr[PR_RAW + o, 0:QR, :] = extra
      return extra

    def z_prod(p):
      res = _dot(_ldb(pe_z, p), _ldb(ve, NT, p, slice(0, 64), slice(None)))
      oacc[p, 0:QR, :] = res
      return res

    def left_round(m, tiles, z_too):
      res = None
      for t in tiles:
        res = s_prod(m, t, *raw[5])
        prs[t][left[t], 0:QR, :] = res
      if z_too:
        res = z_prod(48)
      return res

    def z_round(k):
      return [z_prod(p) for p in range(4 * k, 4 * k + 4)][-1]

    def pv_round(second, p):
      pe = pe_b if second else pe_a
      lhs = jnp.concatenate([_ldb(pe, 49 * i + p) for i in range(4)], axis=1)
      rhs = jnp.concatenate([_ldb(ve, 4 * second + i, p, slice(0, 64), slice(None)) for i in range(4)], axis=0)
      res = _dot(lhs, rhs)
      (ofin if second else oacc)[p, 0:QR, :] = oacc[p, 0:QR, :] + res
      return res

    def comb_piece(t, r, i):
      rows = slice(r, r + 8)
      pr = prs[t]

      def inner(o):
        if o < 5:
          xx, yy = pr[21 + 2 * o, rows, :], pr[22 + 2 * o, rows, :]
        else:
          slots = [PR_RAW + n if n < 5 else left[t]
                   for n in range(3 * (o - 5), 3 * (o - 5) + 3)]
          m1, m3, m5 = [pr[n, rows, :] for n in slots]
          xx, yy = m1 - m5, m3 + m5
        if i == 0:
          return {(0, 0): xx + pr[3 * o, rows, :], (0, 1): yy}
        return {(1, 0): pr[3 * o + 1, rows, :], (1, 1): xx + yy + pr[3 * o + 2, rows, :]}
      c = _decode_outer(inner)
      if t == NT:
        for (a, k), v in c.items():
          v = _gelu(v)
          sb[SL_U + 4 * a + k, rows, :] = v
        return v
      if t == NT - 1:
        lane = lax.broadcasted_iota(jnp.int32, (8, 128), 1)
      for a in (i, i + 2):
        vs = [c[(a, k)] for k in range(4)]
        if t == NT - 1:
          vs = [jnp.where(lane < min(QS, T - k * QS) - 128 * t, v, -jnp.inf)
                for k, v in enumerate(vs)]
        for k in range(4):
          sb[16 * t + 4 * a + k, rows, :] = vs[k]
        mx = jnp.maximum(jnp.maximum(vs[0], vs[1]), jnp.maximum(vs[2], vs[3]))
        if t > 0:
          m_old = sb[SL_M + a, rows, :]
          mx = jnp.maximum(mx, m_old)
        e = [jnp.exp2(v - mx) for v in vs]
        ls = (e[0] + e[1]) + (e[2] + e[3])
        if t > 0:
          ls = ls + sb[SL_L + a, rows, :] * jnp.exp2(m_old - mx)
        sb[SL_M + a, rows, :] = mx
        sb[SL_L + a, rows, :] = ls
      return mx

    def norm_const_steps(r):
      rows = slice(r, r + 8)
      off = []

      def compute():
        for a in range(4):
          mx = sb[SL_M + a, rows, :]
          m_row = jnp.max(mx, axis=-1, keepdims=True)
          l_row = jnp.sum(sb[SL_L + a, rows, :] * jnp.exp2(mx - m_row), axis=-1, keepdims=True)
          off.append(jnp.broadcast_to(m_row + jnp.log2(l_row), (8, 128)))
        return off[-1]

      def store():
        for a in range(4):
          sb[SL_OFF + a, rows, :] = off[a]
      return compute, store

    def prep_steps(t, r):
      rows = slice(r, r + 16)

      def fetch(a, k):
        if t < NT:
          return jnp.exp2(sb[16 * t + 4 * a + k, rows, :] - sb[SL_OFF + a, rows, :])
        return sb[SL_U + 4 * a + k, rows, :] * cv[4 * a + k, rows, :]

      def store(p, v):
        if t == NT:
          pe_z[p, rows, :] = v.astype(BF16)
        else:
          (pe_a if t < 4 else pe_b)[49 * (t % 4) + p, rows, :] = v.astype(BF16)
      return _encode_steps(fetch, _A_STEPS, _A_TERMS, _enc_a, store)

    def window_piece(j, a, r):
      for c in range(4):
        v = gb[c, pl.ds(_aligned(a * QS + r + j * QR, 16), 16), :]
        gw[4 * a + c, r:r + 16, :] = v
      return v

    def conv_steps(a, c, r):
      base = GOFF - KW // 2 + r
      acc = [None] * CONV_N

      def step(shifts):
        for sh in shifts:
          taps = range(sh, KW, 8)
          g = [gw[4 * a + c, pl.ds(base + sh + 8 * i, 8), :] for i in range(CONV_N + len(taps) - 1)]
          for q, k in enumerate(taps):
            w = dwb[c, k]
            for h in range(CONV_N):
              v = g[h + q] * w
              acc[h] = v if acc[h] is None else acc[h] + v
        if shifts[-1] == 7:
          for h in range(CONV_N):
            cv[4 * a + c, r + 8 * h:r + 8 * h + 8, :] = acc[h]
        return acc[-1]
      return [functools.partial(step, range(s0, s0 + CONV_SH)) for s0 in range(0, 8, CONV_SH)]

    def out_piece(j, par, r):
      halves = []
      for h in range(2):
        rows = slice(r + 8 * h, r + 8 * h + 8)
        halves.append(_decode_outer(
            lambda o: _decode_inner([ofin[7 * o + p, rows, :] for p in range(7)])))
      for a in range(4):
        xr = pl.ds(_aligned(a * QS + r + j * QR, 16), 16)
        for k in range(4):
          cols = slice(k * 128, k * 128 + 128)
          y = jnp.concatenate([halves[0][(a, k)], halves[1][(a, k)]], axis=0)
          y = xb[b, xr, cols].astype(F32) + y
          stage[par, a, r:r + 16, cols] = y.astype(BF16)
      return y

    def ganchor(v):
      gb[3, pl.ds(pl.multiple_of(GOFF + XROWS + z, 8), 8), :] = v

    def zanchor(v):
      anchor(sb, SL_DUMMY)(v)
      anchor(cv, 16)(v)

    def iteration(m, do_s, do_p, do_o):
      part = functools.partial
      par = m % 2
      convs = [[(fn, anchor(gw, 16), CONV_N * CONV_SH * CW, CCH) for fn in conv_steps(a, c, r)]
               for a in range(4) for c in range(4) for r in range(0, QR, 8 * CONV_N)]
      outs = [[(part(out_piece, m - 2, par, r), anchor(ofin, 49), 90, OCH)]
              for r in range(0, QR, 16)]
      if do_o and not do_p:
        norms, encs = norm_pieces(jnp.minimum(b + 1, nbatch - 1), z, 0, 0)
        next_rows = norms + encs
      first, zk = [[] for _ in range(5)], 0
      for j, (n_b, n_z) in enumerate(((12, 0), (9, 3), (9, 3), (10, 3), (9, 3))):
        p0 = sum((0, 12, 9, 9, 10)[:j + 1])
        bs = [part(pv_round, 1, p) for p in range(p0, p0 + n_b)] if do_o else []
        zs = [part(z_round, k) for k in range(zk, zk + n_z)] if do_p else []
        zk += n_z
        first[j] = bs + zs if j == 4 else _merge(bs, zs)
      pv_split = [0, 12, 24, 36, 49]
      for j in range(NT + 1):
        s_rounds, v_rounds = [], []
        if do_s:
          if j in (0, 4):
            s_rounds.append(part(left_round, m, range(j, j + 4), False))
          for o in range(7):
            s_rounds.append(part(s_round_a, m, j, o))
            if o < 5:
              s_rounds.append(part(s_round_b, m, j, o))
        if j < 5:
          v_rounds = first[j]
        if j == 4 and (do_s or do_p):
          v_rounds.append(part(left_round, m, [NT] if do_s else [], do_p))
        if do_p and j > 4:
          if j == 5:
            anchor(oacc, 49)(jnp.zeros((8, 128), F32))
            pe_a[4 * 49 + z, 0:16, :] = jnp.zeros((16, 128), BF16)
          v_rounds = [part(pv_round, 0, p) for p in range(pv_split[j - 5], pv_split[j - 4])]
        t = j - 1 if j > 0 else NT
        main = []
        for r in range(0, QR, 8):
          combs = [[(part(comb_piece, t, r, i), anchor(prs[t], PR_DUMMY), CC if j else UC, 1)]
                   for i in range(2)]
          if j > 0:
            if do_p and r % 16 == 0:
              main.append([(fn, anchor(sb, SL_DUMMY), c, 1)
                           for fn, c in zip(prep_steps(t, r), PC)])
            if do_s:
              main += combs
          elif do_p:
            main += combs
            if r % 16 == 8:
              main.append([(fn, zanchor, c, 1)
                           for fn, c in zip(prep_steps(t, r - 8), ZC)])
        lists = [main]
        if do_s and do_p and not do_o:
          if j > 4:
            n = len(convs) // 4
            lists.append(convs[(j - 5) * n:(j - 4) * n])
        elif do_s and j > 0:
          n = len(convs) // NT
          lists.append(convs[(j - 1) * n:j * n])
        if do_s and j == 0:
          lists.append([[(part(window_piece, m, a, r), ganchor, 6, 0)]
                        for a in range(4) for r in range(0, QR + 2 * GOFF, 16)])
        if do_p and j == 0:
          steps = [norm_const_steps(r) for r in range(0, QR, 8)]
          seq = []
          for n in range(len(steps) + 3):
            if n < len(steps):
              seq.append([(steps[n][0], anchor(sb, SL_DUMMY), NC, 10 + n % NCH if NCH else None)])
            if n >= 3:
              seq.append([(steps[n - 3][1], lambda v: None, 1, None)])
          lists.append(seq)
        if do_o and not do_p and j < 5:
          lists.append(next_rows[8 * j:8 * j + 8])
        if do_o and j > 4:
          lists.append(outs[(9 * (j - 5)) // 4:(9 * (j - 4)) // 4])
        _run(_merge(s_rounds, v_rounds), _merge_groups(*lists), QR, span=SPAN)

    if _DEV is not None:
      lax.fori_loop(2, NB, lambda m, c: iteration(m, *_DEV), None)
      return
    with _scope('it0'):
      iteration(0, True, False, False)

    @pl.when(b > 0)
    def _():
      for cp in o_copies(b - 1, NB - 2, 1) + o_copies(b - 1, NB - 1, 0, last=True):
        cp.wait()
    with _scope('it1'):
      iteration(1, True, True, False)

    def steady(m, carry):
      @pl.when(m >= 4)
      def _():
        for cp in o_copies(b, m - 4, m % 2):
          cp.wait()
      with _scope('steady'):
        iteration(m, True, True, True)
      for cp in o_copies(b, m - 2, m % 2):
        cp.start()
      return carry
    lax.fori_loop(2, NB, steady, None)
    for cp in o_copies(b, NB - 4, NB % 2):
      cp.wait()
    with _scope('it7'):
      iteration(NB, False, True, True)
    for cp in o_copies(b, NB - 2, NB % 2):
      cp.start()
    for cp in o_copies(b, NB - 3, (NB + 1) % 2):
      cp.wait()

    @pl.when(b + 1 < nbatch)
    def _():
      for cp in x_copies(b + 1, 0):
        cp.wait()
    with _scope('it8'):
      iteration(NB + 1, False, False, True)
    for cp in o_copies(b, NB - 1, (NB + 1) % 2, last=True):
      cp.start()

  def batch(b, carry):
    z = lax.shift_right_logical(b, 8)
    st = pltpu.VMEM((D + 8, D), F32)

    if _DEV is None or _DEV == 'p1':
     with _scope('p1'):
      pl.run_scoped(functools.partial(phase1, b, z), st, st, st)

    @pl.when(b + 1 < nbatch)
    def _():
      for cp in x_copies(b + 1, 0) + x_copies(b + 1, 1):
        cp.start()
    blocks = lambda n: pltpu.VMEM((n, QR + FPAD, 128), F32)
    if _DEV == 'p1':
      @pl.when(z > 0)
      def _():
        stage[0, 0, :, 0:128] = gb[z, 0:QR, :].astype(BF16) + ae[z, 0:QR, :] + ke[z, z, 0:16, :].sum() + ve[z, z, 0:16, :].sum()
    if _DEV != 'p1': pl.run_scoped(
        functools.partial(phase2, b, z),
        blocks(SL_DUMMY + 1), blocks(PR_DUMMY + 1), blocks(PR_DUMMY + 1), blocks(PR_DUMMY + 1),
        pltpu.VMEM((4 * 49 + 1, QR, 128), BF16), pltpu.VMEM((4 * 49, QR, 128), BF16),
        pltpu.VMEM((49, QR, 128), BF16), blocks(50), blocks(50), blocks(17),
        pltpu.VMEM((17, QR + 2 * GOFF + GPAD, 128), F32))
    return carry

  if _DEV == 'w':
    for cp in x_copies(0, 1): cp.wait()
    stage[0, 0, :, 0:128] = ae[0, 0:QR, :] + wdm[0:QR, 0:128].astype(BF16) + wqk[0:QR, 0:128] + wvom[0:QR, 0:128] + xa0[0:QR, 0:128]
  else: lax.fori_loop(0, nbatch, batch, None)
  if _DEV is not None:
    for cp in o_copies(0, 0, 0):
      cp.start(); cp.wait()
    return
  for cp in o_copies(nbatch - 1, NB - 2, 1) + o_copies(nbatch - 1, NB - 1, 0, last=True):
    cp.wait()


@jax.jit
def pallas_standalone__conformer_family_branchformer__speech_kernel(
    x: jax.Array,
    w_q: jax.Array,
    w_k: jax.Array,
    w_v: jax.Array,
    w_ao: jax.Array,
    w_up: jax.Array,
    dw: jax.Array,
    w_dn: jax.Array,
    w_merge: jax.Array,
):
  nbatch = x.shape[0]
  assert x.shape[1:] == (T, D) and dw.shape == (KW, D)
  any_spec = pl.BlockSpec(memory_space=pl.ANY)
  return pl.pallas_call(
      _kernel,
      out_shape=jax.ShapeDtypeStruct(x.shape, x.dtype),
      in_specs=[any_spec] * 9,
      out_specs=any_spec,
      scratch_shapes=[
          pltpu.VMEM((nbatch, XROWS + 16, D), BF16),
          pltpu.VMEM((NB + 1, AE_ROWS, 128), BF16),
          pltpu.VMEM((NT + 1, 49, 128 + WPAD, 128), BF16),
          pltpu.VMEM((NT + 1, 49, 128 + WPAD, 128), BF16),
          pltpu.VMEM((4, GOFF + XROWS + 32, 128), F32),
          pltpu.VMEM((4, KW, 8, 128), F32),
          pltpu.VMEM((D, D), BF16),
          pltpu.VMEM((D, D), BF16),
          pltpu.VMEM((D + 16, 2 * D), BF16),
          pltpu.VMEM((D + 8, D), F32),
          pltpu.VMEM((KW, D), BF16),
          pltpu.VMEM((2, 4, QR, D), BF16),
          pltpu.VMEM((D, D), BF16),
          pltpu.VMEM((D, D), BF16),
          pltpu.VMEM((D + 8, D), F32),
          pltpu.SemaphoreType.DMA((8,)),
          pltpu.SemaphoreType.DMA((8 * nbatch,)),
          pltpu.SemaphoreType.DMA((8,)),
      ],
      compiler_params=pltpu.CompilerParams(vmem_limit_bytes=126 * 1024 * 1024, flags=_FLAGS),
      name="branchformer",
  )(x, w_q, w_k, w_v, w_ao, w_up, dw, w_dn, w_merge)
```

```python
import functools

import jax
import jax.numpy as jnp
from jax import lax
import jax.experimental.pallas as pl
import jax.experimental.pallas.tpu as pltpu

F32, BF16, U32 = jnp.float32, jnp.bfloat16, jnp.uint32

T, D, KW = 4000, 512, 31
QS = 1008
QR = 144
NB = 7
NT = 8
XROWS = 3 * QS + NT * 128
AE_ROWS = 7104
GOFF = 16
EPS = 1e-5
LOG2E = 1.4426950408889634

_DEV = None
_SCOPES = False
_FLAGS = None


def _scope(name):
  import contextlib
  return jax.named_scope(name) if _SCOPES else contextlib.nullcontext()


CONV_N = 3
CONV_SH = 2
SPAN = 0.99
CW, CCH, OCH = 2.8, 0, 1
PC = (50, 32, 32)
CC = 30
NRM_CH, GATE_CH = 0, 0
NE2, NV1, NK3, NN1, NG2 = 0, 4, 2, 32, 32
CV0 = (0, 1, 1, 1, 1, 1, 1, 1, 1)
CV1 = (0, 0, 0, 0, 0, 1, 1, 1, 1)
CVS = (0, 1, 1, 1, 1, 1, 1, 1, 1)
FPAD, WPAD, GPAD = 8, 0, 0
NC, NCH, UC = 10, 0, 50
ZC = (30, 24, 24)
P1UNROLL = False
P1S3 = 0.85
WSTART = ([0, 1], [2], [3], [4], [5], [])
ENC_COST = (35, 25, 25)
P1SPAN = 0.95

SL_U = 16 * NT
SL_M = SL_U + 16
SL_L = SL_M + 4
SL_OFF = SL_L + 4
SL_DUMMY = SL_OFF + 4
PR_RAW = 31
PR_LEFT = 36
PR_DUMMY = 40


def _enc_a(a11, a12, a21, a22):
  return [a11 + a22, a21 + a22, a11, a22, a11 + a12, a21 - a11, a12 - a22]


def _enc_b(b11, b12, b21, b22):
  return [b11 + b22, b11, b12 - b22, b21 - b11, b22, b11 + b12, b21 + b22]


_A_TERMS = ([(0, 0, 1), (1, 1, 1)], [(1, 0, 1), (1, 1, 1)], [(0, 0, 1)], [(1, 1, 1)],
            [(0, 0, 1), (0, 1, 1)], [(1, 0, 1), (0, 0, -1)], [(0, 1, 1), (1, 1, -1)])
_B_TERMS = ([(0, 0, 1), (1, 1, 1)], [(0, 0, 1)], [(0, 1, 1), (1, 1, -1)],
            [(1, 0, 1), (0, 0, -1)], [(1, 1, 1)], [(0, 0, 1), (0, 1, 1)],
            [(1, 0, 1), (1, 1, 1)])
_USE = ([((0, 0), 1), ((1, 1), 1)], [((1, 0), 1), ((1, 1), -1)],
        [((0, 1), 1), ((1, 1), 1)], [((0, 0), 1), ((1, 0), 1)],
        [((0, 0), -1), ((0, 1), 1)], [((1, 1), 1)], [((0, 0), 1)])


def _lin(terms):
  acc = None
  for v, s in terms:
    if acc is None:
      acc = v
    else:
      acc = acc + v if s > 0 else acc - v
  return acc


def _encode2(blk, terms, enc, store, outer=range(7)):
  for o in outer:
    q = [[_lin([(blk[2 * r + i][2 * c + j], s) for r, c, s in terms[o]])
          for j in range(2)] for i in range(2)]
    for p, v in enumerate(enc(q[0][0], q[0][1], q[1][0], q[1][1])):
      store(7 * o + p, v)
  return v


_A_STEPS = (([(0, 0), (1, 1)], (2, 0, 3)), ([(1, 0)], (1, 5)), ([(0, 1)], (4, 6)))
_B_STEPS = (([(0, 0), (1, 1)], (1, 0, 4)), ([(0, 1)], (2, 5)), ([(1, 0)], (3, 6)))


def _encode_steps(fetch, steps, terms, enc, store):
  blk = [[None] * 4 for _ in range(4)]

  def step(quads, outer):
    for r, c in quads:
      for i in range(2):
        for j in range(2):
          blk[2 * r + i][2 * c + j] = fetch(2 * r + i, 2 * c + j)
    return _encode2(blk, terms, enc, store, outer)
  return [functools.partial(step, *st) for st in steps]


def _decode_outer(inner):
  c = {}
  for o in range(7):
    quad = inner(o)
    for qi, v in quad.items():
      for qo, s in _USE[o]:
        key = (2 * qo[0] + qi[0], 2 * qo[1] + qi[1])
        if key not in c:
          c[key] = v
        else:
          c[key] = c[key] + v if s > 0 else c[key] - v
  return c


def _decode_inner(m):
  return {(0, 0): m[0] + m[3] - m[4] + m[6], (0, 1): m[2] + m[4],
          (1, 0): m[1] + m[3], (1, 1): m[0] - m[1] + m[2] + m[5]}


def _layernorm(v):
  mean = jnp.sum(v, axis=-1, keepdims=True) * (1.0 / D)
  d = v - mean
  var = jnp.sum(d * d, axis=-1, keepdims=True) * (1.0 / D)
  return d * lax.rsqrt(var + EPS)


def _gelu(v):
  c1 = 0.7978845608028654
  inner = v * (c1 + (c1 * 0.044715) * (v * v))
  h = 0.5 * v
  return h + h * jnp.tanh(inner)


def _dot(a, b):
  return jnp.dot(a, b, preferred_element_type=F32)


def _dot_nt(a, b):
  return lax.dot_general(a, b, (((1,), (1,)), ((), ())), preferred_element_type=F32)


def _aligned(i, n):
  return i if isinstance(i, int) else pl.multiple_of(i, n)


def _ldb(ref, *idx):
  return pltpu.bitcast(ref.bitcast(U32)[idx], BF16)


def _run(rounds, pieces, rows, span=1.0):
  if not rounds:
    for fn, _, _, _ in pieces:
      fn()
    return
  per = rows // 8
  total = len(rounds) * per * span / max(1, sum(p[2] for p in pieces))
  j, done, last = 0, 0, {}
  for k, rnd in enumerate(rounds):
    res = rnd()
    while j < len(pieces) and int(done * total) < (k + 1) * per:
      r = (int(done * total) - k * per) * 8
      fn, anchor, cost, chain = pieces[j]
      pin = res[r:r + 8, 0:128]
      anchor(pin + last[chain] if chain in last else pin)
      tok = fn()
      if chain is not None:
        last[chain] = tok[0:8, 0:128]
      j += 1
      done += cost


def _merge(*lists, cost=lambda v: 1):
  keyed = []
  for n, l in enumerate(lists):
    total, done = max(1, sum(cost(v) for v in l)), 0
    for i, v in enumerate(l):
      keyed.append(((done + 0.5 * cost(v)) / total, n, i, v))
      done += cost(v)
  return [v for _, _, _, v in sorted(keyed, key=lambda e: e[:3])]


def _merge_groups(*lists):
  merged = _merge(*lists, cost=lambda g: sum(p[2] for p in g))
  return [p for g in merged for p in g]


def _kernel(x_hbm, wq_hbm, wk_hbm, wv_hbm, wao_hbm, wup_hbm, dw_hbm, wdn_hbm, wm_hbm,
            o_hbm, xb, ae, ke, ve, gb, dwb, wqk, wvom, wup, wdm, taps, stage, xa0, xa1, xf,
            w_sem, x_sem, o_sem):
  nbatch = x_hbm.shape[0]
  xas = (xa0, xa1)

  def x_copies(b, part):
    cps = []
    if _DEV is not None and _DEV != 'w': return cps
    for a in range(4):
      lo, hi = (0, 256) if part == 0 else (256, min(QS, T - a * QS))
      rows = pl.ds(a * QS + lo, hi - lo)
      cps.append(pltpu.make_async_copy(
          x_hbm.at[b, rows, :], xb.at[b, rows, :], x_sem.at[b * 8 + part * 4 + a]))
    return cps

  def o_copies(b, j, par, last=False):
    cps = []
    for a in range(4):
      n = min(QR, T - (a * QS + (NB - 1) * QR)) if last else QR
      cps.append(pltpu.make_async_copy(
          stage.at[par, a, pl.ds(0, n), :],
          o_hbm.at[b, pl.ds(a * QS + j * QR, n), :], o_sem.at[par * 4 + a]))
    return cps

  def block_fetch(src, g):
    def fetch(i, j):
      return src[i * 128 + 16 * g:i * 128 + 16 * g + 16, j * 128:j * 128 + 128].astype(F32)
    return fetch

  def encode_b(src, dst, t, g):
    def store(p, v):
      dst[t, p, 16 * g:16 * g + 16, :] = v.astype(BF16)
    return _encode_steps(block_fetch(src, g), _B_STEPS, _B_TERMS, _enc_b, store)

  def stage_anchor(ref, z):
    def put(v):
      if ref.dtype == BF16:
        ref[pl.ds(pl.multiple_of(D + z, 16), 16), 0:128] = jnp.concatenate(
            [v, v], axis=0).astype(BF16)
      else:
        ref[pl.ds(pl.multiple_of(D + z, 8), 8), 0:128] = v
    return put

  def norm_pieces(b, z, t, par):
    def norm(a, g):
      r0 = _aligned(a * QS + 16 * g + 128 * t, 16)
      xa = _layernorm(xb[b, pl.ds(r0, 16), :].astype(F32))
      rows = slice(a * 128 + 16 * g, a * 128 + 16 * g + 16)
      for k in range(4):
        xas[par][k, rows, :] = xa[:, k * 128:k * 128 + 128].astype(BF16)
      xf[rows, :] = xa
      return xa

    def encode_a(g):
      pos = 128 * t + 16 * g
      j, r = pos // QR, pos % QR

      view = ae.at[j, pl.ds(_aligned(r, 16), 48 * QR + 16), :]

      def store(p, v):
        view[p * QR:p * QR + 16, :] = v.astype(BF16)
      return _encode_steps(block_fetch(xf, g), _A_STEPS, _A_TERMS, _enc_a, store)

    def xanchor(v):
      xb[0, pl.ds(pl.multiple_of(XROWS + z, 16), 16), 0:128] = jnp.concatenate(
          [v, v], axis=0).astype(BF16)
    norms = [[(functools.partial(norm, a, g), xanchor, 30, 20 + a % NRM_CH if NRM_CH else None)]
             for g in range(8) for a in range(4)]
    encs = [[(fn, stage_anchor(xf, z), c, 1) for fn, c in zip(encode_a(g), ENC_COST)]
            for g in range(8)]
    return norms, encs

  def enc_pieces(src, dst, t, z):
    return [[(fn, stage_anchor(src, z), c, 1)
             for fn, c in zip(encode_b(src, dst, t, g), ENC_COST)] for g in range(8)]

  def col_rounds(dst, fn, post=lambda v: v):
    def rnd(cols):
      res = fn(cols)
      if len(dst.shape) == 3:
        dst[cols.start // 128] = post(res)
      else:
        dst[0:D, cols] = post(res)
      return res
    return [functools.partial(rnd, slice(n * 128, n * 128 + 128)) for n in range(4)]

  def weights(wq, wk, wv, wao, wdn, wm, t1):
    srcs = (wq_hbm, wk_hbm, wv_hbm, wao_hbm, wm_hbm, wdn_hbm, wup_hbm, dw_hbm)
    dsts = (wq, wk, wv, wao, wm, wdn, wup.at[0:D, :], taps)
    cps = [pltpu.make_async_copy(s, d, w_sem.at[i])
           for i, (s, d) in enumerate(zip(srcs, dsts))]

    groups = [cps[0:2], cps[2:4], cps[4:5], cps[5:6] + x_copies(0, 0), cps[6:8], x_copies(0, 1)]

    def need(i):
      for cp in groups[i]:
        cp.wait()
      for g in WSTART[i + 1]:
        for cp in groups[g]:
          cp.start()
    for g in WSTART[0]:
      for cp in groups[g]:
        cp.start()
    for b in range(nbatch):
      xb[b, T:XROWS, :] = jnp.zeros((XROWS - T, D), BF16)
    for c in range(4):
      gb[c, 0:GOFF, :] = jnp.zeros((GOFF, 128), F32)
    to_bf16 = lambda v: v.astype(BF16)
    need(0)
    _run(col_rounds(wqk, lambda c: _dot_nt(wq[...], wk[c, :]),
                    lambda v: to_bf16(v * (LOG2E * D ** -0.5))), [], D)
    need(1)
    _run(col_rounds(t1, lambda c: _dot(wv[...], wao[:, c]), to_bf16), [], D)
    need(2)
    _run(col_rounds(wvom, lambda c: _dot(t1[...], wm[0:D, c]), to_bf16), [], D)
    need(3)
    norms, encs = norm_pieces(0, None, 0, 0)
    _run(col_rounds(wdm, lambda c: _dot(wdn[...], wm[D:2 * D, c])),
         [(fn, lambda v: None, c, None) for fn, _, c, _ in _merge_groups(norms)], D, span=0.7)
    _run([], _merge_groups(encs), D)
    need(4)

  sq = pltpu.VMEM((D, D), BF16)
  if _DEV is None or _DEV == 'w':
   with _scope('w'):
    pl.run_scoped(weights, sq, sq, sq, sq, sq, pltpu.VMEM((2 * D, D), BF16), sq)

  def phase1(b, z, ks, vs, gs):
    def gate_piece(t, a, g):
      v = _layernorm(_gelu(gs[a * 128 + 8 * g:a * 128 + 8 * g + 8, :]))
      rows = pl.ds(_aligned(GOFF + a * QS + 8 * g + 128 * t, 8), 8)
      for c in range(4):
        gb[c, rows, :] = v[:, c * 128:c * 128 + 128]
      return v

    def spread_taps():
      rows = taps[...].astype(F32)
      for c in range(4):
        for k in range(KW):
          dwb[c, k] = jnp.broadcast_to(rows[k:k + 1, c * 128:c * 128 + 128], (8, 128))

    def step(t, par, first, last):
      xa = xas[par]
      wide = lambda ref, *rows: jnp.concatenate(
          [_ldb(ref, k, *rows) for k in range(4)], axis=1)
      gates = [[(functools.partial(gate_piece, t, a, g), stage_anchor(gs, z), 30,
                 30 + g % GATE_CH if GATE_CH else None)]
               for a in range(4) for g in range(16)]
      keys = enc_pieces(ks, ke, t, z)
      if first:
        prev_k = enc_pieces(wup, ke, NT, z) + [[(spread_taps, lambda v: None, 40, None)]]
        prev_v = enc_pieces(wdm, ve, NT, z)
      else:
        prev_k = enc_pieces(ks, ke, t - 1, z)[NK3:]
        prev_v = enc_pieces(vs, ve, t - 1, z)
      norms, encs = ([], []) if last else norm_pieces(b, z, t + 1, 1 - par)
      _run(col_rounds(gs, lambda c: _dot(wide(xa), wup[0:D, D + c.start:D + c.stop])),
           _merge_groups(prev_k + prev_v[:NV1], norms[:NN1]), D, span=P1SPAN)
      _run(col_rounds(ks, lambda c: _dot_nt(
          wide(wqk), wide(xa, slice(c.start // 2, c.stop // 2), slice(None)))),
           _merge_groups(prev_v[NV1:] + encs[:NE2], norms[NN1:] + gates[:NG2]), D, span=P1SPAN)
      _run(col_rounds(vs, lambda c: _dot(wide(xa), wvom[:, c])),
           _merge_groups((keys if last else encs[NE2:] + keys[:NK3]), gates[NG2:]), D,
           span=P1S3)

    step(0, 0, True, False)
    for cp in x_copies(b, 1):
      cp.wait()

    def pair(i, carry):
      step(2 * i + 1, 1, False, False)
      step(2 * i + 2, 0, False, False)
      return carry
    if P1UNROLL:
      for i in range((NT - 2) // 2):
        pair(i, None)
    else:
      lax.fori_loop(0, (NT - 2) // 2, pair, None)
    step(NT - 1, 1, False, True)
    _run([], _merge_groups(enc_pieces(vs, ve, NT - 1, z)), D)

  def phase2(b, z, sb, pr0, pr1, pr2, pe_a, pe_b, pe_z, oacc, ofin, cv, gw):
    prs = [(pr0, pr1)[t % 2] for t in range(NT)] + [pr2]
    left = [PR_LEFT + t // 2 for t in range(NT)] + [PR_LEFT]

    def anchor(ref, slot):
      def put(v):
        ref[slot + z, 0:8, :] = v
      return put

    def s_prod(m, t, o, p):
      lhs = _ldb(ae, m, pl.ds((7 * o + p) * (QR // 2), QR // 2), slice(None))
      return _dot(lhs, _ldb(ke, t, 7 * o + p, slice(0, 64), slice(None)))

    raw = [(o, p) for o in (5, 6) for p in (0, 2, 4)]

    def s_round_a(m, t, o):
      m2, m4, m6, m7 = [s_prod(m, t, o, p) for p in (1, 3, 5, 6)]
      pr = prs[t]
      pr[3 * o, 0:QR, :] = m4 + m7
      pr[3 * o + 1, 0:QR, :] = m2 + m4
      pr[3 * o + 2, 0:QR, :] = m6 - m2
      return m7

    def s_round_b(m, t, o):
      m1, m3, m5 = [s_prod(m, t, o, p) for p in (0, 2, 4)]
      extra = s_prod(m, t, *raw[o])
      pr = prs[t]
      pr[21 + 2 * o, 0:QR, :] = m1 - m5
      pr[22 + 2 * o, 0:QR, :] = m3 + m5
      pr[PR_RAW + o, 0:QR, :] = extra
      return extra

    def z_prod(p):
      res = _dot(_ldb(pe_z, p), _ldb(ve, NT, p, slice(0, 64), slice(None)))
      oacc[p, 0:QR, :] = res
      return res

    def left_round(m, tiles, z_too):
      res = None
      for t in tiles:
        res = s_prod(m, t, *raw[5])
        prs[t][left[t], 0:QR, :] = res
      if z_too:
        res = z_prod(48)
      return res

    def z_round(k):
      return [z_prod(p) for p in range(4 * k, 4 * k + 4)][-1]

    def pv_round(second, p):
      pe = pe_b if second else pe_a
      lhs = jnp.concatenate([_ldb(pe, 49 * i + p) for i in range(4)], axis=1)
      rhs = jnp.concatenate([_ldb(ve, 4 * second + i, p, slice(0, 64), slice(None)) for i in range(4)], axis=0)
      res = _dot(lhs, rhs)
      (ofin if second else oacc)[p, 0:QR, :] = oacc[p, 0:QR, :] + res
      return res

    def comb_piece(t, r, i):
      rows = slice(r, r + 8)
      pr = prs[t]

      def inner(o):
        if o < 5:
          xx, yy = pr[21 + 2 * o, rows, :], pr[22 + 2 * o, rows, :]
        else:
          slots = [PR_RAW + n if n < 5 else left[t]
                   for n in range(3 * (o - 5), 3 * (o - 5) + 3)]
          m1, m3, m5 = [pr[n, rows, :] for n in slots]
          xx, yy = m1 - m5, m3 + m5
        if i == 0:
          return {(0, 0): xx + pr[3 * o, rows, :], (0, 1): yy}
        return {(1, 0): pr[3 * o + 1, rows, :], (1, 1): xx + yy + pr[3 * o + 2, rows, :]}
      c = _decode_outer(inner)
      if t == NT:
        for (a, k), v in c.items():
          v = _gelu(v)
          sb[SL_U + 4 * a + k, rows, :] = v
        return v
      if t == NT - 1:
        lane = lax.broadcasted_iota(jnp.int32, (8, 128), 1)
      for a in (i, i + 2):
        vs = [c[(a, k)] for k in range(4)]
        if t == NT - 1:
          vs = [jnp.where(lane < min(QS, T - k * QS) - 128 * t, v, -jnp.inf)
                for k, v in enumerate(vs)]
        for k in range(4):
          sb[16 * t + 4 * a + k, rows, :] = vs[k]
        mx = jnp.maximum(jnp.maximum(vs[0], vs[1]), jnp.maximum(vs[2], vs[3]))
        if t > 0:
          m_old = sb[SL_M + a, rows, :]
          mx = jnp.maximum(mx, m_old)
        e = [jnp.exp2(v - mx) for v in vs]
        ls = (e[0] + e[1]) + (e[2] + e[3])
        if t > 0:
          ls = ls + sb[SL_L + a, rows, :] * jnp.exp2(m_old - mx)
        sb[SL_M + a, rows, :] = mx
        sb[SL_L + a, rows, :] = ls
      return mx

    def norm_const_steps(r):
      rows = slice(r, r + 8)
      off = []

      def compute():
        for a in range(4):
          mx = sb[SL_M + a, rows, :]
          m_row = jnp.max(mx, axis=-1, keepdims=True)
          l_row = jnp.sum(sb[SL_L + a, rows, :] * jnp.exp2(mx - m_row), axis=-1, keepdims=True)
          off.append(jnp.broadcast_to(m_row + jnp.log2(l_row), (8, 128)))
        return off[-1]

      def store():
        for a in range(4):
          sb[SL_OFF + a, rows, :] = off[a]
      return compute, store

    def prep_steps(t, r):
      rows = slice(r, r + 16)

      def fetch(a, k):
        if t < NT:
          return jnp.exp2(sb[16 * t + 4 * a + k, rows, :] - sb[SL_OFF + a, rows, :])
        return sb[SL_U + 4 * a + k, rows, :] * cv[4 * a + k, rows, :]

      def store(p, v):
        if t == NT:
          pe_z[p, rows, :] = v.astype(BF16)
        else:
          (pe_a if t < 4 else pe_b)[49 * (t % 4) + p, rows, :] = v.astype(BF16)
      return _encode_steps(fetch, _A_STEPS, _A_TERMS, _enc_a, store)

    def window_piece(j, a, r):
      for c in range(4):
        v = gb[c, pl.ds(_aligned(a * QS + r + j * QR, 16), 16), :]
        gw[4 * a + c, r:r + 16, :] = v
      return v

    def conv_steps(a, c, r):
      base = GOFF - KW // 2 + r
      acc = [None] * CONV_N

      def step(shifts):
        for sh in shifts:
          taps = range(sh, KW, 8)
          g = [gw[4 * a + c, pl.ds(base + sh + 8 * i, 8), :] for i in range(CONV_N + len(taps) - 1)]
          for q, k in enumerate(taps):
            w = dwb[c, k]
            for h in range(CONV_N):
              v = g[h + q] * w
              acc[h] = v if acc[h] is None else acc[h] + v
        if shifts[-1] == 7:
          for h in range(CONV_N):
            cv[4 * a + c, r + 8 * h:r + 8 * h + 8, :] = acc[h]
        return acc[-1]
      return [functools.partial(step, range(s0, s0 + CONV_SH)) for s0 in range(0, 8, CONV_SH)]

    def out_piece(j, par, r):
      halves = []
      for h in range(2):
        rows = slice(r + 8 * h, r + 8 * h + 8)
        halves.append(_decode_outer(
            lambda o: _decode_inner([ofin[7 * o + p, rows, :] for p in range(7)])))
      for a in range(4):
        xr = pl.ds(_aligned(a * QS + r + j * QR, 16), 16)
        for k in range(4):
          cols = slice(k * 128, k * 128 + 128)
          y = jnp.concatenate([halves[0][(a, k)], halves[1][(a, k)]], axis=0)
          y = xb[b, xr, cols].astype(F32) + y
          stage[par, a, r:r + 16, cols] = y.astype(BF16)
      return y

    def ganchor(v):
      gb[3, pl.ds(pl.multiple_of(GOFF + XROWS + z, 8), 8), :] = v

    def zanchor(v):
      anchor(sb, SL_DUMMY)(v)
      anchor(cv, 16)(v)

    def iteration(m, do_s, do_p, do_o):
      part = functools.partial
      par = m % 2
      convs = [[(fn, anchor(gw, 16), CONV_N * CONV_SH * CW, CCH) for fn in conv_steps(a, c, r)]
               for a in range(4) for c in range(4) for r in range(0, QR, 8 * CONV_N)]
      outs = [[(part(out_piece, m - 2, par, r), anchor(ofin, 49), 90, OCH)]
              for r in range(0, QR, 16)]
      if do_o and not do_p:
        norms, encs = norm_pieces(jnp.minimum(b + 1, nbatch - 1), z, 0, 0)
        next_rows = norms + encs
      first, zk = [[] for _ in range(5)], 0
      for j, (n_b, n_z) in enumerate(((12, 0), (9, 3), (9, 3), (10, 3), (9, 3))):
        p0 = sum((0, 12, 9, 9, 10)[:j + 1])
        bs = [part(pv_round, 1, p) for p in range(p0, p0 + n_b)] if do_o else []
        zs = [part(z_round, k) for k in range(zk, zk + n_z)] if do_p else []
        zk += n_z
        first[j] = bs + zs if j == 4 else _merge(bs, zs)
      pv_split = [0, 12, 24, 36, 49]
      for j in range(NT + 1):
        s_rounds, v_rounds = [], []
        if do_s:
          if j in (0, 4):
            s_rounds.append(part(left_round, m, range(j, j + 4), False))
          for o in range(7):
            s_rounds.append(part(s_round_a, m, j, o))
            if o < 5:
              s_rounds.append(part(s_round_b, m, j, o))
        if j < 5:
          v_rounds = first[j]
        if j == 4 and (do_s or do_p):
          v_rounds.append(part(left_round, m, [NT] if do_s else [], do_p))
        if do_p and j > 4:
          if j == 5:
            anchor(oacc, 49)(jnp.zeros((8, 128), F32))
            pe_a[4 * 49 + z, 0:16, :] = jnp.zeros((16, 128), BF16)
          v_rounds = [part(pv_round, 0, p) for p in range(pv_split[j - 5], pv_split[j - 4])]
        t = j - 1 if j > 0 else NT
        main = []
        for r in range(0, QR, 8):
          combs = [[(part(comb_piece, t, r, i), anchor(prs[t], PR_DUMMY), CC if j else UC, 1)]
                   for i in range(2)]
          if j > 0:
            if do_p and r % 16 == 0:
              main.append([(fn, anchor(sb, SL_DUMMY), c, 1)
                           for fn, c in zip(prep_steps(t, r), PC)])
            if do_s:
              main += combs
          elif do_p:
            main += combs
            if r % 16 == 8:
              main.append([(fn, zanchor, c, 1)
                           for fn, c in zip(prep_steps(t, r - 8), ZC)])
        lists = [main]
        if do_s and j == 0:
          window = [[(part(window_piece, m, a, r), ganchor, 6, 0)]
                    for a in range(4) for r in range(0, QR + 2 * GOFF, 16)]
        if do_s:
          share = CVS if do_o else CV1 if do_p else CV0
          lo, hi = [len(convs) * sum(share[:n]) // sum(share) for n in (j, j + 1)]
          lists.append((window if j == 0 else []) + convs[lo:hi])
        if do_p and j == 0:
          steps = [norm_const_steps(r) for r in range(0, QR, 8)]
          seq = []
          for n in range(len(steps) + 3):
            if n < len(steps):
              seq.append([(steps[n][0], anchor(sb, SL_DUMMY), NC, 10 + n % NCH if NCH else None)])
            if n >= 3:
              seq.append([(steps[n - 3][1], lambda v: None, 1, None)])
          lists.append(seq)
        if do_o and not do_p and j < 5:
          lists.append(next_rows[8 * j:8 * j + 8])
        if do_o and j > 4:
          lists.append(outs[(9 * (j - 5)) // 4:(9 * (j - 4)) // 4])
        _run(_merge(s_rounds, v_rounds), _merge_groups(*lists), QR, span=SPAN)

    if _DEV is not None:
      lax.fori_loop(2, NB, lambda m, c: iteration(m, *_DEV), None)
      stage[0, 0, :, 0:128] = (cv[z, pl.ds(z, QR), :] + sb[z, pl.ds(z, QR), :] + oacc[z, pl.ds(z, QR), :] + pe_b[z, pl.ds(pl.multiple_of(z, 16), QR), :].astype(F32)).astype(BF16)
      return
    with _scope('it0'):
      iteration(0, True, False, False)

    @pl.when(b > 0)
    def _():
      for cp in o_copies(b - 1, NB - 2, 1) + o_copies(b - 1, NB - 1, 0, last=True):
        cp.wait()
    with _scope('it1'):
      iteration(1, True, True, False)

    def steady(m, carry):
      @pl.when(m >= 4)
      def _():
        for cp in o_copies(b, m - 4, m % 2):
          cp.wait()
      with _scope('steady'):
        iteration(m, True, True, True)
      for cp in o_copies(b, m - 2, m % 2):
        cp.start()
      return carry
    lax.fori_loop(2, NB, steady, None)
    for cp in o_copies(b, NB - 4, NB % 2):
      cp.wait()
    with _scope('it7'):
      iteration(NB, False, True, True)
    for cp in o_copies(b, NB - 2, NB % 2):
      cp.start()
    for cp in o_copies(b, NB - 3, (NB + 1) % 2):
      cp.wait()

    @pl.when(b + 1 < nbatch)
    def _():
      for cp in x_copies(b + 1, 0):
        cp.wait()
    with _scope('it8'):
      iteration(NB + 1, False, False, True)
    for cp in o_copies(b, NB - 1, (NB + 1) % 2, last=True):
      cp.start()

  def batch(b, carry):
    z = lax.shift_right_logical(b, 8)
    st = pltpu.VMEM((D + 8, D), F32)

    if _DEV is None or _DEV == 'p1':
     with _scope('p1'):
      pl.run_scoped(functools.partial(phase1, b, z), st, st, st)

    @pl.when(b + 1 < nbatch)
    def _():
      for cp in x_copies(b + 1, 0) + x_copies(b + 1, 1):
        cp.start()
    blocks = lambda n: pltpu.VMEM((n, QR + FPAD, 128), F32)
    if _DEV == 'p1':
      @pl.when(xb[0, 0:16, 0:128].astype(F32)[0, 0] > 1e30)
      def _():
        stage[0, 0, :, 0:128] = (gb[z, pl.ds(z, QR), :] + ae[z, pl.ds(pl.multiple_of(z, 16), QR), :].astype(F32) + ke[z, z, pl.ds(pl.multiple_of(z, 16), 16), :].astype(F32).sum() + ve[z, z, pl.ds(pl.multiple_of(z, 16), 16), :].astype(F32).sum() + dwb[z, z].sum()).astype(BF16)
    if _DEV != 'p1': pl.run_scoped(
        functools.partial(phase2, b, z),
        blocks(SL_DUMMY + 1), blocks(PR_DUMMY + 1), blocks(PR_DUMMY + 1), blocks(PR_DUMMY + 1),
        pltpu.VMEM((4 * 49 + 1, QR, 128), BF16), pltpu.VMEM((4 * 49, QR, 128), BF16),
        pltpu.VMEM((49, QR, 128), BF16), blocks(50), blocks(50), blocks(17),
        pltpu.VMEM((17, QR + 2 * GOFF + GPAD, 128), F32))
    return carry

  if _DEV == 'w':
    for cp in x_copies(0, 1): cp.wait()
    stage[0, 0, :, 0:128] = ae[0, 0:QR, :] + wdm[0:QR, 0:128].astype(BF16) + wqk[0, 0:QR, :] + wvom[0:QR, 0:128] + xa0[0, 0:QR, :]
  else: lax.fori_loop(0, nbatch, batch, None)
  if _DEV is not None:
    for cp in o_copies(0, 0, 0):
      cp.start(); cp.wait()
    return
  for cp in o_copies(nbatch - 1, NB - 2, 1) + o_copies(nbatch - 1, NB - 1, 0, last=True):
    cp.wait()


@jax.jit
def pallas_standalone__conformer_family_branchformer__speech_kernel(
    x: jax.Array,
    w_q: jax.Array,
    w_k: jax.Array,
    w_v: jax.Array,
    w_ao: jax.Array,
    w_up: jax.Array,
    dw: jax.Array,
    w_dn: jax.Array,
    w_merge: jax.Array,
):
  nbatch = x.shape[0]
  assert x.shape[1:] == (T, D) and dw.shape == (KW, D)
  any_spec = pl.BlockSpec(memory_space=pl.ANY)
  return pl.pallas_call(
      _kernel,
      out_shape=jax.ShapeDtypeStruct(x.shape, x.dtype),
      in_specs=[any_spec] * 9,
      out_specs=any_spec,
      scratch_shapes=[
          pltpu.VMEM((nbatch, XROWS + 16, D), BF16),
          pltpu.VMEM((NB + 1, AE_ROWS, 128), BF16),
          pltpu.VMEM((NT + 1, 49, 128 + WPAD, 128), BF16),
          pltpu.VMEM((NT + 1, 49, 128 + WPAD, 128), BF16),
          pltpu.VMEM((4, GOFF + XROWS + 32, 128), F32),
          pltpu.VMEM((4, KW, 8, 128), F32),
          pltpu.VMEM((4, D, 128), BF16),
          pltpu.VMEM((D, D), BF16),
          pltpu.VMEM((D + 16, 2 * D), BF16),
          pltpu.VMEM((D + 8, D), F32),
          pltpu.VMEM((KW, D), BF16),
          pltpu.VMEM((2, 4, QR, D), BF16),
          pltpu.VMEM((4, D, 128), BF16),
          pltpu.VMEM((4, D, 128), BF16),
          pltpu.VMEM((D + 8, D), F32),
          pltpu.SemaphoreType.DMA((8,)),
          pltpu.SemaphoreType.DMA((8 * nbatch,)),
          pltpu.SemaphoreType.DMA((8,)),
      ],
      compiler_params=pltpu.CompilerParams(vmem_limit_bytes=126 * 1024 * 1024, flags=_FLAGS),
      name="branchformer",
  )(x, w_q, w_k, w_v, w_ao, w_up, dw, w_dn, w_merge)
```

```python
import functools

import jax
import jax.numpy as jnp
from jax import lax
import jax.experimental.pallas as pl
import jax.experimental.pallas.tpu as pltpu

F32, BF16, U32 = jnp.float32, jnp.bfloat16, jnp.uint32

T, D, KW = 4000, 512, 31
QS = 1008
QR = 144
NB = 7
NT = 8
XROWS = 3 * QS + NT * 128
AE_ROWS = 7104
GOFF = 16
EPS = 1e-5
LOG2E = 1.4426950408889634

FPAD = 8
CONV_N = 3
ENC_COST, PREP_COST, PREP_Z_COST = (35, 25, 25), (50, 32, 32), (30, 24, 24)

SL_U = 16 * NT
SL_M = SL_U + 16
SL_L = SL_M + 4
SL_OFF = SL_L + 4
SL_DUMMY = SL_OFF + 4
PR_RAW = 31
PR_LEFT = 36
PR_DUMMY = 40


def _enc_a(a11, a12, a21, a22):
  return [a11 + a22, a21 + a22, a11, a22, a11 + a12, a21 - a11, a12 - a22]


def _enc_b(b11, b12, b21, b22):
  return [b11 + b22, b11, b12 - b22, b21 - b11, b22, b11 + b12, b21 + b22]


_A_TERMS = ([(0, 0, 1), (1, 1, 1)], [(1, 0, 1), (1, 1, 1)], [(0, 0, 1)], [(1, 1, 1)],
            [(0, 0, 1), (0, 1, 1)], [(1, 0, 1), (0, 0, -1)], [(0, 1, 1), (1, 1, -1)])
_B_TERMS = ([(0, 0, 1), (1, 1, 1)], [(0, 0, 1)], [(0, 1, 1), (1, 1, -1)],
            [(1, 0, 1), (0, 0, -1)], [(1, 1, 1)], [(0, 0, 1), (0, 1, 1)],
            [(1, 0, 1), (1, 1, 1)])
_USE = ([((0, 0), 1), ((1, 1), 1)], [((1, 0), 1), ((1, 1), -1)],
        [((0, 1), 1), ((1, 1), 1)], [((0, 0), 1), ((1, 0), 1)],
        [((0, 0), -1), ((0, 1), 1)], [((1, 1), 1)], [((0, 0), 1)])


def _lin(terms):
  acc = None
  for v, s in terms:
    if acc is None:
      acc = v
    else:
      acc = acc + v if s > 0 else acc - v
  return acc


def _encode2(blk, terms, enc, store, outer=range(7)):
  for o in outer:
    q = [[_lin([(blk[2 * r + i][2 * c + j], s) for r, c, s in terms[o]])
          for j in range(2)] for i in range(2)]
    for p, v in enumerate(enc(q[0][0], q[0][1], q[1][0], q[1][1])):
      store(7 * o + p, v)
  return v


_A_STEPS = (([(0, 0), (1, 1)], (2, 0, 3)), ([(1, 0)], (1, 5)), ([(0, 1)], (4, 6)))
_B_STEPS = (([(0, 0), (1, 1)], (1, 0, 4)), ([(0, 1)], (2, 5)), ([(1, 0)], (3, 6)))


def _encode_steps(fetch, steps, terms, enc, store):
  blk = [[None] * 4 for _ in range(4)]

  def step(quads, outer):
    for r, c in quads:
      for i in range(2):
        for j in range(2):
          blk[2 * r + i][2 * c + j] = fetch(2 * r + i, 2 * c + j)
    return _encode2(blk, terms, enc, store, outer)
  return [functools.partial(step, *st) for st in steps]


def _decode_outer(inner):
  c = {}
  for o in range(7):
    quad = inner(o)
    for qi, v in quad.items():
      for qo, s in _USE[o]:
        key = (2 * qo[0] + qi[0], 2 * qo[1] + qi[1])
        if key not in c:
          c[key] = v
        else:
          c[key] = c[key] + v if s > 0 else c[key] - v
  return c


def _decode_inner(m):
  return {(0, 0): m[0] + m[3] - m[4] + m[6], (0, 1): m[2] + m[4],
          (1, 0): m[1] + m[3], (1, 1): m[0] - m[1] + m[2] + m[5]}


def _layernorm(v):
  mean = jnp.sum(v, axis=-1, keepdims=True) * (1.0 / D)
  d = v - mean
  var = jnp.sum(d * d, axis=-1, keepdims=True) * (1.0 / D)
  return d * lax.rsqrt(var + EPS)


def _gelu(v):
  c1 = 0.7978845608028654
  inner = v * (c1 + (c1 * 0.044715) * (v * v))
  h = 0.5 * v
  return h + h * jnp.tanh(inner)


def _dot(a, b):
  return jnp.dot(a, b, preferred_element_type=F32)


def _dot_nt(a, b):
  return lax.dot_general(a, b, (((1,), (1,)), ((), ())), preferred_element_type=F32)


def _aligned(i, n):
  return i if isinstance(i, int) else pl.multiple_of(i, n)


def _ldb(ref, *idx):
  return pltpu.bitcast(ref.bitcast(U32)[idx], BF16)


def _run(rounds, pieces, rows, span=1.0):
  if not rounds:
    for fn, _, _, _ in pieces:
      fn()
    return
  per = rows // 8
  total = len(rounds) * per * span / max(1, sum(p[2] for p in pieces))
  j, done, last = 0, 0, {}
  for k, rnd in enumerate(rounds):
    res = rnd()
    while j < len(pieces) and int(done * total) < (k + 1) * per:
      r = (int(done * total) - k * per) * 8
      fn, anchor, cost, chain = pieces[j]
      pin = res[r:r + 8, 0:128]
      anchor(pin + last[chain] if chain in last else pin)
      tok = fn()
      if chain is not None:
        last[chain] = tok[0:8, 0:128]
      j += 1
      done += cost


def _merge(*lists, cost=lambda v: 1):
  keyed = []
  for n, l in enumerate(lists):
    total, done = max(1, sum(cost(v) for v in l)), 0
    for i, v in enumerate(l):
      keyed.append(((done + 0.5 * cost(v)) / total, n, i, v))
      done += cost(v)
  return [v for _, _, _, v in sorted(keyed, key=lambda e: e[:3])]


def _merge_groups(*lists):
  merged = _merge(*lists, cost=lambda g: sum(p[2] for p in g))
  return [p for g in merged for p in g]


def _kernel(x_hbm, wq_hbm, wk_hbm, wv_hbm, wao_hbm, wup_hbm, dw_hbm, wdn_hbm, wm_hbm,
            o_hbm, xb, ae, ke, ve, gb, dwb, wqk, wvom, wup, wdm, taps, stage, xa0, xa1, xf,
            w_sem, x_sem, o_sem):
  nbatch = x_hbm.shape[0]
  xas = (xa0, xa1)

  def x_copies(b, part):
    cps = []
    for a in range(4):
      lo, hi = (0, 256) if part == 0 else (256, min(QS, T - a * QS))
      rows = pl.ds(a * QS + lo, hi - lo)
      cps.append(pltpu.make_async_copy(
          x_hbm.at[b, rows, :], xb.at[b, rows, :], x_sem.at[b * 8 + part * 4 + a]))
    return cps

  def o_copies(b, j, par, last=False):
    cps = []
    for a in range(4):
      n = min(QR, T - (a * QS + (NB - 1) * QR)) if last else QR
      cps.append(pltpu.make_async_copy(
          stage.at[par, a, pl.ds(0, n), :],
          o_hbm.at[b, pl.ds(a * QS + j * QR, n), :], o_sem.at[par * 4 + a]))
    return cps

  def block_fetch(src, g):
    def fetch(i, j):
      return src[i * 128 + 16 * g:i * 128 + 16 * g + 16, j * 128:j * 128 + 128].astype(F32)
    return fetch

  def encode_b(src, dst, t, g):
    def store(p, v):
      dst[t, p, 16 * g:16 * g + 16, :] = v.astype(BF16)
    return _encode_steps(block_fetch(src, g), _B_STEPS, _B_TERMS, _enc_b, store)

  def stage_anchor(ref, z):
    def put(v):
      if ref.dtype == BF16:
        ref[pl.ds(pl.multiple_of(D + z, 16), 16), 0:128] = jnp.concatenate(
            [v, v], axis=0).astype(BF16)
      else:
        ref[pl.ds(pl.multiple_of(D + z, 8), 8), 0:128] = v
    return put

  def norm_pieces(b, z, t, par):
    def norm(a, g):
      r0 = _aligned(a * QS + 16 * g + 128 * t, 16)
      xa = _layernorm(xb[b, pl.ds(r0, 16), :].astype(F32))
      rows = slice(a * 128 + 16 * g, a * 128 + 16 * g + 16)
      for k in range(4):
        xas[par][k, rows, :] = xa[:, k * 128:k * 128 + 128].astype(BF16)
      xf[rows, :] = xa

    def encode_a(g):
      pos = 128 * t + 16 * g
      j, r = pos // QR, pos % QR
      view = ae.at[j, pl.ds(_aligned(r, 16), 48 * QR + 16), :]

      def store(p, v):
        view[p * QR:p * QR + 16, :] = v.astype(BF16)
      return _encode_steps(block_fetch(xf, g), _A_STEPS, _A_TERMS, _enc_a, store)

    def xanchor(v):
      xb[0, pl.ds(pl.multiple_of(XROWS + z, 16), 16), 0:128] = jnp.concatenate(
          [v, v], axis=0).astype(BF16)
    norms = [[(functools.partial(norm, a, g), xanchor, 30, None)]
             for g in range(8) for a in range(4)]
    encs = [[(fn, stage_anchor(xf, z), c, 1) for fn, c in zip(encode_a(g), ENC_COST)]
            for g in range(8)]
    return norms, encs

  def enc_pieces(src, dst, t, z):
    return [[(fn, stage_anchor(src, z), c, 1)
             for fn, c in zip(encode_b(src, dst, t, g), ENC_COST)] for g in range(8)]

  def col_rounds(dst, fn, post=lambda v: v):
    def rnd(cols):
      res = fn(cols)
      if len(dst.shape) == 3:
        dst[cols.start // 128] = post(res)
      else:
        dst[0:D, cols] = post(res)
      return res
    return [functools.partial(rnd, slice(n * 128, n * 128 + 128)) for n in range(4)]

  def weights(wq, wk, wv, wao, wdn, wm, t1):
    srcs = (wq_hbm, wk_hbm, wv_hbm, wao_hbm, wm_hbm, wdn_hbm, wup_hbm, dw_hbm)
    dsts = (wq, wk, wv, wao, wm, wdn, wup.at[0:D, :], taps)
    cps = [pltpu.make_async_copy(s, d, w_sem.at[i])
           for i, (s, d) in enumerate(zip(srcs, dsts))]

    groups = [cps[0:2], cps[2:4], cps[4:5], cps[5:6] + x_copies(0, 0), cps[6:8],
              x_copies(0, 1), []]

    def need(i):
      for cp in groups[i]:
        cp.wait()
      for cp in groups[i + 2]:
        cp.start()
    for cp in groups[0] + groups[1]:
      cp.start()
    for b in range(nbatch):
      xb[b, T:XROWS, :] = jnp.zeros((XROWS - T, D), BF16)
    for c in range(4):
      gb[c, 0:GOFF, :] = jnp.zeros((GOFF, 128), F32)
    to_bf16 = lambda v: v.astype(BF16)
    need(0)
    _run(col_rounds(wqk, lambda c: _dot_nt(wq[...], wk[c, :]),
                    lambda v: to_bf16(v * (LOG2E * D ** -0.5))), [], D)
    need(1)
    _run(col_rounds(t1, lambda c: _dot(wv[...], wao[:, c]), to_bf16), [], D)
    need(2)
    _run(col_rounds(wvom, lambda c: _dot(t1[...], wm[0:D, c]), to_bf16), [], D)
    need(3)
    norms, encs = norm_pieces(0, None, 0, 0)
    _run(col_rounds(wdm, lambda c: _dot(wdn[...], wm[D:2 * D, c])),
         [(fn, lambda v: None, c, None) for fn, _, c, _ in _merge_groups(norms)], D, span=0.7)
    _run([], _merge_groups(encs), D)
    need(4)

  sq = pltpu.VMEM((D, D), BF16)
  pl.run_scoped(weights, sq, sq, sq, sq, sq, pltpu.VMEM((2 * D, D), BF16), sq)

  def phase1(b, z, ks, vs, gs):
    def gate_piece(t, a, g):
      v = _layernorm(_gelu(gs[a * 128 + 8 * g:a * 128 + 8 * g + 8, :]))
      rows = pl.ds(_aligned(GOFF + a * QS + 8 * g + 128 * t, 8), 8)
      for c in range(4):
        gb[c, rows, :] = v[:, c * 128:c * 128 + 128]

    def spread_taps():
      rows = taps[...].astype(F32)
      for c in range(4):
        for k in range(KW):
          dwb[c, k] = jnp.broadcast_to(rows[k:k + 1, c * 128:c * 128 + 128], (8, 128))

    def step(t, par, first, last):
      xa = xas[par]
      wide = lambda ref, *rows: jnp.concatenate(
          [_ldb(ref, k, *rows) for k in range(4)], axis=1)
      gates = [[(functools.partial(gate_piece, t, a, g), stage_anchor(gs, z), 30, None)]
               for a in range(4) for g in range(16)]
      keys = enc_pieces(ks, ke, t, z)
      if first:
        prev_k = enc_pieces(wup, ke, NT, z) + [[(spread_taps, lambda v: None, 40, None)]]
        prev_v = enc_pieces(wdm, ve, NT, z)
      else:
        prev_k = enc_pieces(ks, ke, t - 1, z)[2:]
        prev_v = enc_pieces(vs, ve, t - 1, z)
      norms, encs = ([], []) if last else norm_pieces(b, z, t + 1, 1 - par)
      _run(col_rounds(gs, lambda c: _dot(wide(xa), wup[0:D, D + c.start:D + c.stop])),
           _merge_groups(prev_k + prev_v[:4], norms), D, span=0.95)
      _run(col_rounds(ks, lambda c: _dot_nt(
          wide(wqk), wide(xa, slice(c.start // 2, c.stop // 2), slice(None)))),
           _merge_groups(prev_v[4:], gates[:32]), D, span=0.95)
      _run(col_rounds(vs, lambda c: _dot(wide(xa), wvom[:, c])),
           _merge_groups(keys if last else encs + keys[:2], gates[32:]), D, span=0.85)

    step(0, 0, True, False)
    for cp in x_copies(b, 1):
      cp.wait()

    def pair(i, carry):
      step(2 * i + 1, 1, False, False)
      step(2 * i + 2, 0, False, False)
      return carry
    lax.fori_loop(0, (NT - 2) // 2, pair, None)
    step(NT - 1, 1, False, True)
    _run([], _merge_groups(enc_pieces(vs, ve, NT - 1, z)), D)

  def phase2(b, z, sb, pr0, pr1, pr2, pe_a, pe_b, pe_z, oacc, ofin, cv, gw):
    prs = [(pr0, pr1)[t % 2] for t in range(NT)] + [pr2]
    left = [PR_LEFT + t // 2 for t in range(NT)] + [PR_LEFT]

    def anchor(ref, slot):
      def put(v):
        ref[slot + z, 0:8, :] = v
      return put

    def s_prod(m, t, o, p):
      lhs = _ldb(ae, m, pl.ds((7 * o + p) * (QR // 2), QR // 2), slice(None))
      return _dot(lhs, _ldb(ke, t, 7 * o + p))

    raw = [(o, p) for o in (5, 6) for p in (0, 2, 4)]

    def s_round_a(m, t, o):
      m2, m4, m6, m7 = [s_prod(m, t, o, p) for p in (1, 3, 5, 6)]
      pr = prs[t]
      pr[3 * o, 0:QR, :] = m4 + m7
      pr[3 * o + 1, 0:QR, :] = m2 + m4
      pr[3 * o + 2, 0:QR, :] = m6 - m2
      return m7

    def s_round_b(m, t, o):
      m1, m3, m5 = [s_prod(m, t, o, p) for p in (0, 2, 4)]
      extra = s_prod(m, t, *raw[o])
      pr = prs[t]
      pr[21 + 2 * o, 0:QR, :] = m1 - m5
      pr[22 + 2 * o, 0:QR, :] = m3 + m5
      pr[PR_RAW + o, 0:QR, :] = extra
      return extra

    def z_round(k):
      for p in range(4 * k, 4 * k + 4):
        res = _dot(_ldb(pe_z, p), _ldb(ve, NT, p))
        oacc[p, 0:QR, :] = res
      return res

    def left_round(m, tiles):
      for t in tiles:
        res = s_prod(m, t, *raw[5])
        prs[t][left[t], 0:QR, :] = res
      return res

    def last_left_round(m, do_s, do_z):
      outs = []
      for lo, hi in ((0, 80), (80, QR)):
        if do_s:
          lhs = _ldb(ae, m, pl.ds(46 * (QR // 2) + lo // 2, (hi - lo) // 2), slice(None))
          res = _dot(lhs, _ldb(ke, NT, 46))
          prs[NT][left[NT], lo:hi, :] = res
        if do_z:
          res = _dot(_ldb(pe_z, 48, slice(lo // 2, hi // 2), slice(None)), _ldb(ve, NT, 48))
          oacc[48, lo:hi, :] = res
        outs.append(res)
      return jnp.concatenate(outs, axis=0)

    def pv_round(second, p):
      pe = pe_b if second else pe_a
      lhs = jnp.concatenate([_ldb(pe, 49 * i + p) for i in range(4)], axis=1)
      rhs = jnp.concatenate([_ldb(ve, 4 * second + i, p) for i in range(4)], axis=0)
      res = _dot(lhs, rhs)
      (ofin if second else oacc)[p, 0:QR, :] = oacc[p, 0:QR, :] + res
      return res

    def comb_piece(t, r, i):
      rows = slice(r, r + 8)
      pr = prs[t]

      def inner(o):
        if o < 5:
          xx, yy = pr[21 + 2 * o, rows, :], pr[22 + 2 * o, rows, :]
        else:
          slots = [PR_RAW + n if n < 5 else left[t]
                   for n in range(3 * (o - 5), 3 * (o - 5) + 3)]
          m1, m3, m5 = [pr[n, rows, :] for n in slots]
          xx, yy = m1 - m5, m3 + m5
        if i == 0:
          return {(0, 0): xx + pr[3 * o, rows, :], (0, 1): yy}
        return {(1, 0): pr[3 * o + 1, rows, :], (1, 1): xx + yy + pr[3 * o + 2, rows, :]}
      c = _decode_outer(inner)
      if t == NT:
        for (a, k), v in c.items():
          v = _gelu(v)
          sb[SL_U + 4 * a + k, rows, :] = v
        return v
      if t == NT - 1:
        lane = lax.broadcasted_iota(jnp.int32, (8, 128), 1)
      for a in (i, i + 2):
        vs = [c[(a, k)] for k in range(4)]
        if t == NT - 1:
          vs = [jnp.where(lane < min(QS, T - k * QS) - 128 * t, v, -jnp.inf)
                for k, v in enumerate(vs)]
        for k in range(4):
          sb[16 * t + 4 * a + k, rows, :] = vs[k]
        mx = jnp.maximum(jnp.maximum(vs[0], vs[1]), jnp.maximum(vs[2], vs[3]))
        if t > 0:
          m_old = sb[SL_M + a, rows, :]
          mx = jnp.maximum(mx, m_old)
        e = [jnp.exp2(v - mx) for v in vs]
        ls = (e[0] + e[1]) + (e[2] + e[3])
        if t > 0:
          ls = ls + sb[SL_L + a, rows, :] * jnp.exp2(m_old - mx)
        sb[SL_M + a, rows, :] = mx
        sb[SL_L + a, rows, :] = ls
      return mx

    def norm_const_steps(r):
      rows = slice(r, r + 8)
      off = []

      def compute():
        for a in range(4):
          mx = sb[SL_M + a, rows, :]
          m_row = jnp.max(mx, axis=-1, keepdims=True)
          l_row = jnp.sum(sb[SL_L + a, rows, :] * jnp.exp2(mx - m_row), axis=-1, keepdims=True)
          off.append(jnp.broadcast_to(m_row + jnp.log2(l_row), (8, 128)))

      def store():
        for a in range(4):
          sb[SL_OFF + a, rows, :] = off[a]
      return compute, store

    def prep_steps(t, r):
      rows = slice(r, r + 16)

      def fetch(a, k):
        if t < NT:
          return jnp.exp2(sb[16 * t + 4 * a + k, rows, :] - sb[SL_OFF + a, rows, :])
        return sb[SL_U + 4 * a + k, rows, :] * cv[4 * a + k, rows, :]

      def store(p, v):
        if t == NT:
          pe_z[p, rows, :] = v.astype(BF16)
        else:
          (pe_a if t < 4 else pe_b)[49 * (t % 4) + p, rows, :] = v.astype(BF16)
      return _encode_steps(fetch, _A_STEPS, _A_TERMS, _enc_a, store)

    def window_piece(j, a, r):
      for c in range(4):
        v = gb[c, pl.ds(_aligned(a * QS + r + j * QR, 16), 16), :]
        gw[4 * a + c, r:r + 16, :] = v
      return v

    def conv_steps(a, c, r):
      base = GOFF - KW // 2 + r
      acc = [None] * CONV_N

      def step(shifts):
        for sh in shifts:
          ks = range(sh, KW, 8)
          g = [gw[4 * a + c, pl.ds(base + sh + 8 * i, 8), :]
               for i in range(CONV_N + len(ks) - 1)]
          for q, k in enumerate(ks):
            w = dwb[c, k]
            for h in range(CONV_N):
              v = g[h + q] * w
              acc[h] = v if acc[h] is None else acc[h] + v
        if shifts[-1] == 7:
          for h in range(CONV_N):
            cv[4 * a + c, r + 8 * h:r + 8 * h + 8, :] = acc[h]
        return acc[-1]
      return [functools.partial(step, (s0, s0 + 1)) for s0 in range(0, 8, 2)]

    def out_piece(j, par, r):
      halves = []
      for h in range(2):
        rows = slice(r + 8 * h, r + 8 * h + 8)
        halves.append(_decode_outer(
            lambda o: _decode_inner([ofin[7 * o + p, rows, :] for p in range(7)])))
      for a in range(4):
        xr = pl.ds(_aligned(a * QS + r + j * QR, 16), 16)
        for k in range(4):
          cols = slice(k * 128, k * 128 + 128)
          y = jnp.concatenate([halves[0][(a, k)], halves[1][(a, k)]], axis=0)
          y = xb[b, xr, cols].astype(F32) + y
          stage[par, a, r:r + 16, cols] = y.astype(BF16)
      return y

    def ganchor(v):
      gb[3, pl.ds(pl.multiple_of(GOFF + XROWS + z, 8), 8), :] = v

    def zanchor(v):
      anchor(sb, SL_DUMMY)(v)
      anchor(cv, 16)(v)

    def iteration(m, do_s, do_p, do_o):
      part = functools.partial
      par = m % 2
      convs = [[(fn, anchor(gw, 16), CONV_N * 2 * 2.8, 0) for fn in conv_steps(a, c, r)]
               for a in range(4) for c in range(4) for r in range(0, QR, 8 * CONV_N)]
      outs = [[(part(out_piece, m - 2, par, r), anchor(ofin, 49), 90, 1)]
              for r in range(0, QR, 16)]
      if do_o and not do_p:
        norms, encs = norm_pieces(jnp.minimum(b + 1, nbatch - 1), z, 0, 0)
        next_rows = norms + encs
      first, zk = [[] for _ in range(5)], 0
      for j, (n_b, n_z) in enumerate(((12, 0), (9, 3), (9, 3), (10, 3), (9, 3))):
        p0 = sum((0, 12, 9, 9, 10)[:j + 1])
        bs = [part(pv_round, 1, p) for p in range(p0, p0 + n_b)] if do_o else []
        zs = [part(z_round, k) for k in range(zk, zk + n_z)] if do_p else []
        zk += n_z
        first[j] = bs + zs if j == 4 else _merge(bs, zs)
      pv_split = [0, 12, 24, 36, 49]
      for j in range(NT + 1):
        s_rounds, v_rounds = [], []
        if do_s:
          if j in (0, 4):
            s_rounds.append(part(left_round, m, range(j, j + 4)))
          for o in range(7):
            s_rounds.append(part(s_round_a, m, j, o))
            if o < 5:
              s_rounds.append(part(s_round_b, m, j, o))
        if j < 5:
          v_rounds = first[j]
        if j == 4 and (do_s or do_p):
          v_rounds.append(part(last_left_round, m, do_s, do_p))
        if do_p and j > 4:
          if j == 5:
            anchor(oacc, 49)(jnp.zeros((8, 128), F32))
            pe_a[4 * 49 + z, 0:16, :] = jnp.zeros((16, 128), BF16)
          v_rounds = [part(pv_round, 0, p) for p in range(pv_split[j - 5], pv_split[j - 4])]
        t = j - 1 if j > 0 else NT
        main = []
        for r in range(0, QR, 8):
          combs = [[(part(comb_piece, t, r, i), anchor(prs[t], PR_DUMMY),
                     30 if j else 50, 1)]
                   for i in range(2)]
          if j > 0:
            if do_p and r % 16 == 0:
              main.append([(fn, anchor(sb, SL_DUMMY), c, 1)
                           for fn, c in zip(prep_steps(t, r), PREP_COST)])
            if do_s:
              main += combs
          elif do_p:
            main += combs
            if r % 16 == 8:
              main.append([(fn, zanchor, c, 1)
                           for fn, c in zip(prep_steps(t, r - 8), PREP_Z_COST)])
        lists = [main]
        if do_s and j == 0:
          lists.append([[(part(window_piece, m, a, r), ganchor, 6, 0)]
                        for a in range(4) for r in range(0, QR + 2 * GOFF, 16)])
        j0 = 5 if do_p and not do_o else 1
        if do_s and j >= j0:
          n = len(convs) // (NT + 1 - j0)
          lists.append([[st] for g in convs[(j - j0) * n:(j - j0 + 1) * n] for st in g])
        if do_p and j == 0:
          steps = [norm_const_steps(r) for r in range(0, QR, 8)]
          seq = []
          for n in range(len(steps) + 3):
            if n < len(steps):
              seq.append([(steps[n][0], anchor(sb, SL_DUMMY), 10, None)])
            if n >= 3:
              seq.append([(steps[n - 3][1], lambda v: None, 1, None)])
          lists.append(seq)
        if do_o and not do_p and j < 5:
          lists.append(next_rows[8 * j:8 * j + 8])
        if do_o and j > 4:
          lists.append(outs[(9 * (j - 5)) // 4:(9 * (j - 4)) // 4])
        _run(_merge(s_rounds, v_rounds), _merge_groups(*lists), QR, span=0.99)

    iteration(0, True, False, False)

    @pl.when(b > 0)
    def _():
      for cp in o_copies(b - 1, NB - 2, 1) + o_copies(b - 1, NB - 1, 0, last=True):
        cp.wait()
    iteration(1, True, True, False)

    def steady(m, carry):
      @pl.when(m >= 4)
      def _():
        for cp in o_copies(b, m - 4, m % 2):
          cp.wait()
      iteration(m, True, True, True)
      for cp in o_copies(b, m - 2, m % 2):
        cp.start()
      return carry
    lax.fori_loop(2, NB, steady, None)
    for cp in o_copies(b, NB - 4, NB % 2):
      cp.wait()
    iteration(NB, False, True, True)
    for cp in o_copies(b, NB - 2, NB % 2):
      cp.start()
    for cp in o_copies(b, NB - 3, (NB + 1) % 2):
      cp.wait()

    @pl.when(b + 1 < nbatch)
    def _():
      for cp in x_copies(b + 1, 0):
        cp.wait()
    iteration(NB + 1, False, False, True)
    for cp in o_copies(b, NB - 1, (NB + 1) % 2, last=True):
      cp.start()

  def batch(b, carry):
    z = lax.shift_right_logical(b, 8)
    st = pltpu.VMEM((D + 8, D), F32)

    pl.run_scoped(functools.partial(phase1, b, z), st, st, st)

    @pl.when(b + 1 < nbatch)
    def _():
      for cp in x_copies(b + 1, 0) + x_copies(b + 1, 1):
        cp.start()
    blocks = lambda n: pltpu.VMEM((n, QR + FPAD, 128), F32)
    pl.run_scoped(
        functools.partial(phase2, b, z),
        blocks(SL_DUMMY + 1), blocks(PR_DUMMY + 1), blocks(PR_DUMMY + 1), blocks(PR_DUMMY + 1),
        pltpu.VMEM((4 * 49 + 1, QR, 128), BF16), pltpu.VMEM((4 * 49, QR, 128), BF16),
        pltpu.VMEM((49, QR, 128), BF16), blocks(50), blocks(50), blocks(17),
        pltpu.VMEM((17, QR + 2 * GOFF, 128), F32))
    return carry

  lax.fori_loop(0, nbatch, batch, None)
  for cp in o_copies(nbatch - 1, NB - 2, 1) + o_copies(nbatch - 1, NB - 1, 0, last=True):
    cp.wait()


@jax.jit
def pallas_standalone__conformer_family_branchformer__speech_kernel(
    x: jax.Array,
    w_q: jax.Array,
    w_k: jax.Array,
    w_v: jax.Array,
    w_ao: jax.Array,
    w_up: jax.Array,
    dw: jax.Array,
    w_dn: jax.Array,
    w_merge: jax.Array,
):
  nbatch = x.shape[0]
  assert x.shape[1:] == (T, D) and dw.shape == (KW, D)
  any_spec = pl.BlockSpec(memory_space=pl.ANY)
  return pl.pallas_call(
      _kernel,
      out_shape=jax.ShapeDtypeStruct(x.shape, x.dtype),
      in_specs=[any_spec] * 9,
      out_specs=any_spec,
      scratch_shapes=[
          pltpu.VMEM((nbatch, XROWS + 16, D), BF16),
          pltpu.VMEM((NB + 1, AE_ROWS, 128), BF16),
          pltpu.VMEM((NT + 1, 49, 128, 128), BF16),
          pltpu.VMEM((NT + 1, 49, 128, 128), BF16),
          pltpu.VMEM((4, GOFF + XROWS + 32, 128), F32),
          pltpu.VMEM((4, KW, 8, 128), F32),
          pltpu.VMEM((4, D, 128), BF16),
          pltpu.VMEM((D, D), BF16),
          pltpu.VMEM((D + 16, 2 * D), BF16),
          pltpu.VMEM((D + 8, D), F32),
          pltpu.VMEM((KW, D), BF16),
          pltpu.VMEM((2, 4, QR, D), BF16),
          pltpu.VMEM((4, D, 128), BF16),
          pltpu.VMEM((4, D, 128), BF16),
          pltpu.VMEM((D + 8, D), F32),
          pltpu.SemaphoreType.DMA((8,)),
          pltpu.SemaphoreType.DMA((8 * nbatch,)),
          pltpu.SemaphoreType.DMA((8,)),
      ],
      compiler_params=pltpu.CompilerParams(vmem_limit_bytes=126 * 1024 * 1024),
      name="branchformer",
  )(x, w_q, w_k, w_v, w_ao, w_up, dw, w_dn, w_merge)
```

```python
import functools

import jax
import jax.numpy as jnp
from jax import lax
import jax.experimental.pallas as pl
import jax.experimental.pallas.tpu as pltpu

F32, BF16, U32 = jnp.float32, jnp.bfloat16, jnp.uint32

T, D, KW = 4000, 512, 31
QS = 1008
QR = 144
NB = 7
NT = 8
XROWS = 3 * QS + NT * 128
AE_ROWS = 7104
GOFF = 16
EPS = 1e-5
LOG2E = 1.4426950408889634

FPAD = 8
CONV_N = 3
ENC_COST, PREP_COST, PREP_Z_COST = (35, 25, 25), (22, 32, 32, 32), (14, 24, 24, 24)

SL_U = 16 * NT
SL_M = SL_U + 16
SL_L = SL_M + 4
SL_OFF = SL_L + 4
SL_DUMMY = SL_OFF + 4
PR_RAW = 31
PR_LEFT = 36
PR_DUMMY = 40


def _enc_a(a11, a12, a21, a22):
  return [a11 + a22, a21 + a22, a11, a22, a11 + a12, a21 - a11, a12 - a22]


def _enc_b(b11, b12, b21, b22):
  return [b11 + b22, b11, b12 - b22, b21 - b11, b22, b11 + b12, b21 + b22]


_A_TERMS = ([(0, 0, 1), (1, 1, 1)], [(1, 0, 1), (1, 1, 1)], [(0, 0, 1)], [(1, 1, 1)],
            [(0, 0, 1), (0, 1, 1)], [(1, 0, 1), (0, 0, -1)], [(0, 1, 1), (1, 1, -1)])
_B_TERMS = ([(0, 0, 1), (1, 1, 1)], [(0, 0, 1)], [(0, 1, 1), (1, 1, -1)],
            [(1, 0, 1), (0, 0, -1)], [(1, 1, 1)], [(0, 0, 1), (0, 1, 1)],
            [(1, 0, 1), (1, 1, 1)])
_USE = ([((0, 0), 1), ((1, 1), 1)], [((1, 0), 1), ((1, 1), -1)],
        [((0, 1), 1), ((1, 1), 1)], [((0, 0), 1), ((1, 0), 1)],
        [((0, 0), -1), ((0, 1), 1)], [((1, 1), 1)], [((0, 0), 1)])


def _lin(terms):
  acc = None
  for v, s in terms:
    if acc is None:
      acc = v
    else:
      acc = acc + v if s > 0 else acc - v
  return acc


def _encode2(blk, terms, enc, store, outer=range(7)):
  for o in outer:
    q = [[_lin([(blk[2 * r + i][2 * c + j], s) for r, c, s in terms[o]])
          for j in range(2)] for i in range(2)]
    for p, v in enumerate(enc(q[0][0], q[0][1], q[1][0], q[1][1])):
      store(7 * o + p, v)
  return v


_A_STEPS = (([(0, 0), (1, 1)], (2, 0, 3)), ([(1, 0)], (1, 5)), ([(0, 1)], (4, 6)))
_P_STEPS = (([(0, 0)], (2,)), ([(1, 1)], (0, 3)), ([(1, 0)], (1, 5)), ([(0, 1)], (4, 6)))
_B_STEPS = (([(0, 0), (1, 1)], (1, 0, 4)), ([(0, 1)], (2, 5)), ([(1, 0)], (3, 6)))


def _encode_steps(fetch, steps, terms, enc, store):
  blk = [[None] * 4 for _ in range(4)]

  def step(quads, outer):
    for r, c in quads:
      for i in range(2):
        for j in range(2):
          blk[2 * r + i][2 * c + j] = fetch(2 * r + i, 2 * c + j)
    return _encode2(blk, terms, enc, store, outer)
  return [functools.partial(step, *st) for st in steps]


def _decode_outer(inner):
  c = {}
  for o in range(7):
    quad = inner(o)
    for qi, v in quad.items():
      for qo, s in _USE[o]:
        key = (2 * qo[0] + qi[0], 2 * qo[1] + qi[1])
        if key not in c:
          c[key] = v
        else:
          c[key] = c[key] + v if s > 0 else c[key] - v
  return c


def _decode_inner(m):
  return {(0, 0): m[0] + m[3] - m[4] + m[6], (0, 1): m[2] + m[4],
          (1, 0): m[1] + m[3], (1, 1): m[0] - m[1] + m[2] + m[5]}


def _layernorm(v):
  mean = jnp.sum(v, axis=-1, keepdims=True) * (1.0 / D)
  d = v - mean
  var = jnp.sum(d * d, axis=-1, keepdims=True) * (1.0 / D)
  return d * lax.rsqrt(var + EPS)


def _gelu(v):
  c1 = 0.7978845608028654
  inner = v * (c1 + (c1 * 0.044715) * (v * v))
  h = 0.5 * v
  return h + h * jnp.tanh(inner)


def _dot(a, b):
  return jnp.dot(a, b, preferred_element_type=F32)


def _dot_nt(a, b):
  return lax.dot_general(a, b, (((1,), (1,)), ((), ())), preferred_element_type=F32)


def _aligned(i, n):
  return i if isinstance(i, int) else pl.multiple_of(i, n)


def _ldb(ref, *idx):
  return pltpu.bitcast(ref.bitcast(U32)[idx], BF16)


def _run(rounds, pieces, rows, span=1.0):
  if not rounds:
    for fn, _, _, _ in pieces:
      fn()
    return
  per = rows // 8
  total = len(rounds) * per * span / max(1, sum(p[2] for p in pieces))
  j, done, last = 0, 0, {}
  for k, rnd in enumerate(rounds):
    res = rnd()
    while j < len(pieces) and int(done * total) < (k + 1) * per:
      r = (int(done * total) - k * per) * 8
      fn, anchor, cost, chain = pieces[j]
      pin = res[r:r + 8, 0:128]
      anchor(pin + last[chain] if chain in last else pin)
      tok = fn()
      if chain is not None:
        last[chain] = tok[0:8, 0:128]
      j += 1
      done += cost


def _merge(*lists, cost=lambda v: 1):
  keyed = []
  for n, l in enumerate(lists):
    total, done = max(1, sum(cost(v) for v in l)), 0
    for i, v in enumerate(l):
      keyed.append(((done + 0.5 * cost(v)) / total, n, i, v))
      done += cost(v)
  return [v for _, _, _, v in sorted(keyed, key=lambda e: e[:3])]


def _merge_groups(*lists):
  merged = _merge(*lists, cost=lambda g: sum(p[2] for p in g))
  return [p for g in merged for p in g]


def _kernel(x_hbm, wq_hbm, wk_hbm, wv_hbm, wao_hbm, wup_hbm, dw_hbm, wdn_hbm, wm_hbm,
            o_hbm, xb, ae, ke, ve, gb, dwb, wqk, wvom, wup, wdm, taps, stage, xa0, xa1, xf, vs,
            w_sem, x_sem, o_sem):
  nbatch = x_hbm.shape[0]
  xas = (xa0, xa1)

  def x_copies(b, part):
    cps = []
    for a in range(4):
      lo, hi = (0, 256) if part == 0 else (256, min(QS, T - a * QS))
      rows = pl.ds(a * QS + lo, hi - lo)
      cps.append(pltpu.make_async_copy(
          x_hbm.at[b, rows, :], xb.at[b, rows, :], x_sem.at[b * 8 + part * 4 + a]))
    return cps

  def o_copies(b, j, par, last=False):
    cps = []
    for a in range(4):
      n = min(QR, T - (a * QS + (NB - 1) * QR)) if last else QR
      cps.append(pltpu.make_async_copy(
          stage.at[par, a, pl.ds(0, n), :],
          o_hbm.at[b, pl.ds(a * QS + j * QR, n), :], o_sem.at[par * 4 + a]))
    return cps

  def block_fetch(src, g):
    def fetch(i, j):
      return src[i * 128 + 16 * g:i * 128 + 16 * g + 16, j * 128:j * 128 + 128].astype(F32)
    return fetch

  def encode_b(src, dst, t, g):
    def store(p, v):
      dst[t, p, 16 * g:16 * g + 16, :] = v.astype(BF16)
    return _encode_steps(block_fetch(src, g), _B_STEPS, _B_TERMS, _enc_b, store)

  def stage_anchor(ref, z):
    def put(v):
      if ref.dtype == BF16:
        ref[pl.ds(pl.multiple_of(D + z, 16), 16), 0:128] = jnp.concatenate(
            [v, v], axis=0).astype(BF16)
      else:
        ref[pl.ds(pl.multiple_of(D + z, 8), 8), 0:128] = v
    return put

  def norm_pieces(b, z, t, par):
    def norm(a, g):
      r0 = _aligned(a * QS + 16 * g + 128 * t, 16)
      xa = _layernorm(xb[b, pl.ds(r0, 16), :].astype(F32))
      rows = slice(a * 128 + 16 * g, a * 128 + 16 * g + 16)
      for k in range(4):
        xas[par][k, rows, :] = xa[:, k * 128:k * 128 + 128].astype(BF16)
      xf[rows, :] = xa

    def encode_a(g):
      pos = 128 * t + 16 * g
      j, r = pos // QR, pos % QR
      view = ae.at[j, pl.ds(_aligned(r, 16), 48 * QR + 16), :]

      def store(p, v):
        view[p * QR:p * QR + 16, :] = v.astype(BF16)
      return _encode_steps(block_fetch(xf, g), _A_STEPS, _A_TERMS, _enc_a, store)

    def xanchor(v):
      xb[0, pl.ds(pl.multiple_of(XROWS + z, 16), 16), 0:128] = jnp.concatenate(
          [v, v], axis=0).astype(BF16)
    norms = [[(functools.partial(norm, a, g), xanchor, 30, None)]
             for g in range(8) for a in range(4)]
    encs = [[(fn, stage_anchor(xf, z), c, 1) for fn, c in zip(encode_a(g), ENC_COST)]
            for g in range(8)]
    return norms, encs

  def enc_pieces(src, dst, t, z):
    return [[(fn, stage_anchor(src, z), c, 1)
             for fn, c in zip(encode_b(src, dst, t, g), ENC_COST)] for g in range(8)]

  def col_rounds(dst, fn, post=lambda v: v):
    def rnd(cols):
      res = fn(cols)
      if len(dst.shape) == 3:
        dst[cols.start // 128] = post(res)
      else:
        dst[0:D, cols] = post(res)
      return res
    return [functools.partial(rnd, slice(n * 128, n * 128 + 128)) for n in range(4)]

  def weights(wq, wk, wv, wao, wdn, wm, t1):
    srcs = (wq_hbm, wk_hbm, wv_hbm, wao_hbm, wm_hbm, wdn_hbm, wup_hbm, dw_hbm)
    dsts = (wq, wk, wv, wao, wm, wdn, wup.at[0:D, :], taps)
    cps = [pltpu.make_async_copy(s, d, w_sem.at[i])
           for i, (s, d) in enumerate(zip(srcs, dsts))]

    groups = [cps[0:2], cps[2:4], cps[4:5], cps[5:6] + x_copies(0, 0), cps[6:8],
              x_copies(0, 1), []]

    def need(i):
      for cp in groups[i]:
        cp.wait()
      for cp in groups[i + 2]:
        cp.start()
    for cp in groups[0] + groups[1]:
      cp.start()
    for b in range(nbatch):
      xb[b, T:XROWS, :] = jnp.zeros((XROWS - T, D), BF16)
    for c in range(4):
      gb[c, 0:GOFF, :] = jnp.zeros((GOFF, 128), F32)
    to_bf16 = lambda v: v.astype(BF16)
    need(0)
    _run(col_rounds(wqk, lambda c: _dot_nt(wq[...], wk[c, :]),
                    lambda v: to_bf16(v * (LOG2E * D ** -0.5))), [], D)
    need(1)
    _run(col_rounds(t1, lambda c: _dot(wv[...], wao[:, c]), to_bf16), [], D)
    need(2)
    _run(col_rounds(wvom, lambda c: _dot(t1[...], wm[0:D, c]), to_bf16), [], D)
    need(3)
    norms, encs = norm_pieces(0, None, 0, 0)
    _run(col_rounds(wdm, lambda c: _dot(wdn[...], wm[D:2 * D, c])),
         [(fn, lambda v: None, c, None) for fn, _, c, _ in _merge_groups(norms)], D, span=0.7)
    _run([], _merge_groups(encs), D)
    need(4)

  sq = pltpu.VMEM((D, D), BF16)
  pl.run_scoped(weights, sq, sq, sq, sq, sq, pltpu.VMEM((2 * D, D), BF16), sq)

  def phase1(b, z, ks, gs):
    def gate_piece(t, a, g):
      v = _layernorm(_gelu(gs[a * 128 + 8 * g:a * 128 + 8 * g + 8, :]))
      rows = pl.ds(_aligned(GOFF + a * QS + 8 * g + 128 * t, 8), 8)
      for c in range(4):
        gb[c, rows, :] = v[:, c * 128:c * 128 + 128]

    def spread_taps():
      rows = taps[...].astype(F32)
      for c in range(4):
        for k in range(KW):
          dwb[c, k] = jnp.broadcast_to(rows[k:k + 1, c * 128:c * 128 + 128], (8, 128))

    def step(t, par, first, last):
      xa = xas[par]
      wide = lambda ref, *rows: jnp.concatenate(
          [_ldb(ref, k, *rows) for k in range(4)], axis=1)
      gates = [[(functools.partial(gate_piece, t, a, g), stage_anchor(gs, z), 30, None)]
               for a in range(4) for g in range(16)]
      keys = enc_pieces(ks, ke, t, z)
      if first:
        prev_k = enc_pieces(wup, ke, NT, z) + [[(spread_taps, lambda v: None, 40, None)]]
        prev_v = enc_pieces(wdm, ve, NT, z)
      else:
        prev_k = enc_pieces(ks, ke, t - 1, z)[2:]
        prev_v = enc_pieces(vs, ve, t - 1, z)
      norms, encs = ([], []) if last else norm_pieces(b, z, t + 1, 1 - par)
      _run(col_rounds(gs, lambda c: _dot(wide(xa), wup[0:D, D + c.start:D + c.stop])),
           _merge_groups(prev_k + prev_v[:4], norms), D, span=0.95)
      _run(col_rounds(ks, lambda c: _dot_nt(
          wide(wqk), wide(xa, slice(c.start // 2, c.stop // 2), slice(None)))),
           _merge_groups(prev_v[4:], gates[:32]), D, span=0.95)
      _run(col_rounds(vs, lambda c: _dot(wide(xa), wvom[:, c])),
           _merge_groups(keys if last else encs + keys[:2], gates[32:]), D, span=0.85)

    step(0, 0, True, False)
    for cp in x_copies(b, 1):
      cp.wait()

    def pair(i, carry):
      step(2 * i + 1, 1, False, False)
      step(2 * i + 2, 0, False, False)
      return carry
    lax.fori_loop(0, (NT - 2) // 2, pair, None)
    step(NT - 1, 1, False, True)

  def phase2(b, z, sb, pr0, pr1, pr2, pe_a, pe_b, pe_z, oacc, ofin, cv, gw):
    prs = [(pr0, pr1)[t % 2] for t in range(NT)] + [pr2]
    left = [PR_LEFT + t // 2 for t in range(NT)] + [PR_LEFT]

    def anchor(ref, slot):
      def put(v):
        ref[slot + z, 0:8, :] = v
      return put

    def s_prod(m, t, o, p):
      lhs = _ldb(ae, m, pl.ds((7 * o + p) * (QR // 2), QR // 2), slice(None))
      return _dot(lhs, _ldb(ke, t, 7 * o + p))

    raw = [(o, p) for o in (5, 6) for p in (0, 2, 4)]

    def s_round_a(m, t, o):
      m2, m4, m6, m7 = [s_prod(m, t, o, p) for p in (1, 3, 5, 6)]
      pr = prs[t]
      pr[3 * o, 0:QR, :] = m4 + m7
      pr[3 * o + 1, 0:QR, :] = m2 + m4
      pr[3 * o + 2, 0:QR, :] = m6 - m2
      return m7

    def s_round_b(m, t, o):
      m1, m3, m5 = [s_prod(m, t, o, p) for p in (0, 2, 4)]
      extra = s_prod(m, t, *raw[o])
      pr = prs[t]
      pr[21 + 2 * o, 0:QR, :] = m1 - m5
      pr[22 + 2 * o, 0:QR, :] = m3 + m5
      pr[PR_RAW + o, 0:QR, :] = extra
      return extra

    def z_round(k):
      for p in range(4 * k, 4 * k + 4):
        res = _dot(_ldb(pe_z, p), _ldb(ve, NT, p))
        oacc[p, 0:QR, :] = res
      return res

    def left_round(m, tiles):
      for t in tiles:
        res = s_prod(m, t, *raw[5])
        prs[t][left[t], 0:QR, :] = res
      return res

    def last_left_round(m, do_s, do_z):
      outs = []
      for lo, hi in ((0, 80), (80, QR)):
        if do_s:
          lhs = _ldb(ae, m, pl.ds(46 * (QR // 2) + lo // 2, (hi - lo) // 2), slice(None))
          res = _dot(lhs, _ldb(ke, NT, 46))
          prs[NT][left[NT], lo:hi, :] = res
        if do_z:
          res = _dot(_ldb(pe_z, 48, slice(lo // 2, hi // 2), slice(None)), _ldb(ve, NT, 48))
          oacc[48, lo:hi, :] = res
        outs.append(res)
      return jnp.concatenate(outs, axis=0)

    def pv_round(second, p):
      pe = pe_b if second else pe_a
      lhs = jnp.concatenate([_ldb(pe, 49 * i + p) for i in range(4)], axis=1)
      rhs = jnp.concatenate([_ldb(ve, 4 * second + i, p) for i in range(4)], axis=0)
      res = _dot(lhs, rhs)
      (ofin if second else oacc)[p, 0:QR, :] = oacc[p, 0:QR, :] + res
      return res

    def comb_piece(t, r, i):
      rows = slice(r, r + 8)
      pr = prs[t]

      def inner(o):
        if o < 5:
          xx, yy = pr[21 + 2 * o, rows, :], pr[22 + 2 * o, rows, :]
        else:
          slots = [PR_RAW + n if n < 5 else left[t]
                   for n in range(3 * (o - 5), 3 * (o - 5) + 3)]
          m1, m3, m5 = [pr[n, rows, :] for n in slots]
          xx, yy = m1 - m5, m3 + m5
        if i == 0:
          return {(0, 0): xx + pr[3 * o, rows, :], (0, 1): yy}
        return {(1, 0): pr[3 * o + 1, rows, :], (1, 1): xx + yy + pr[3 * o + 2, rows, :]}
      c = _decode_outer(inner)
      if t == NT:
        for (a, k), v in c.items():
          v = _gelu(v)
          sb[SL_U + 4 * a + k, rows, :] = v
        return v
      if t == NT - 1:
        lane = lax.broadcasted_iota(jnp.int32, (8, 128), 1)
      for a in (i, i + 2):
        vs = [c[(a, k)] for k in range(4)]
        if t == NT - 1:
          vs = [jnp.where(lane < min(QS, T - k * QS) - 128 * t, v, -jnp.inf)
                for k, v in enumerate(vs)]
        for k in range(4):
          sb[16 * t + 4 * a + k, rows, :] = vs[k]
        mx = jnp.maximum(jnp.maximum(vs[0], vs[1]), jnp.maximum(vs[2], vs[3]))
        if t > 0:
          m_old = sb[SL_M + a, rows, :]
          mx = jnp.maximum(mx, m_old)
        e = [jnp.exp2(v - mx) for v in vs]
        ls = (e[0] + e[1]) + (e[2] + e[3])
        if t > 0:
          ls = ls + sb[SL_L + a, rows, :] * jnp.exp2(m_old - mx)
        sb[SL_M + a, rows, :] = mx
        sb[SL_L + a, rows, :] = ls
      return mx

    def norm_const_steps(r):
      rows = slice(r, r + 8)
      off = []

      def compute():
        for a in range(4):
          mx = sb[SL_M + a, rows, :]
          m_row = jnp.max(mx, axis=-1, keepdims=True)
          l_row = jnp.sum(sb[SL_L + a, rows, :] * jnp.exp2(mx - m_row), axis=-1, keepdims=True)
          off.append(jnp.broadcast_to(m_row + jnp.log2(l_row), (8, 128)))

      def store():
        for a in range(4):
          sb[SL_OFF + a, rows, :] = off[a]
      return compute, store

    def prep_steps(t, r):
      rows = slice(r, r + 16)

      def fetch(a, k):
        if t < NT:
          return jnp.exp2(sb[16 * t + 4 * a + k, rows, :] - sb[SL_OFF + a, rows, :])
        return sb[SL_U + 4 * a + k, rows, :] * cv[4 * a + k, rows, :]

      def store(p, v):
        if t == NT:
          pe_z[p, rows, :] = v.astype(BF16)
        else:
          (pe_a if t < 4 else pe_b)[49 * (t % 4) + p, rows, :] = v.astype(BF16)
      return _encode_steps(fetch, _P_STEPS, _A_TERMS, _enc_a, store)

    def window_piece(j, a, r):
      for c in range(4):
        v = gb[c, pl.ds(_aligned(a * QS + r + j * QR, 16), 16), :]
        gw[4 * a + c, r:r + 16, :] = v
      return v

    def conv_steps(a, c, r):
      base = GOFF - KW // 2 + r
      acc = [None] * CONV_N

      def step(shifts):
        for sh in shifts:
          ks = range(sh, KW, 8)
          g = [gw[4 * a + c, pl.ds(base + sh + 8 * i, 8), :]
               for i in range(CONV_N + len(ks) - 1)]
          for q, k in enumerate(ks):
            w = dwb[c, k]
            for h in range(CONV_N):
              v = g[h + q] * w
              acc[h] = v if acc[h] is None else acc[h] + v
        if shifts[-1] == 7:
          for h in range(CONV_N):
            cv[4 * a + c, r + 8 * h:r + 8 * h + 8, :] = acc[h]
        return acc[-1]
      return [functools.partial(step, (s0, s0 + 1)) for s0 in range(0, 8, 2)]

    def out_piece(j, par, r, i):
      rows = slice(r, r + 16)

      def inner(o):
        m = lambda p: ofin[7 * o + p, rows, :]
        if i == 0:
          m5 = m(4)
          return {(0, 0): m(0) + m(3) - m5 + m(6), (0, 1): m(2) + m5}
        m2 = m(1)
        return {(1, 0): m2 + m(3), (1, 1): m(0) - m2 + m(2) + m(5)}
      for (a, k), y in _decode_outer(inner).items():
        cols = slice(k * 128, k * 128 + 128)
        y = xb[b, pl.ds(_aligned(a * QS + r + j * QR, 16), 16), cols].astype(F32) + y
        stage[par, a, r:r + 16, cols] = y.astype(BF16)
      return y

    def ganchor(v):
      gb[3, pl.ds(pl.multiple_of(GOFF + XROWS + z, 8), 8), :] = v

    def zanchor(v):
      anchor(sb, SL_DUMMY)(v)
      anchor(cv, 16)(v)

    def iteration(m, do_s, do_p, do_o):
      part = functools.partial
      par = m % 2
      convs = [[(fn, anchor(gw, 16), CONV_N * 2 * 2.8, 0) for fn in conv_steps(a, c, r)]
               for a in range(4) for c in range(4) for r in range(0, QR, 8 * CONV_N)]
      outs = [[(part(out_piece, m - 2, par, r, i), anchor(ofin, 49), 70, 1)]
              for r in range(0, QR, 16) for i in range(2)]
      if do_o and not do_p:
        norms, encs = norm_pieces(jnp.minimum(b + 1, nbatch - 1), z, 0, 0)
        next_rows = [norms[:11], norms[11:22], norms[22:], encs[:4], encs[4:]]
      first, zk = [[] for _ in range(5)], 0
      n_bs = (25, 6, 6, 6, 6) if do_p and not do_s else (12, 9, 9, 10, 9)
      for j, (n_b, n_z) in enumerate(zip(n_bs, (0, 3, 3, 3, 3))):
        p0 = sum(n_bs[:j])
        bs = [part(pv_round, 1, p) for p in range(p0, p0 + n_b)] if do_o else []
        zs = [part(z_round, k) for k in range(zk, zk + n_z)] if do_p else []
        zk += n_z
        first[j] = bs + zs if j == 4 else _merge(bs, zs)
      pv_split = [0, 12, 24, 36, 49]
      for j in range(NT + 1):
        s_rounds, v_rounds = [], []
        if do_s:
          if j == 0:
            s_rounds += [part(left_round, m, range(0, 4)), part(left_round, m, range(4, 8))]
          for o in range(7):
            s_rounds.append(part(s_round_a, m, j, o))
            if o < 5:
              s_rounds.append(part(s_round_b, m, j, o))
        if j < 5:
          v_rounds = first[j]
        if j == 4 and (do_s or do_p):
          v_rounds.append(part(last_left_round, m, do_s, do_p))
        if do_p and j > 4:
          if j == 5:
            anchor(oacc, 49)(jnp.zeros((8, 128), F32))
            pe_a[4 * 49 + z, 0:16, :] = jnp.zeros((16, 128), BF16)
          v_rounds = [part(pv_round, 0, p) for p in range(pv_split[j - 5], pv_split[j - 4])]
        t = j - 1 if j > 0 else NT
        main = []
        for r in range(0, QR, 8):
          combs = [[(part(comb_piece, t, r, i), anchor(prs[t], PR_DUMMY),
                     30 if j else 50, 1)]
                   for i in range(2)]
          if j > 0:
            if do_p and r % 16 == 0:
              main += [[(fn, anchor(sb, SL_DUMMY), c, 1)]
                       for fn, c in zip(prep_steps(t, r), PREP_COST)]
            if do_s:
              main += combs
          elif do_p:
            main += combs
            if r % 16 == 8:
              main.append([(fn, zanchor, c, 1)
                           for fn, c in zip(prep_steps(t, r - 8), PREP_Z_COST)])
        lists = [main]
        if do_s and j == 0:
          lists.append([[(part(window_piece, m, a, r), ganchor, 6, 0)]
                        for a in range(4) for r in range(0, QR + 2 * GOFF, 16)])
        j0 = 5 if do_p and not do_o else 1
        if do_s and j >= j0:
          n = len(convs) // (NT + 1 - j0)
          lists.append([[st] for g in convs[(j - j0) * n:(j - j0 + 1) * n] for st in g])
        if do_p and j == 0:
          steps = [norm_const_steps(r) for r in range(0, QR, 8)]
          seq = []
          for n in range(len(steps) + 3):
            if n < len(steps):
              seq.append([(steps[n][0], anchor(sb, SL_DUMMY), 5, None)])
            if n >= 3:
              seq.append([(steps[n - 3][1], lambda v: None, 1, None)])
          lists.append(seq)
        if do_o and not do_p and j < 5:
          lists.append(next_rows[j])
        if do_o and j > 4:
          lists.append(outs[(18 * (j - 5)) // 4:(18 * (j - 4)) // 4])
        _run(_merge(s_rounds, v_rounds), _merge_groups(*lists), QR, span=0.99)

    iteration(0, True, False, False)

    @pl.when(b > 0)
    def _():
      for cp in o_copies(b - 1, NB - 2, 1) + o_copies(b - 1, NB - 1, 0, last=True):
        cp.wait()
    iteration(1, True, True, False)

    def steady(m, carry):
      @pl.when(m >= 4)
      def _():
        for cp in o_copies(b, m - 4, m % 2):
          cp.wait()
      iteration(m, True, True, True)
      for cp in o_copies(b, m - 2, m % 2):
        cp.start()
      return carry
    lax.fori_loop(2, NB, steady, None)
    for cp in o_copies(b, NB - 4, NB % 2):
      cp.wait()
    iteration(NB, False, True, True)
    for cp in o_copies(b, NB - 2, NB % 2):
      cp.start()
    for cp in o_copies(b, NB - 3, (NB + 1) % 2):
      cp.wait()

    @pl.when(b + 1 < nbatch)
    def _():
      for cp in x_copies(b + 1, 0):
        cp.wait()
    iteration(NB + 1, False, False, True)
    for cp in o_copies(b, NB - 1, (NB + 1) % 2, last=True):
      cp.start()

  def batch(b, carry):
    z = lax.shift_right_logical(b, 8)
    st = pltpu.VMEM((D + 8, D), F32)

    pl.run_scoped(functools.partial(phase1, b, z), st, st)

    @pl.when(b + 1 < nbatch)
    def _():
      for cp in x_copies(b + 1, 0) + x_copies(b + 1, 1):
        cp.start()
    blocks = lambda n: pltpu.VMEM((n, QR + FPAD, 128), F32)
    pl.run_scoped(
        functools.partial(phase2, b, z),
        blocks(SL_DUMMY + 1), blocks(PR_DUMMY + 1), blocks(PR_DUMMY + 1), blocks(PR_DUMMY + 1),
        pltpu.VMEM((4 * 49 + 1, QR, 128), BF16), pltpu.VMEM((4 * 49, QR, 128), BF16),
        pltpu.VMEM((49, QR, 128), BF16), blocks(50), blocks(50), blocks(17),
        pltpu.VMEM((17, QR + 2 * GOFF, 128), F32))
    return carry

  lax.fori_loop(0, nbatch, batch, None)
  for cp in o_copies(nbatch - 1, NB - 2, 1) + o_copies(nbatch - 1, NB - 1, 0, last=True):
    cp.wait()


@jax.jit
def pallas_standalone__conformer_family_branchformer__speech_kernel(
    x: jax.Array,
    w_q: jax.Array,
    w_k: jax.Array,
    w_v: jax.Array,
    w_ao: jax.Array,
    w_up: jax.Array,
    dw: jax.Array,
    w_dn: jax.Array,
    w_merge: jax.Array,
):
  nbatch = x.shape[0]
  assert x.shape[1:] == (T, D) and dw.shape == (KW, D)
  any_spec = pl.BlockSpec(memory_space=pl.ANY)
  return pl.pallas_call(
      _kernel,
      out_shape=jax.ShapeDtypeStruct(x.shape, x.dtype),
      in_specs=[any_spec] * 9,
      out_specs=any_spec,
      scratch_shapes=[
          pltpu.VMEM((nbatch, XROWS + 16, D), BF16),
          pltpu.VMEM((NB + 1, AE_ROWS, 128), BF16),
          pltpu.VMEM((NT + 1, 49, 128, 128), BF16),
          pltpu.VMEM((NT + 1, 49, 128, 128), BF16),
          pltpu.VMEM((4, GOFF + XROWS + 32, 128), F32),
          pltpu.VMEM((4, KW, 8, 128), F32),
          pltpu.VMEM((4, D, 128), BF16),
          pltpu.VMEM((D, D), BF16),
          pltpu.VMEM((D + 16, 2 * D), BF16),
          pltpu.VMEM((D + 8, D), F32),
          pltpu.VMEM((KW, D), BF16),
          pltpu.VMEM((2, 4, QR, D), BF16),
          pltpu.VMEM((4, D, 128), BF16),
          pltpu.VMEM((4, D, 128), BF16),
          pltpu.VMEM((D + 8, D), F32),
          pltpu.VMEM((D + 8, D), F32),
          pltpu.SemaphoreType.DMA((8,)),
          pltpu.SemaphoreType.DMA((8 * nbatch,)),
          pltpu.SemaphoreType.DMA((8,)),
      ],
      compiler_params=pltpu.CompilerParams(vmem_limit_bytes=126 * 1024 * 1024),
      name="branchformer",
  )(x, w_q, w_k, w_v, w_ao, w_up, dw, w_dn, w_merge)
```

```python
import functools

import jax
import jax.numpy as jnp
from jax import lax
import jax.experimental.pallas as pl
import jax.experimental.pallas.tpu as pltpu

F32, BF16, U32 = jnp.float32, jnp.bfloat16, jnp.uint32

T, D, KW = 4000, 512, 31
QS = 1008
QR = 144
NB = 7
NT = 8
XROWS = 3 * QS + NT * 128
AE_ROWS = 7104
GOFF = 16
EPS = 1e-5
LOG2E = 1.4426950408889634

FPAD = 8
CONV_N = 3
ENC_COST, PREP_COST, PREP_Z_COST = (35, 25, 25), (22, 32, 32, 32), (14, 24, 24, 24)

SL_U = 16 * NT
SL_M = SL_U + 16
SL_L = SL_M + 4
SL_OFF = SL_L + 4
SL_DUMMY = SL_OFF + 4
PR_RAW = 31
PR_LEFT = 36
PR_DUMMY = 40


def _enc_a(a11, a12, a21, a22):
  return [a11 + a22, a21 + a22, a11, a22, a11 + a12, a21 - a11, a12 - a22]


def _enc_b(b11, b12, b21, b22):
  return [b11 + b22, b11, b12 - b22, b21 - b11, b22, b11 + b12, b21 + b22]


_A_TERMS = ([(0, 0, 1), (1, 1, 1)], [(1, 0, 1), (1, 1, 1)], [(0, 0, 1)], [(1, 1, 1)],
            [(0, 0, 1), (0, 1, 1)], [(1, 0, 1), (0, 0, -1)], [(0, 1, 1), (1, 1, -1)])
_B_TERMS = ([(0, 0, 1), (1, 1, 1)], [(0, 0, 1)], [(0, 1, 1), (1, 1, -1)],
            [(1, 0, 1), (0, 0, -1)], [(1, 1, 1)], [(0, 0, 1), (0, 1, 1)],
            [(1, 0, 1), (1, 1, 1)])
_USE = ([((0, 0), 1), ((1, 1), 1)], [((1, 0), 1), ((1, 1), -1)],
        [((0, 1), 1), ((1, 1), 1)], [((0, 0), 1), ((1, 0), 1)],
        [((0, 0), -1), ((0, 1), 1)], [((1, 1), 1)], [((0, 0), 1)])


def _lin(terms):
  acc = None
  for v, s in terms:
    if acc is None:
      acc = v
    else:
      acc = acc + v if s > 0 else acc - v
  return acc


def _encode2(blk, terms, enc, store, outer=range(7)):
  for o in outer:
    q = [[_lin([(blk[2 * r + i][2 * c + j], s) for r, c, s in terms[o]])
          for j in range(2)] for i in range(2)]
    for p, v in enumerate(enc(q[0][0], q[0][1], q[1][0], q[1][1])):
      store(7 * o + p, v)
  return v


_A_STEPS = (([(0, 0), (1, 1)], (2, 0, 3)), ([(1, 0)], (1, 5)), ([(0, 1)], (4, 6)))
_P_STEPS = (([(0, 0)], (2,)), ([(1, 1)], (0, 3)), ([(1, 0)], (1, 5)), ([(0, 1)], (4, 6)))
_B_STEPS = (([(0, 0), (1, 1)], (1, 0, 4)), ([(0, 1)], (2, 5)), ([(1, 0)], (3, 6)))


def _encode_steps(fetch, steps, terms, enc, store):
  blk = [[None] * 4 for _ in range(4)]

  def step(quads, outer):
    for r, c in quads:
      for i in range(2):
        for j in range(2):
          blk[2 * r + i][2 * c + j] = fetch(2 * r + i, 2 * c + j)
    return _encode2(blk, terms, enc, store, outer)
  return [functools.partial(step, *st) for st in steps]


def _decode_outer(inner):
  c = {}
  for o in range(7):
    quad = inner(o)
    for qi, v in quad.items():
      for qo, s in _USE[o]:
        key = (2 * qo[0] + qi[0], 2 * qo[1] + qi[1])
        if key not in c:
          c[key] = v
        else:
          c[key] = c[key] + v if s > 0 else c[key] - v
  return c


def _decode_inner(m):
  return {(0, 0): m[0] + m[3] - m[4] + m[6], (0, 1): m[2] + m[4],
          (1, 0): m[1] + m[3], (1, 1): m[0] - m[1] + m[2] + m[5]}


def _layernorm(v, eps=EPS):
  mean = jnp.sum(v, axis=-1, keepdims=True) * (1.0 / D)
  d = v - mean
  var = jnp.sum(d * d, axis=-1, keepdims=True) * (1.0 / D)
  return d * lax.rsqrt(var + eps)


def _gelu2(v):
  c1 = 0.7978845608028654
  return v + v * jnp.tanh(v * (c1 + (c1 * 0.044715) * (v * v)))


def _dot(a, b):
  return jnp.dot(a, b, preferred_element_type=F32)


def _dot_nt(a, b):
  return lax.dot_general(a, b, (((1,), (1,)), ((), ())), preferred_element_type=F32)


def _aligned(i, n):
  return i if isinstance(i, int) else pl.multiple_of(i, n)


def _ldb(ref, *idx):
  return pltpu.bitcast(ref.bitcast(U32)[idx], BF16)


def _run(rounds, pieces, rows, span=1.0):
  if not rounds:
    for fn, _, _, _ in pieces:
      fn()
    return
  per = rows // 8
  total = len(rounds) * per * span / max(1, sum(p[2] for p in pieces))
  j, done, last = 0, 0, {}
  for k, rnd in enumerate(rounds):
    res = rnd()
    while j < len(pieces) and int(done * total) < (k + 1) * per:
      r = (int(done * total) - k * per) * 8
      fn, anchor, cost, chain = pieces[j]
      pin = res[r:r + 8, 0:128]
      anchor(pin + last[chain] if chain in last else pin)
      tok = fn()
      if chain is not None:
        last[chain] = tok[0:8, 0:128]
      j += 1
      done += cost


def _merge(*lists, cost=lambda v: 1):
  keyed = []
  for n, l in enumerate(lists):
    total, done = max(1, sum(cost(v) for v in l)), 0
    for i, v in enumerate(l):
      keyed.append(((done + 0.5 * cost(v)) / total, n, i, v))
      done += cost(v)
  return [v for _, _, _, v in sorted(keyed, key=lambda e: e[:3])]


def _merge_groups(*lists):
  merged = _merge(*lists, cost=lambda g: sum(p[2] for p in g))
  return [p for g in merged for p in g]


def _kernel(x_hbm, wq_hbm, wk_hbm, wv_hbm, wao_hbm, wup_hbm, dw_hbm, wdn_hbm, wm_hbm,
            o_hbm, xb, ae, ke, ve, gb, dwb, wqk, wvom, wup, wdm, taps, stage, xa0, xa1, xf, vs,
            w_sem, x_sem, o_sem):
  nbatch = x_hbm.shape[0]
  xas = (xa0, xa1)

  def x_copies(b, part):
    cps = []
    for a in range(4):
      lo, hi = (0, 256) if part == 0 else (256, min(QS, T - a * QS))
      rows = pl.ds(a * QS + lo, hi - lo)
      cps.append(pltpu.make_async_copy(
          x_hbm.at[b, rows, :], xb.at[b, rows, :], x_sem.at[b * 8 + part * 4 + a]))
    return cps

  def o_copies(b, j, par, last=False):
    cps = []
    for a in range(4):
      n = min(QR, T - (a * QS + (NB - 1) * QR)) if last else QR
      cps.append(pltpu.make_async_copy(
          stage.at[par, a, pl.ds(0, n), :],
          o_hbm.at[b, pl.ds(a * QS + j * QR, n), :], o_sem.at[par * 4 + a]))
    return cps

  def block_fetch(src, g):
    def fetch(i, j):
      return src[i * 128 + 16 * g:i * 128 + 16 * g + 16, j * 128:j * 128 + 128].astype(F32)
    return fetch

  def encode_b(src, dst, t, g):
    def store(p, v):
      dst[t, p, 16 * g:16 * g + 16, :] = v.astype(BF16)
    return _encode_steps(block_fetch(src, g), _B_STEPS, _B_TERMS, _enc_b, store)

  def stage_anchor(ref, z):
    def put(v):
      if ref.dtype == BF16:
        ref[pl.ds(pl.multiple_of(D + z, 16), 16), 0:128] = jnp.concatenate(
            [v, v], axis=0).astype(BF16)
      else:
        ref[pl.ds(pl.multiple_of(D + z, 8), 8), 0:128] = v
    return put

  def norm_pieces(b, z, t, par):
    def norm(a, g):
      r0 = _aligned(a * QS + 16 * g + 128 * t, 16)
      xa = _layernorm(xb[b, pl.ds(r0, 16), :].astype(F32))
      rows = slice(a * 128 + 16 * g, a * 128 + 16 * g + 16)
      for k in range(4):
        xas[par][k, rows, :] = xa[:, k * 128:k * 128 + 128].astype(BF16)
      xf[rows, :] = xa

    def encode_a(g):
      pos = 128 * t + 16 * g
      j, r = pos // QR, pos % QR
      view = ae.at[j, pl.ds(_aligned(r, 16), 48 * QR + 16), :]

      def store(p, v):
        view[p * QR:p * QR + 16, :] = v.astype(BF16)
      return _encode_steps(block_fetch(xf, g), _A_STEPS, _A_TERMS, _enc_a, store)

    def xanchor(v):
      xb[0, pl.ds(pl.multiple_of(XROWS + z, 16), 16), 0:128] = jnp.concatenate(
          [v, v], axis=0).astype(BF16)
    norms = [[(functools.partial(norm, a, g), xanchor, 30, None)]
             for g in range(8) for a in range(4)]
    encs = [[(fn, stage_anchor(xf, z), c, 1) for fn, c in zip(encode_a(g), ENC_COST)]
            for g in range(8)]
    return norms, encs

  def enc_pieces(src, dst, t, z):
    return [[(fn, stage_anchor(src, z), c, 1)
             for fn, c in zip(encode_b(src, dst, t, g), ENC_COST)] for g in range(8)]

  def col_rounds(dst, fn, post=lambda v: v):
    def rnd(cols):
      res = fn(cols)
      if len(dst.shape) == 3:
        dst[cols.start // 128] = post(res)
      else:
        dst[0:D, cols] = post(res)
      return res
    return [functools.partial(rnd, slice(n * 128, n * 128 + 128)) for n in range(4)]

  def weights(wq, wk, wv, wao, wdn, wm, t1):
    srcs = (wq_hbm, wk_hbm, wv_hbm, wao_hbm, wm_hbm, wdn_hbm, wup_hbm, dw_hbm)
    dsts = (wq, wk, wv, wao, wm, wdn, wup.at[0:D, :], taps)
    cps = [pltpu.make_async_copy(s, d, w_sem.at[i])
           for i, (s, d) in enumerate(zip(srcs, dsts))]

    groups = [cps[0:2], cps[2:4], cps[4:5], cps[5:6] + x_copies(0, 0), cps[6:8],
              x_copies(0, 1), []]

    def need(i):
      for cp in groups[i]:
        cp.wait()
      for cp in groups[i + 2]:
        cp.start()
    for cp in groups[0] + groups[1]:
      cp.start()
    for b in range(nbatch):
      xb[b, T:XROWS, :] = jnp.zeros((XROWS - T, D), BF16)
    for c in range(4):
      gb[c, 0:GOFF, :] = jnp.zeros((GOFF, 128), F32)
      gb[c, GOFF + 4 * QS:GOFF + XROWS, :] = jnp.zeros((XROWS - 4 * QS, 128), F32)
    to_bf16 = lambda v: v.astype(BF16)
    need(0)
    _run(col_rounds(wqk, lambda c: _dot_nt(wq[...], wk[c, :]),
                    lambda v: to_bf16(v * (LOG2E * D ** -0.5))), [], D)
    need(1)
    _run(col_rounds(t1, lambda c: _dot(wv[...], wao[:, c]), to_bf16), [], D)
    need(2)
    _run(col_rounds(wvom, lambda c: _dot(t1[...], wm[0:D, c]), to_bf16), [], D)
    need(3)
    norms, encs = norm_pieces(0, None, 0, 0)
    _run(col_rounds(wdm, lambda c: _dot(wdn[...], wm[D:2 * D, c])),
         [(fn, lambda v: None, c, None) for fn, _, c, _ in _merge_groups(norms)], D, span=0.7)
    _run([], _merge_groups(encs), D)
    need(4)

  sq = pltpu.VMEM((D, D), BF16)
  pl.run_scoped(weights, sq, sq, sq, sq, sq, pltpu.VMEM((2 * D, D), BF16), sq)

  def phase1(b, z, ks, gs):
    def gate_piece(t, a, g):
      v = _layernorm(_gelu2(gs[a * 128 + 8 * g:a * 128 + 8 * g + 8, :]), 4 * EPS)
      rows = pl.ds(_aligned(GOFF + a * QS + 8 * g + 128 * t, 8), 8)
      for c in range(4):
        gb[c, rows, :] = v[:, c * 128:c * 128 + 128]

    def spread_taps():
      rows = taps[...].astype(F32) * 0.5
      for c in range(4):
        for k in range(KW):
          dwb[c, k] = jnp.broadcast_to(rows[k:k + 1, c * 128:c * 128 + 128], (8, 128))

    def step(t, par, first, last):
      xa = xas[par]
      wide = lambda ref, *rows: jnp.concatenate(
          [_ldb(ref, k, *rows) for k in range(4)], axis=1)
      gates = [[(functools.partial(gate_piece, t, a, g), stage_anchor(gs, z), 30, None)]
               for a in range(4) for g in range(16)]
      keys = enc_pieces(ks, ke, t, z)
      if last:
        n = QS % 128
        gates = [gt for i, gt in enumerate(gates) if i % 16 < n // 8]

        def row_rounds(dst, w):
          def rnd(cols):
            lhs = jnp.concatenate([wide(xa, slice(64 * a, 64 * a + n // 2), slice(None))
                                   for a in range(4)], axis=0)
            res = _dot(lhs, w(cols))
            for a in range(4):
              dst[128 * a:128 * a + n, cols] = res[n * a:n * a + n]
            return res
          return [functools.partial(rnd, slice(c * 128, c * 128 + 128)) for c in range(4)]
      else:
        n = 128
        row_rounds = lambda dst, w: col_rounds(dst, lambda c: _dot(wide(xa), w(c)))
      if first:
        prev_k = enc_pieces(wup, ke, NT, z) + [[(spread_taps, lambda v: None, 40, None)]]
        prev_v = enc_pieces(wdm, ve, NT, z)
      else:
        prev_k = enc_pieces(ks, ke, t - 1, z)[2:]
        prev_v = enc_pieces(vs, ve, t - 1, z)
      norms, encs = ([], []) if last else norm_pieces(b, z, t + 1, 1 - par)
      _run(row_rounds(gs, lambda c: wup[0:D, D + c.start:D + c.stop]),
           _merge_groups(prev_k + prev_v[:4], norms), 4 * n, span=0.95)
      _run(col_rounds(ks, lambda c: _dot_nt(
          wide(wqk), wide(xa, slice(c.start // 2, c.stop // 2), slice(None)))),
           _merge_groups(prev_v[4:], gates[:32]), D, span=0.95)
      _run(row_rounds(vs, lambda c: wvom[:, c]),
           _merge_groups(keys if last else encs + keys[:2], gates[32:]), 4 * n, span=0.85)

    step(0, 0, True, False)
    for cp in x_copies(b, 1):
      cp.wait()

    def pair(i, carry):
      step(2 * i + 1, 1, False, False)
      step(2 * i + 2, 0, False, False)
      return carry
    lax.fori_loop(0, (NT - 2) // 2, pair, None)
    step(NT - 1, 1, False, True)

  def phase2(b, z, sb, pr0, pr1, pr2, pe_a, pe_b, pe_z, oacc, ofin, cv, gw):
    prs = [(pr0, pr1)[t % 2] for t in range(NT)] + [pr2]
    left = [PR_LEFT + t // 2 for t in range(NT)] + [PR_LEFT]

    def anchor(ref, slot):
      def put(v):
        ref[slot + z, 0:8, :] = v
      return put

    def s_prod(m, t, o, p):
      lhs = _ldb(ae, m, pl.ds((7 * o + p) * (QR // 2), QR // 2), slice(None))
      return _dot(lhs, _ldb(ke, t, 7 * o + p))

    raw = [(o, p) for o in (5, 6) for p in (0, 2, 4)]

    def s_round_a(m, t, o):
      m2, m4, m6, m7 = [s_prod(m, t, o, p) for p in (1, 3, 5, 6)]
      pr = prs[t]
      pr[3 * o, 0:QR, :] = m4 + m7
      pr[3 * o + 1, 0:QR, :] = m2 + m4
      pr[3 * o + 2, 0:QR, :] = m6 - m2
      return m7

    def s_round_b(m, t, o):
      m1, m3, m5 = [s_prod(m, t, o, p) for p in (0, 2, 4)]
      extra = s_prod(m, t, *raw[o])
      pr = prs[t]
      pr[21 + 2 * o, 0:QR, :] = m1 - m5
      pr[22 + 2 * o, 0:QR, :] = m3 + m5
      pr[PR_RAW + o, 0:QR, :] = extra
      return extra

    def z_round(k):
      for p in range(4 * k, 4 * k + 4):
        res = _dot(_ldb(pe_z, p), _ldb(ve, NT, p))
        oacc[p, 0:QR, :] = res
      return res

    def left_round(m, tiles):
      for t in tiles:
        res = s_prod(m, t, *raw[5])
        prs[t][left[t], 0:QR, :] = res
      return res

    def last_left_round(m, do_s, do_z):
      outs = []
      for lo, hi in ((0, 80), (80, QR)):
        if do_s:
          lhs = _ldb(ae, m, pl.ds(46 * (QR // 2) + lo // 2, (hi - lo) // 2), slice(None))
          res = _dot(lhs, _ldb(ke, NT, 46))
          prs[NT][left[NT], lo:hi, :] = res
        if do_z:
          res = _dot(_ldb(pe_z, 48, slice(lo // 2, hi // 2), slice(None)), _ldb(ve, NT, 48))
          oacc[48, lo:hi, :] = res
        outs.append(res)
      return jnp.concatenate(outs, axis=0)

    def pv_round(second, p):
      pe = pe_b if second else pe_a
      lhs = jnp.concatenate([_ldb(pe, 49 * i + p) for i in range(4)], axis=1)
      rhs = jnp.concatenate([_ldb(ve, 4 * second + i, p) for i in range(4)], axis=0)
      res = _dot(lhs, rhs)
      (ofin if second else oacc)[p, 0:QR, :] = oacc[p, 0:QR, :] + res
      return res

    def comb_piece(t, r, i):
      rows = slice(r, r + 8)
      pr = prs[t]

      def inner(o):
        if o < 5:
          xx, yy = pr[21 + 2 * o, rows, :], pr[22 + 2 * o, rows, :]
        else:
          slots = [PR_RAW + n if n < 5 else left[t]
                   for n in range(3 * (o - 5), 3 * (o - 5) + 3)]
          m1, m3, m5 = [pr[n, rows, :] for n in slots]
          xx, yy = m1 - m5, m3 + m5
        if i == 0:
          return {(0, 0): xx + pr[3 * o, rows, :], (0, 1): yy}
        return {(1, 0): pr[3 * o + 1, rows, :], (1, 1): xx + yy + pr[3 * o + 2, rows, :]}
      c = _decode_outer(inner)
      if t == NT:
        for (a, k), v in c.items():
          v = _gelu2(v)
          sb[SL_U + 4 * a + k, rows, :] = v
        return v
      if t == NT - 1:
        lane = lax.broadcasted_iota(jnp.int32, (8, 128), 1)
      for a in (i, i + 2):
        vs = [c[(a, k)] for k in range(4)]
        if t == NT - 1:
          vs = [jnp.where(lane < min(QS, T - k * QS) - 128 * t, v, -jnp.inf)
                for k, v in enumerate(vs)]
        for k in range(4):
          sb[16 * t + 4 * a + k, rows, :] = vs[k]
        mx = jnp.maximum(jnp.maximum(vs[0], vs[1]), jnp.maximum(vs[2], vs[3]))
        if t > 0:
          m_old = sb[SL_M + a, rows, :]
          mx = jnp.maximum(mx, m_old)
        e = [jnp.exp2(v - mx) for v in vs]
        ls = (e[0] + e[1]) + (e[2] + e[3])
        if t > 0:
          ls = ls + sb[SL_L + a, rows, :] * jnp.exp2(m_old - mx)
        sb[SL_M + a, rows, :] = mx
        sb[SL_L + a, rows, :] = ls
      return mx

    def norm_const_steps(r):
      rows = slice(r, r + 8)
      off = []

      def compute():
        for a in range(4):
          mx = sb[SL_M + a, rows, :]
          m_row = jnp.max(mx, axis=-1, keepdims=True)
          l_row = jnp.sum(sb[SL_L + a, rows, :] * jnp.exp2(mx - m_row), axis=-1, keepdims=True)
          off.append(jnp.broadcast_to(m_row + jnp.log2(l_row), (8, 128)))

      def store():
        for a in range(4):
          sb[SL_OFF + a, rows, :] = off[a]
      return compute, store

    def prep_steps(t, r):
      rows = slice(r, r + 16)

      def fetch(a, k):
        if t < NT:
          return jnp.exp2(sb[16 * t + 4 * a + k, rows, :] - sb[SL_OFF + a, rows, :])
        return sb[SL_U + 4 * a + k, rows, :] * cv[4 * a + k, rows, :]

      def store(p, v):
        if t == NT:
          pe_z[p, rows, :] = v.astype(BF16)
        else:
          (pe_a if t < 4 else pe_b)[49 * (t % 4) + p, rows, :] = v.astype(BF16)
      return _encode_steps(fetch, _P_STEPS, _A_TERMS, _enc_a, store)

    def window_piece(j, a, r):
      for c in range(4):
        v = gb[c, pl.ds(_aligned(a * QS + r + j * QR, 16), 16), :]
        gw[4 * a + c, r:r + 16, :] = v
      return v

    def conv_steps(a, c, r):
      base = GOFF - KW // 2 + r
      acc = [None] * CONV_N

      def step(shifts):
        for sh in shifts:
          ks = range(sh, KW, 8)
          g = [gw[4 * a + c, pl.ds(base + sh + 8 * i, 8), :]
               for i in range(CONV_N + len(ks) - 1)]
          for q, k in enumerate(ks):
            w = dwb[c, k]
            for h in range(CONV_N):
              v = g[h + q] * w
              acc[h] = v if acc[h] is None else acc[h] + v
        if shifts[-1] == 7:
          for h in range(CONV_N):
            cv[4 * a + c, r + 8 * h:r + 8 * h + 8, :] = acc[h]
        return acc[-1]
      return [functools.partial(step, (s0, s0 + 1)) for s0 in range(0, 8, 2)]

    def out_piece(j, par, r, i):
      rows = slice(r, r + 16)

      def inner(o):
        m = lambda p: ofin[7 * o + p, rows, :]
        if i == 0:
          m5 = m(4)
          return {(0, 0): m(0) + m(3) - m5 + m(6), (0, 1): m(2) + m5}
        m2 = m(1)
        return {(1, 0): m2 + m(3), (1, 1): m(0) - m2 + m(2) + m(5)}
      for (a, k), y in _decode_outer(inner).items():
        cols = slice(k * 128, k * 128 + 128)
        y = xb[b, pl.ds(_aligned(a * QS + r + j * QR, 16), 16), cols].astype(F32) + y
        stage[par, a, r:r + 16, cols] = y.astype(BF16)
      return y

    def ganchor(v):
      gb[3, pl.ds(pl.multiple_of(GOFF + XROWS + z, 8), 8), :] = v

    def zanchor(v):
      anchor(sb, SL_DUMMY)(v)
      anchor(cv, 16)(v)

    def iteration(m, do_s, do_p, do_o):
      part = functools.partial
      par = m % 2
      convs = [[(fn, anchor(gw, 16), CONV_N * 2 * 2.8, 0) for fn in conv_steps(a, c, r)]
               for a in range(4) for c in range(4) for r in range(0, QR, 8 * CONV_N)]
      outs = [[(part(out_piece, m - 2, par, r, i), anchor(ofin, 49), 70, 1)]
              for r in range(0, QR, 16) for i in range(2)]
      if do_o and not do_p:
        norms, encs = norm_pieces(jnp.minimum(b + 1, nbatch - 1), z, 0, 0)
        next_rows = [norms[:11], norms[11:22], norms[22:], encs[:4], encs[4:]]
      first, zk = [[] for _ in range(5)], 0
      n_bs = (25, 6, 6, 6, 6) if do_p and not do_s else (12, 9, 9, 10, 9)
      for j, (n_b, n_z) in enumerate(zip(n_bs, (0, 3, 3, 3, 3))):
        p0 = sum(n_bs[:j])
        bs = [part(pv_round, 1, p) for p in range(p0, p0 + n_b)] if do_o else []
        zs = [part(z_round, k) for k in range(zk, zk + n_z)] if do_p else []
        zk += n_z
        first[j] = bs + zs if j == 4 else _merge(bs, zs)
      pv_split = [0, 12, 24, 36, 49]
      for j in range(NT + 1):
        s_rounds, v_rounds = [], []
        if do_s:
          if j == 0:
            s_rounds += [part(left_round, m, range(0, 4)), part(left_round, m, range(4, 8))]
          for o in range(7):
            s_rounds.append(part(s_round_a, m, j, o))
            if o < 5:
              s_rounds.append(part(s_round_b, m, j, o))
        if j < 5:
          v_rounds = first[j]
        if j == 4 and (do_s or do_p):
          v_rounds.append(part(last_left_round, m, do_s, do_p))
        if do_p and j > 4:
          if j == 5:
            anchor(oacc, 49)(jnp.zeros((8, 128), F32))
            pe_a[4 * 49 + z, 0:16, :] = jnp.zeros((16, 128), BF16)
          v_rounds = [part(pv_round, 0, p) for p in range(pv_split[j - 5], pv_split[j - 4])]
        t = j - 1 if j > 0 else NT
        main = []
        for r in range(0, QR, 8):
          combs = [[(part(comb_piece, t, r, i), anchor(prs[t], PR_DUMMY),
                     30 if j else 50, 1)]
                   for i in range(2)]
          if j > 0:
            if do_p and r % 16 == 0:
              main += [[(fn, anchor(sb, SL_DUMMY), c, 1)]
                       for fn, c in zip(prep_steps(t, r), PREP_COST)]
            if do_s:
              main += combs
          elif do_p:
            main += combs
            if r % 16 == 8:
              main.append([(fn, zanchor, c, 1)
                           for fn, c in zip(prep_steps(t, r - 8), PREP_Z_COST)])
        lists = [main]
        if do_s and j == 0:
          lists.append([[(part(window_piece, m, a, r), ganchor, 6, 0)]
                        for a in range(4) for r in range(0, QR + 2 * GOFF, 16)])
        j0 = 5 if do_p and not do_o else 1
        if do_s and j >= j0:
          n = len(convs) // (NT + 1 - j0)
          lists.append([[st] for g in convs[(j - j0) * n:(j - j0 + 1) * n] for st in g])
        if do_s and not do_p and j == 0:
          lists.append(enc_pieces(vs, ve, NT - 1, z))
        if do_p and j == 0:
          steps = [norm_const_steps(r) for r in range(0, QR, 8)]
          seq = []
          for n in range(len(steps) + 3):
            if n < len(steps):
              seq.append([(steps[n][0], anchor(sb, SL_DUMMY), 5, None)])
            if n >= 3:
              seq.append([(steps[n - 3][1], lambda v: None, 1, None)])
          lists.append(seq)
        if do_o and not do_p and j < 5:
          lists.append(next_rows[j])
        if do_o and j > 4:
          lists.append(outs[(18 * (j - 5)) // 4:(18 * (j - 4)) // 4])
        _run(_merge(s_rounds, v_rounds), _merge_groups(*lists), QR, span=0.99)

    iteration(0, True, False, False)

    @pl.when(b > 0)
    def _():
      for cp in o_copies(b - 1, NB - 2, 1) + o_copies(b - 1, NB - 1, 0, last=True):
        cp.wait()
    iteration(1, True, True, False)

    def steady(m, carry):
      @pl.when(m >= 4)
      def _():
        for cp in o_copies(b, m - 4, m % 2):
          cp.wait()
      iteration(m, True, True, True)
      for cp in o_copies(b, m - 2, m % 2):
        cp.start()
      return carry
    lax.fori_loop(2, NB, steady, None)
    for cp in o_copies(b, NB - 4, NB % 2):
      cp.wait()
    iteration(NB, False, True, True)
    for cp in o_copies(b, NB - 2, NB % 2):
      cp.start()
    for cp in o_copies(b, NB - 3, (NB + 1) % 2):
      cp.wait()

    @pl.when(b + 1 < nbatch)
    def _():
      for cp in x_copies(b + 1, 0):
        cp.wait()
    iteration(NB + 1, False, False, True)
    for cp in o_copies(b, NB - 1, (NB + 1) % 2, last=True):
      cp.start()

  def batch(b, carry):
    z = lax.shift_right_logical(b, 8)
    st = pltpu.VMEM((D + 8, D), F32)

    pl.run_scoped(functools.partial(phase1, b, z), st, st)

    @pl.when(b + 1 < nbatch)
    def _():
      for cp in x_copies(b + 1, 0) + x_copies(b + 1, 1):
        cp.start()
    blocks = lambda n: pltpu.VMEM((n, QR + FPAD, 128), F32)
    pl.run_scoped(
        functools.partial(phase2, b, z),
        blocks(SL_DUMMY + 1), blocks(PR_DUMMY + 1), blocks(PR_DUMMY + 1), blocks(PR_DUMMY + 1),
        pltpu.VMEM((4 * 49 + 1, QR, 128), BF16), pltpu.VMEM((4 * 49, QR, 128), BF16),
        pltpu.VMEM((49, QR, 128), BF16), blocks(50), blocks(50), blocks(17),
        pltpu.VMEM((17, QR + 2 * GOFF, 128), F32))
    return carry

  lax.fori_loop(0, nbatch, batch, None)
  for cp in o_copies(nbatch - 1, NB - 2, 1) + o_copies(nbatch - 1, NB - 1, 0, last=True):
    cp.wait()


@jax.jit
def pallas_standalone__conformer_family_branchformer__speech_kernel(
    x: jax.Array,
    w_q: jax.Array,
    w_k: jax.Array,
    w_v: jax.Array,
    w_ao: jax.Array,
    w_up: jax.Array,
    dw: jax.Array,
    w_dn: jax.Array,
    w_merge: jax.Array,
):
  nbatch = x.shape[0]
  assert x.shape[1:] == (T, D) and dw.shape == (KW, D)
  any_spec = pl.BlockSpec(memory_space=pl.ANY)
  return pl.pallas_call(
      _kernel,
      out_shape=jax.ShapeDtypeStruct(x.shape, x.dtype),
      in_specs=[any_spec] * 9,
      out_specs=any_spec,
      scratch_shapes=[
          pltpu.VMEM((nbatch, XROWS + 16, D), BF16),
          pltpu.VMEM((NB + 1, AE_ROWS, 128), BF16),
          pltpu.VMEM((NT + 1, 49, 128, 128), BF16),
          pltpu.VMEM((NT + 1, 49, 128, 128), BF16),
          pltpu.VMEM((4, GOFF + XROWS + 32, 128), F32),
          pltpu.VMEM((4, KW, 8, 128), F32),
          pltpu.VMEM((4, D, 128), BF16),
          pltpu.VMEM((D, D), BF16),
          pltpu.VMEM((D + 16, 2 * D), BF16),
          pltpu.VMEM((D + 8, D), F32),
          pltpu.VMEM((KW, D), BF16),
          pltpu.VMEM((2, 4, QR, D), BF16),
          pltpu.VMEM((4, D, 128), BF16),
          pltpu.VMEM((4, D, 128), BF16),
          pltpu.VMEM((D + 8, D), F32),
          pltpu.VMEM((D + 8, D), F32),
          pltpu.SemaphoreType.DMA((8,)),
          pltpu.SemaphoreType.DMA((8 * nbatch,)),
          pltpu.SemaphoreType.DMA((8,)),
      ],
      compiler_params=pltpu.CompilerParams(vmem_limit_bytes=126 * 1024 * 1024),
      name="branchformer",
  )(x, w_q, w_k, w_v, w_ao, w_up, dw, w_dn, w_merge)
```
